```python
import jax
import jax.numpy as jnp

def _softmax(x, axis=-1):
    return jax.nn.softmax(x, axis=axis)

def _gelu(x):
    return jax.nn.gelu(x, approximate=True)

def _silu(x):
    return jax.nn.silu(x)

def _sigmoid(x):
    return jax.nn.sigmoid(x)

def _layernorm(x, axis=-1, eps=1e-05):
    m = jnp.mean(x, axis=axis, keepdims=True)
    v = jnp.var(x, axis=axis, keepdims=True)
    return (x - m) / jnp.sqrt(v + eps)

def _scatter_add(tgt, idx, src, axis=0):
    return tgt.at[idx].add(src)

def _segment_sum(src, seg, n):
    return jax.ops.segment_sum(src, seg, n)

class _Rng:

    def __init__(self, key):
        self._k = key

    def _next(self):
        self._k, sub = jax.random.split(self._k)
        return sub

    def normal(self, shape):
        return jax.random.normal(self._next(), shape, dtype=jnp.bfloat16)

    def randint(self, lo, hi, shape):
        return jax.random.randint(self._next(), shape, lo, hi, dtype=jnp.int32)

    def uniform(self, shape, lo=0.0, hi=1.0):
        return jax.random.uniform(self._next(), shape, jnp.bfloat16, lo, hi)

    def permutation(self, n):
        return jax.random.permutation(self._next(), n)
kernel_name = 'gated_mix__memory_aug_recurrent_mem_tr__moe_arch_mod__prompt'

def setup_inputs():
    _rng = _Rng(jax.random.key(int.from_bytes(__import__("os").urandom(4), "little")))
    _w = lambda a: (lambda t: t.astype(jnp.bfloat16) if jnp.issubdtype(t.dtype, jnp.floating) else t)(jnp.asarray(a))

    def _A_setup():
        B, S, Dm = (1, 2048, 1024)
        H, Dh = (32, 128)
        M, seg = (8, 32)
        seg = min(seg, S)
        S = S // seg * seg
        return {'x': _w((lambda *s: _rng.normal(s) * 0.05)(B, S, Dm)), 'mem0': _w((lambda *s: _rng.normal(s) * 0.05)(B, M, Dm)), 'Wq': _w((lambda *s: _rng.normal(s) * 0.05)(Dm, H, Dh) * Dm ** (-0.5)), 'Wk': _w((lambda *s: _rng.normal(s) * 0.05)(Dm, H, Dh) * Dm ** (-0.5)), 'Wv': _w((lambda *s: _rng.normal(s) * 0.05)(Dm, H, Dh) * Dm ** (-0.5)), 'Wo': _w((lambda *s: _rng.normal(s) * 0.05)(H, Dh, Dm) * (H * Dh) ** (-0.5)), 'seg_len': seg}
    _A_in = _A_setup()

    def _B_setup():
        B, S, D, F, C = (1, 2048, 1024, 3584, 8)
        return {'x': _w((lambda *s: _rng.normal(s) * 0.05)(B, S, D)), 'w_r': _w((lambda *s: _rng.normal(s) * 0.05)(D)), 'w_gate': _w((lambda *s: _rng.normal(s) * 0.05)(D, F)), 'w_up': _w((lambda *s: _rng.normal(s) * 0.05)(D, F)), 'w_down': _w((lambda *s: _rng.normal(s) * 0.05)(F, D))}
    _B_in = _B_setup()
    return {'A_x': _A_in['x'], 'A_mem0': _A_in['mem0'], 'A_Wq': _A_in['Wq'], 'A_Wk': _A_in['Wk'], 'A_Wv': _A_in['Wv'], 'A_Wo': _A_in['Wo'], 'A_seg_len': _A_in['seg_len'], 'B_x': _B_in['x'], 'B_w_r': _B_in['w_r'], 'B_w_gate': _B_in['w_gate'], 'B_w_up': _B_in['w_up'], 'B_w_down': _B_in['w_down'], 'gate_w': _w((lambda *s: _rng.normal(s) * 0.05)(1024))}

def reference(A_x, A_mem0, A_Wq, A_Wk, A_Wv, A_Wo, A_seg_len, B_x, B_w_r, B_w_gate, B_w_up, B_w_down, gate_w):

    def _A_ref(x, mem0, Wq, Wk, Wv, Wo, seg_len):
        B, S, Dm = x.shape
        H, Dh = (Wq.shape[1], Wq.shape[2])
        M = mem0.shape[1]
        scale = Dh ** (-0.5)
        n_seg = S // seg_len
        L = M + seg_len
        idx = jnp.arange(L)
        mask = (idx[:, None] < M) | (idx[:, None] >= idx[None, :])
        mem = mem0
        outs = []
        for s in range(n_seg):
            xs = x[:, s * seg_len:(s + 1) * seg_len, :].copy()
            h = jnp.concatenate([mem, xs], axis=1)
            q = jnp.einsum('btd,dhe->bhte', h, Wq)
            k = jnp.einsum('btd,dhe->bhte', h, Wk)
            v = jnp.einsum('btd,dhe->bhte', h, Wv)
            scores = jnp.einsum('bhqe,bhke->bhqk', q, k) * scale
            scores = jnp.where(mask[None, None], scores, -1000000000.0)
            p = _softmax(scores, axis=-1)
            o = jnp.einsum('bhqk,bhke->bhqe', p, v)
            o = jnp.einsum('bhte,hed->btd', o, Wo)
            mem = o[:, :M, :].copy()
            outs.append(o[:, M:, :])
        return jnp.concatenate(outs, axis=1)

    def _B_ref(x, w_r, w_gate, w_up, w_down):
        B, S, D = x.shape
        C = 8
        r = x @ w_r
        idx = jnp.argsort(-r, axis=-1)[:, :C]
        idx_e = jnp.repeat(idx.reshape(B, C, 1), D, axis=2)
        x_sel = jnp.take_along_axis(x, idx_e, axis=1)
        g = _silu(x_sel @ w_gate)
        u = x_sel @ w_up
        y = g * u @ w_down
        r_sel = _sigmoid(jnp.take_along_axis(r, idx, axis=1))
        y = y * r_sel.reshape(B, C, 1)
        b_off = (jnp.arange(B) * S).reshape(B, 1)
        flat_idx = (idx + b_off).reshape(B * C)
        zero = (x * 0.0).reshape(B * S, D)
        upd = _scatter_add(zero, flat_idx, y.reshape(B * C, D), axis=0)
        return x + upd.reshape(B, S, D)
    x = A_x
    g = _sigmoid((x * gate_w).sum(-1, keepdims=True))
    a = _A_ref(x, A_mem0, A_Wq, A_Wk, A_Wv, A_Wo, A_seg_len)
    b = _B_ref(x, B_w_r, B_w_gate, B_w_up, B_w_down)
    return g * a + (1 - g) * b
```

```python
import functools

import jax
import jax.numpy as jnp
import numpy as np
from jax import lax
import jax.experimental.pallas as pl
import jax.experimental.pallas.tpu as pltpu

_F32 = jnp.float32
_BF16 = jnp.bfloat16
_U32 = jnp.uint32
_I32 = jnp.int32
_NN = (((1,), (0,)), ((), ()))
_NT = (((1,), (1,)), ((), ()))

_LANE = 128
_TOPK = 8
_NSLOT = 4
_B_STEP = 5
_LAG = _B_STEP


def _dot(a, b, dims=_NN):
    return lax.dot_general(a, b, dims, preferred_element_type=_F32)


def _sigmoid(v):
    return 1.0 / (1.0 + jnp.exp(-v))


def _kernel(x_hbm, mem_hbm, wq_hbm, wk_hbm, wv_hbm, wo_hbm, wr_hbm, wg_hbm, wu_hbm,
            wd_hbm, gw_hbm, out_hbm,
            xbuf, membuf, stage, wqkv, wo, wg, wu, wd, wr, gw, ring, qkv_last, obuf,
            abuf, ybuf, outbuf, idx_smem,
            sem_stage, sem_xh, sem_xt, sem_small, sem_wo, sem_b, sem_out,
            *, S, D, H, DH, M, SEG, F):
    L = M + SEG
    n_seg = S // SEG
    KT = D // _LANE
    XR = SEG - M
    HEAD = S - (n_seg - 1) * XR
    FAT = HEAD + M
    RING = ring.shape[1]
    NCH = 3 * KT
    G = H // 4
    FT = F // _LANE
    scale = DH ** (-0.5)
    w_hbm = (wq_hbm, wk_hbm, wv_hbm)
    rows_per_chunk = _LANE * H

    def stage_copy(j, kt, slot):
        return pltpu.make_async_copy(
            w_hbm[j].at[pl.ds(kt * rows_per_chunk, rows_per_chunk), :],
            stage.at[slot], sem_stage.at[slot])

    def xhead_copy(kt):
        return pltpu.make_async_copy(
            x_hbm.at[pl.ds(0, FAT), pl.ds(kt * _LANE, _LANE)],
            xbuf.at[kt, pl.ds(0, FAT), :], sem_xh.at[kt])

    def xtail_copy(kt):
        return pltpu.make_async_copy(
            x_hbm.at[pl.ds(FAT, S - FAT), pl.ds(kt * _LANE, _LANE)],
            xbuf.at[kt, pl.ds(FAT, S - FAT), :], sem_xt)

    def strip_copy(src, dst, n, sem):
        return pltpu.make_async_copy(src.at[:, pl.ds(n * _LANE, _LANE)], dst.at[n], sem)

    mem_copies = [strip_copy(mem_hbm, membuf, kt, sem_small.at[0]) for kt in range(KT)]
    wr_copy = pltpu.make_async_copy(wr_hbm, wr, sem_small.at[1])
    gw_copy = pltpu.make_async_copy(gw_hbm, gw, sem_small.at[2])
    wo_copies = [strip_copy(wo_hbm, wo, n, sem_wo) for n in range(KT)]
    b_copies = ([strip_copy(wg_hbm, wg, n, sem_b) for n in range(FT)]
                + [strip_copy(wu_hbm, wu, n, sem_b) for n in range(FT)]
                + [strip_copy(wd_hbm, wd, n, sem_b) for n in range(KT)])

    stage_copy(0, 0, 0).start()
    xhead_copy(0).start()
    for cp in mem_copies:
        cp.start()
    for c in range(1, _NSLOT):
        stage_copy(0, c, c).start()
        xhead_copy(c).start()
    for kt in range(_NSLOT, KT):
        xhead_copy(kt).start()
    wr_copy.start()
    gw_copy.start()

    stage_u = stage.bitcast(_U32)
    xbuf_u = xbuf.bitcast(_U32)
    membuf_u = membuf.bitcast(_U32)

    def relayout(slot, j, kt, db):
        hp = H // 2
        for half in range(hp // 8):
            lo, hi = [], []
            for t in range(8):
                r0 = (db * 16 + 2 * t) * hp + half * 8
                a = stage_u[slot, pl.ds(r0, 8), :]
                b = stage_u[slot, pl.ds(r0 + hp, 8), :]
                lo.append((a & np.uint32(0xFFFF)) | (b << 16))
                hi.append((a >> 16) | (b & np.uint32(0xFFFF0000)))
            lo = jnp.swapaxes(jnp.stack(lo), 0, 1)
            hi = jnp.swapaxes(jnp.stack(hi), 0, 1)
            r = pl.ds(pl.multiple_of(kt * (_LANE // 2) + db * 8, 8), 8)
            for t in range(8):
                h0 = half * 16 + 2 * t
                wqkv[j * H + h0, r, :] = lo[t]
                wqkv[j * H + h0 + 1, r, :] = hi[t]

    stage_copy(0, 0, 0).wait()
    for db in range(_LANE // 16):
        relayout(0, 0, 0, db)
    for cp in mem_copies:
        cp.wait()

    def chunk(c, carry):
        j, kt = c // KT, c % KT
        nxt = jnp.minimum(c + 1, NCH - 1)
        jn, ktn, slot_n = nxt // KT, nxt % KT, nxt % _NSLOT

        pre = c + _NSLOT
        for jj in range(3):
            @pl.when(pre // KT == jj)
            def _():
                stage_copy(jj, pre % KT, c % _NSLOT).start()

        @pl.when(jnp.logical_and(c >= 2, c < 2 + KT))
        def _():
            xtail_copy(c - 2).start()

        @pl.when(jnp.logical_and(c >= 6, c < 6 + KT))
        def _():
            strip_copy(wo_hbm, wo, c - 6, sem_wo).start()

        for i in range(4):
            @pl.when(jnp.logical_and(c >= 14, c < 14 + FT // 4))
            def _():
                strip_copy(wg_hbm, wg, (c - 14) * 4 + i, sem_b).start()

        @pl.when(c == NCH - 3)
        def _():
            for cp in b_copies[FT:]:
                cp.start()

        @pl.when(c < KT)
        def _():
            xhead_copy(kt).wait()

        @pl.when(c + 1 < NCH)
        def _():
            stage_copy(0, 0, slot_n).wait()

        lhs = pltpu.bitcast(
            jnp.concatenate([xbuf_u[kt, pl.ds(0, HEAD // 2), :], membuf_u[kt]], axis=0),
            _BF16)
        wrow = pl.ds(pl.multiple_of(kt * (_LANE // 2), _LANE // 2), _LANE // 2)
        for g in range(G):
            for i in range(4):
                t = j * H + 4 * g + i
                r = _dot(lhs, pltpu.bitcast(wqkv[t, wrow, :], _BF16))
                old = ring[t, pl.ds(0, FAT), :]
                ring[t, pl.ds(0, FAT), :] = jnp.where(kt > 0, old, 0.0) + r
            relayout(slot_n, jn, ktn, g)
        return carry

    lax.fori_loop(0, NCH, chunk, 0)

    row = lax.broadcasted_iota(_I32, (L, L), 0)
    col = lax.broadcasted_iota(_I32, (L, L), 1)
    mask = (row < M) | (row >= col)

    def probs(q, k):
        sc = jnp.where(mask, _dot(q, k, _NT) * scale, -1000000000.0)
        e = jnp.exp(sc - jnp.max(sc, axis=-1, keepdims=True))
        return e * pltpu.reciprocal(jnp.sum(e, axis=-1, keepdims=True), approx=False)

    for kt in range(KT):
        xtail_copy(kt).wait()
    wr_copy.wait()
    gw_copy.wait()
    wr8 = jnp.broadcast_to(wr[...].astype(_F32), (8, D))
    nblk = S // _LANE
    sub = lax.broadcasted_iota(_I32, (nblk, _LANE), 0)
    pos = sub * _LANE + lax.broadcasted_iota(_I32, (nblk, _LANE), 1)
    r_all = jnp.zeros((nblk, _LANE), _F32)
    for b in range(nblk):
        xb = jnp.concatenate(
            [pltpu.bitcast(xbuf_u[kt, pl.ds(b * (_LANE // 2), _LANE // 2), :], _BF16)
             for kt in range(KT)], axis=1)
        rb = _dot(wr8, xb, _NT)
        r_all = jnp.where(sub == b, jnp.concatenate([rb] * (nblk // 8), axis=0), r_all)

    def ring_seg0(t):
        return jnp.concatenate([ring[t, pl.ds(HEAD, M), :], ring[t, pl.ds(0, SEG), :]],
                               axis=0)

    p0 = [probs(ring_seg0(h), ring_seg0(H + h)) for h in range(H - 4)]
    for h in range(H - 4):
        obuf[h] = _dot(p0[h], ring_seg0(2 * H + h))
    for j in range(3):
        for i in range(4):
            qkv_last[j * 4 + i] = ring_seg0(j * H + H - 4 + i)

    r_all = r_all.astype(_BF16).astype(_F32) + 0.0
    bits = pltpu.bitcast(r_all, _I32)
    key = jnp.where(bits < 0, bits ^ np.int32(0x7FFFFFFF), bits) >> 16
    key = jnp.where(r_all != r_all, np.int32(-(1 << 15)), key).astype(_F32)
    posf = pos.astype(_F32)
    sub8 = lax.broadcasted_iota(_I32, (_TOPK, _LANE), 0)
    x_sel = [jnp.zeros((_TOPK, _LANE), _F32) for _ in range(KT)]
    r_sel = jnp.zeros((_TOPK, _LANE), _F32)
    for c in range(_TOPK):
        best = jnp.max(key)
        pick = jnp.min(jnp.where(key == best, posf, float(S)))
        hit = posf == pick
        r_c = jnp.sum(jnp.where(hit, r_all, 0.0))
        key = jnp.where(hit, -float(1 << 17), key)
        token = pick.astype(_I32)
        idx_smem[c] = token
        r_sel = jnp.where(sub8 == c, r_c, r_sel)
        base = pl.multiple_of((token // 8) * 8, 8)
        for kt in range(KT):
            grp = xbuf[kt, pl.ds(base, 8), :].astype(_F32)
            one = jnp.sum(jnp.where(sub8 == token % 8, grp, 0.0), axis=0, keepdims=True)
            x_sel[kt] = jnp.where(sub8 == c, one, x_sel[kt])
    ybuf[...] = jnp.concatenate(x_sel, axis=1)
    r_gate = _sigmoid(r_sel)

    wg_u, wu_u, wd_u, wo_u = (w.bitcast(_U32) for w in (wg, wu, wd, wo))

    def ffn():
        for cp in b_copies:
            cp.wait()
        xs = ybuf[...]
        act = []
        for n in range(FT):
            a = _dot(xs, pltpu.bitcast(wg_u[n], _BF16))
            u = _dot(xs, pltpu.bitcast(wu_u[n], _BF16))
            act.append(a * _sigmoid(a) * u)
        act = jnp.concatenate(act, axis=1)
        for n in range(KT):
            ybuf[:, pl.ds(n * _LANE, _LANE)] = (
                _dot(act, pltpu.bitcast(wd_u[n], _BF16)) * r_gate)

    srow = lax.broadcasted_iota(_I32, (SEG, _LANE), 0)

    def mix(seg):
        r0 = pl.multiple_of(seg * SEG, SEG)
        xs = [xbuf[kt, pl.ds(r0, SEG), :].astype(_F32) for kt in range(KT)]
        gwf = gw[...].astype(_F32)
        z = xs[0] * gwf[:, :_LANE]
        for kt in range(1, KT):
            z = z + xs[kt] * gwf[:, kt * _LANE:(kt + 1) * _LANE]
        g = _sigmoid(jnp.sum(z, axis=-1, keepdims=True))
        hits = [srow == idx_smem[c] - r0 for c in range(_TOPK)]
        slot = seg % abuf.shape[0]
        for kt in range(KT):
            cols = pl.ds(kt * _LANE, _LANE)
            upd = jnp.zeros((SEG, _LANE), _F32)
            for c in range(_TOPK):
                upd = jnp.where(hits[c], ybuf[pl.ds(c, 1), cols], upd)
            res = g * abuf[slot, :, cols] + (1.0 - g) * (xs[kt] + upd)
            outbuf[pl.ds(r0, SEG), cols] = res.astype(_BF16)

    def out_copy(seg, n=1):
        r0 = pl.multiple_of(seg * SEG, SEG)
        return pltpu.make_async_copy(outbuf.at[pl.ds(r0, n * SEG), :],
                                     out_hbm.at[pl.ds(r0, n * SEG), :], sem_out)

    def o_projection(seg):
        o = {h: obuf[h] for h in range(H - 4)}
        p = {}
        acc = [None] * KT
        for g in range(G):
            lhs = jnp.concatenate([o[4 * g + i] for i in range(4)], axis=1)
            for n in range(KT):
                w = pltpu.bitcast(wo_u[n, pl.ds(g * 2 * DH, 2 * DH), :], _BF16)
                r = _dot(lhs, w)
                acc[n] = r if acc[n] is None else acc[n] + r
                if g == 0 and n == 1:
                    for i in range(4):
                        p[i] = probs(qkv_last[i], qkv_last[4 + i])
            if g == 3:
                for i in range(4):
                    o[H - 4 + i] = _dot(p[i], qkv_last[8 + i])
        slot = seg % abuf.shape[0]
        for n in range(KT):
            abuf[slot, :, pl.ds(n * _LANE, _LANE)] = acc[n][M:]
        return [a[:M] for a in acc]

    def step(s, carry):
        @pl.when(s == _B_STEP)
        def _():
            ffn()

        mem = o_projection(s - 1)
        x0 = pl.multiple_of(HEAD + (s - 1) * XR, 8)
        wpos = [pl.multiple_of(lax.rem(x0 + 8 * i, RING), 8) for i in range(XR // 8)]
        rpos = pl.multiple_of(lax.rem(s * SEG, RING), SEG)
        h_in = [jnp.concatenate([mem[kt], xbuf[kt, pl.ds(x0, XR), :].astype(_F32)],
                                axis=0).astype(_BF16) for kt in range(KT)]
        qkv = {}
        p = {}

        def finish(t, r):
            for i, w in enumerate(wpos):
                ring[t, pl.ds(w, 8), :] = r[M + 8 * i:M + 8 * i + 8]
            qkv[t] = jnp.concatenate([r[:M], ring[t, pl.ds(rpos, SEG), :]], axis=0)

        def weights(t, lo, hi):
            return pltpu.bitcast(wqkv[t, pl.ds(lo * (_LANE // 2), (hi - lo) * (_LANE // 2)), :],
                                 _BF16)

        first = [j * H + h for h in range(2) for j in range(3)]
        lo = jnp.concatenate(h_in[:KT // 2], axis=1)
        hi = jnp.concatenate(h_in[KT // 2:], axis=1)
        part = [_dot(lo, weights(t, 0, KT // 2)) for t in first]
        for t, r in zip(first, part):
            finish(t, r + _dot(hi, weights(t, KT // 2, KT)))
        h_all = jnp.concatenate(h_in, axis=1)
        for g in range(G):
            for i in range(4):
                for j in range(3):
                    t = j * H + 4 * g + i
                    if t not in qkv:
                        finish(t, _dot(h_all, weights(t, 0, KT)))
                if g > 0 and i == 0:
                    for h in range(4 * g - 4, 4 * g):
                        p[h] = probs(qkv[h], qkv[H + h])
                if g > 0 and i == 2:
                    for h in range(4 * g - 4, 4 * g):
                        obuf[h] = _dot(p[h], qkv[2 * H + h])
            if g == 1:
                mix(jnp.maximum(s - _LAG, 0))
        for j in range(3):
            for i in range(4):
                qkv_last[j * 4 + i] = qkv[j * H + H - 4 + i]

        @pl.when(s >= _LAG)
        def _():
            out_copy(s - _LAG).start()
        return carry

    abuf[0] = jnp.zeros(abuf.shape[1:], _F32)
    for cp in wo_copies:
        cp.wait()
    lax.fori_loop(1, n_seg, step, 0)

    for seg in range(n_seg - _LAG, n_seg - 1):
        mix(seg)
    out_copy(n_seg - _LAG, _LAG - 1).start()
    o_projection(n_seg - 1)
    mix(n_seg - 1)
    out_copy(n_seg - 1).start()
    pltpu.make_async_copy(outbuf, out_hbm, sem_out).wait()


@functools.partial(jax.jit, static_argnames=("A_seg_len",))
def pallas_gated_mix__memory_aug_recurrent_mem_tr__moe_arch_mod__prompt_kernel(
    A_x, A_mem0, A_Wq, A_Wk, A_Wv, A_Wo, A_seg_len, B_x, B_w_r, B_w_gate, B_w_up,
    B_w_down, gate_w,
):
    del B_x
    B, S, D = A_x.shape
    _, H, DH = A_Wq.shape
    M = A_mem0.shape[1]
    SEG = int(A_seg_len)
    F = B_w_gate.shape[1]
    assert (B, DH, M, SEG) == (1, _LANE, 8, 32) and H == 32 and D == 1024 and S == 2048
    L = M + SEG
    KT, FT = D // _LANE, F // _LANE
    ring_rows = S - (S // SEG - 1) * (SEG - M) + M

    any_spec = pl.BlockSpec(memory_space=pl.ANY)
    out = pl.pallas_call(
        functools.partial(_kernel, S=S, D=D, H=H, DH=DH, M=M, SEG=SEG, F=F),
        out_shape=jax.ShapeDtypeStruct((S, D), A_x.dtype),
        in_specs=[any_spec] * 11,
        out_specs=any_spec,
        scratch_shapes=[
            pltpu.VMEM((KT, S, _LANE), _BF16),
            pltpu.VMEM((KT, M, _LANE), _BF16),
            pltpu.VMEM((_NSLOT, _LANE * H, DH), _BF16),
            pltpu.VMEM((3 * H, D // 2, DH), _U32),
            pltpu.VMEM((KT, H * DH, _LANE), _BF16),
            pltpu.VMEM((FT, D, _LANE), _BF16),
            pltpu.VMEM((FT, D, _LANE), _BF16),
            pltpu.VMEM((KT, F, _LANE), _BF16),
            pltpu.VMEM((1, D), _BF16),
            pltpu.VMEM((1, D), _BF16),
            pltpu.VMEM((3 * H, ring_rows, DH), _F32),
            pltpu.VMEM((12, L, DH), _F32),
            pltpu.VMEM((H - 4, L, DH), _F32),
            pltpu.VMEM((8, SEG, D), _F32),
            pltpu.VMEM((_TOPK, D), _F32),
            pltpu.VMEM((S, D), _BF16),
            pltpu.SMEM((_TOPK,), _I32),
            pltpu.SemaphoreType.DMA((_NSLOT,)),
            pltpu.SemaphoreType.DMA((KT,)),
            pltpu.SemaphoreType.DMA(()),
            pltpu.SemaphoreType.DMA((3,)),
            pltpu.SemaphoreType.DMA(()),
            pltpu.SemaphoreType.DMA(()),
            pltpu.SemaphoreType.DMA(()),
        ],
        compiler_params=pltpu.CompilerParams(vmem_limit_bytes=120 * 1024 * 1024),
        name="gated_mix_rmt_mod",
    )(
        A_x.reshape(S, D), A_mem0.reshape(M, D),
        A_Wq.reshape(D * H, DH), A_Wk.reshape(D * H, DH), A_Wv.reshape(D * H, DH),
        A_Wo.reshape(H * DH, D), B_w_r.reshape(1, D), B_w_gate, B_w_up, B_w_down,
        gate_w.reshape(1, D),
    )
    return out.reshape(B, S, D)
```

```python
import functools, contextlib
_SCOPES = False
def _scope(n):
    return jax.named_scope(n) if _SCOPES else contextlib.nullcontext()

import jax
import jax.numpy as jnp
import numpy as np
from jax import lax
import jax.experimental.pallas as pl
import jax.experimental.pallas.tpu as pltpu

_F32 = jnp.float32
_BF16 = jnp.bfloat16
_U32 = jnp.uint32
_I32 = jnp.int32
_NN = (((1,), (0,)), ((), ()))
_NT = (((1,), (1,)), ((), ()))

_LANE = 128
_TOPK = 8
_ANCHOR = 3
_CUTS = {1: (0, 544), 2: (0, 272, 544), 4: (0, 272, 544)}
_QKN = 0
_PVN = 4
_QKG = 5
_PVG = 6
_UNROLL = 3
_NFIRST = 6
_PVI = 2
_RBW = False
_MIX = True
_INLOOP_DMA = True
_STAGES = (1, 1, 2, 2, 2, 4, 4, 8, 8, 8, 8)
_B_STEP = 4
_LAG = _B_STEP


def _dot(a, b, dims=_NN):
    return lax.dot_general(a, b, dims, preferred_element_type=_F32)


def _aligned(i, n):
    return i if isinstance(i, int) else pl.multiple_of(i, n)


def _sigmoid(v):
    return 1.0 / (1.0 + jnp.exp(-v))


def _kernel(x_hbm, mem_hbm, wq_hbm, wk_hbm, wv_hbm, wo_hbm, wr_hbm, wg_hbm, wu_hbm,
            wd_hbm, gw_hbm, out_hbm,
            xbuf, stage, wqkv, wo, wg, wu, wd, rings, abuf, obuf, pbuf, mqkv, ybuf, membuf,
            wr, gw, gwf, idx_smem,
            sem_stage, sem_xh, sem_xt, sem_small, sem_wo, sem_b, sem_out,
            *, S, D, H, DH, M, SEG, F):
    L = M + SEG
    n_seg = S // SEG
    KT = D // _LANE
    XR = SEG - M
    HEAD = S - (n_seg - 1) * XR
    FAT = HEAD + M
    RING = rings[0].shape[1]

    def ring_at(t):
        j, h = divmod(t, H)
        return rings[h // 4].at[j * 4 + h % 4]

    NCH = 3 * KT
    G = H // 4
    FT = F // _LANE
    scale = DH ** (-0.5)
    w_hbm = (wq_hbm, wk_hbm, wv_hbm)
    HH = H // 2
    bounds = np.cumsum((0,) + _STAGES).tolist()
    stage_of = [i for i, n in enumerate(_STAGES) for _ in range(n)]

    def unit_copy(u):
        j, kt, half = u // (2 * KT), u // 2 % KT, u % 2
        return pltpu.make_async_copy(w_hbm[j].at[pl.ds(kt * _LANE, _LANE), half],
                                     stage.at[u], sem_stage.at[stage_of[u]])

    def xhead_copy(kt):
        return pltpu.make_async_copy(
            x_hbm.at[pl.ds(0, FAT), pl.ds(kt * _LANE, _LANE)],
            xbuf.at[kt, pl.ds(0, FAT), :], sem_xh.at[kt])

    def xtail_copy(kt):
        return pltpu.make_async_copy(
            x_hbm.at[pl.ds(FAT, S - FAT), pl.ds(kt * _LANE, _LANE)],
            xbuf.at[kt, pl.ds(FAT, S - FAT), :], sem_xt)

    def strip_copy(src, dst, n, sem):
        return pltpu.make_async_copy(src.at[:, pl.ds(n * _LANE, _LANE)], dst.at[n], sem)

    mem_copies = [strip_copy(mem_hbm, membuf, kt, sem_small.at[0]) for kt in range(KT)]
    wr_copy = pltpu.make_async_copy(wr_hbm, wr, sem_small.at[1])
    gw_copy = pltpu.make_async_copy(gw_hbm, gw, sem_small.at[2])
    wo_copies = [strip_copy(wo_hbm, wo, n, sem_wo) for n in range(KT)]
    b_copies = ([strip_copy(wg_hbm, wg, n, sem_b) for n in range(FT)]
                + [strip_copy(wu_hbm, wu, n, sem_b) for n in range(FT)]
                + [strip_copy(wd_hbm, wd, n, sem_b) for n in range(KT)])

    def stage_copies(i):
        units = range(bounds[i], bounds[i + 1])
        return ([xhead_copy(u // 2) for u in units if u < 2 * KT and u % 2 == 0]
                + [unit_copy(u) for u in units])

    stage_u = stage.bitcast(_U32)
    xbuf_u = xbuf.bitcast(_U32)
    membuf_u = membuf.bitcast(_U32)

    for j in range(2):
        idx_smem[j] = j * H
    first_tile = [idx_smem[j] for j in range(2)]

    sublane = lax.broadcasted_iota(_I32, (8, _LANE), 0)

    def transpose8(v):
        c = [v[0]] + [pltpu.roll(v[8 - m], 8 - m, 0) for m in range(1, 8)]
        for d in (1, 2, 4):
            c = [jnp.where((sublane & d) != 0, c[m - d], c[m]) for m in range(8)]
        return [c[0]] + [pltpu.roll(c[k], 8 - k, 0) for k in range(1, 8)]

    def relayout(u, db, odd):
        j, kt, half = u // (2 * KT), u // 2 % KT, u % 2
        words = []
        for t in range(8):
            a = stage_u[u, db * 16 + 2 * t]
            b = stage_u[u, db * 16 + 2 * t + 1]
            if odd:
                words.append((a >> 16) | (b & np.uint32(0xFFFF0000)))
            else:
                words.append((a & np.uint32(0xFFFF)) | (b << 16))
        r = pl.ds(pl.multiple_of(kt * (_LANE // 2) + db * 8 + first_tile[0], 8), 8)
        base = (first_tile[j] if isinstance(j, int) else j * H) + half * HH + odd
        for t, w in enumerate(transpose8(words)):
            wqkv[base + 2 * t, r, :] = w

    def project(j, kt0, nk, heads, nxt, n_nxt):
        lhs = jnp.concatenate(
            [pltpu.bitcast(jnp.concatenate(
                [xbuf_u[kt0 + k, pl.ds(0, HEAD // 2), :], membuf_u[kt0 + k]], axis=0), _BF16)
             for k in range(nk)], axis=1)
        wrow = pl.ds(_aligned(kt0 * (_LANE // 2), _LANE // 2), nk * (_LANE // 2))
        jobs = [(k, db, odd) for k in range(n_nxt) for db in range(_LANE // 16)
                for odd in range(2)]
        cuts = _CUTS[nk]
        parts = [(h, r0, r1) for h in heads for r0, r1 in zip(cuts[:-1], cuts[1:])]
        for i, (h, r0, r1) in enumerate(parts):
            r = _dot(lhs[r0:r1], pltpu.bitcast(wqkv[j * H + h, wrow, :], _BF16))
            dst = rings[h // 4].at[j * 4 + h % 4]
            rows = pl.ds(r0, r1 - r0)
            if not isinstance(kt0, int):
                r = r + jnp.where(kt0 > 0, dst[rows, :], 0.0)
            elif kt0 > 0:
                r = r + dst[rows, :]
            dst[rows, :] = r
            for k, db, odd in jobs[i * len(jobs) // len(parts):
                                   (i + 1) * len(jobs) // len(parts)]:
                relayout(nxt + k, db, odd)

    def start(copies):
        for cp in copies:
            cp.start()

    def wait(copies):
        for cp in copies:
            cp.wait()

    n_peel = len(_STAGES) - 4
    start(mem_copies + stage_copies(0))
    wait(mem_copies)
    start(stage_copies(1))
    wait(stage_copies(0))
    start(stage_copies(2))
    for db in range(_LANE // 16):
        relayout(0, db, 0)
        relayout(0, db, 1)
    background = {
        n_peel - 1: [xtail_copy(kt) for kt in range(KT)] + [wr_copy, gw_copy],
    }
    late = [stage_copies(len(_STAGES) - 1), wo_copies, b_copies[:FT], b_copies[FT:]]
    with _scope('peel'):
        for i in range(n_peel):
            with _scope('w%d' % i):
                wait(stage_copies(i + 1))
            start(stage_copies(i + 3))
            start(background.get(i, []))
            u0, n = bounds[i], _STAGES[i]
            heads = range(H) if n > 1 else range(u0 % 2 * HH, (u0 % 2 + 1) * HH)
            project(0, u0 // 2, max(n // 2, 1), heads, bounds[i + 1], _STAGES[i + 1])

    def half_matrix(i, carry):
        for k in range(4):
            @pl.when(i == k)
            def _():
                if k < 3:
                    wait(stage_copies(n_peel + 1 + k))
                start(late[k])
        nxt = 2 * KT + KT * jnp.minimum(i + 1, 3)
        project(1 + i // 2, i % 2 * (KT // 2), KT // 2, range(H), nxt, KT)
        return carry

    with _scope('chunks'):
        lax.fori_loop(0, 4, half_matrix, 0)

    row = lax.broadcasted_iota(_I32, (L, L), 0)
    col = lax.broadcasted_iota(_I32, (L, L), 1)
    mask = (row < M) | (row >= col)

    def probs(q, k):
        sc = jnp.where(mask, _dot(q, k, _NT) * scale, -1000000000.0)
        e = jnp.exp(sc - jnp.max(sc, axis=-1, keepdims=True))
        return e * pltpu.reciprocal(jnp.sum(e, axis=-1, keepdims=True), approx=False)

    for kt in range(KT):
        xtail_copy(kt).wait()
    wr_copy.wait()
    gw_copy.wait()
    gwf[...] = gw[...].astype(_F32)
    wrf = wr[...].astype(_F32)
    wr8 = jnp.concatenate(
        [jnp.broadcast_to(wrf[kt:kt + 1], (8, _LANE)) for kt in range(KT)], axis=1)
    nblk = S // _LANE
    sub = lax.broadcasted_iota(_I32, (nblk, _LANE), 0)
    pos = sub * _LANE + lax.broadcasted_iota(_I32, (nblk, _LANE), 1)
    r_all = jnp.zeros((nblk, _LANE), _F32)
    for b in range(nblk):
        xb = jnp.concatenate(
            [pltpu.bitcast(xbuf_u[kt, pl.ds(b * (_LANE // 2), _LANE // 2), :], _BF16)
             for kt in range(KT)], axis=1)
        rb = _dot(wr8, xb, _NT)
        r_all = jnp.where(sub == b, jnp.concatenate([rb] * (nblk // 8), axis=0), r_all)

    def ring_seg0(t):
        return jnp.concatenate([ring_at(t)[pl.ds(HEAD, M), :], ring_at(t)[pl.ds(0, SEG), :]],
                               axis=0)

    p0 = [probs(ring_seg0(h), ring_seg0(H + h)) for h in range(8)]
    for h in range(4):
        obuf[h] = _dot(p0[h], ring_seg0(2 * H + h))
        pbuf[h] = p0[4 + h]
    for t in range(3 * H):
        mqkv[t] = ring_at(t)[pl.ds(HEAD, M), :]

    r_all = r_all.astype(_BF16).astype(_F32) + 0.0
    bits = pltpu.bitcast(r_all, _I32)
    key = jnp.where(bits < 0, bits ^ np.int32(0x7FFFFFFF), bits) >> 16
    key = jnp.where(r_all != r_all, np.int32(-(1 << 15)), key).astype(_F32)
    posf = pos.astype(_F32)
    sub8 = lax.broadcasted_iota(_I32, (_TOPK, _LANE), 0)
    x_sel = [jnp.zeros((_TOPK, _LANE), _F32) for _ in range(KT)]
    r_sel = jnp.zeros((_TOPK, _LANE), _F32)
    for c in range(_TOPK):
        best = jnp.max(key)
        pick = jnp.min(jnp.where(key == best, posf, float(S)))
        hit = posf == pick
        r_c = jnp.sum(jnp.where(hit, r_all, 0.0))
        key = jnp.where(hit, -float(1 << 17), key)
        token = pick.astype(_I32)
        idx_smem[c] = token
        r_sel = jnp.where(sub8 == c, r_c, r_sel)
        base = pl.multiple_of((token // 8) * 8, 8)
        for kt in range(KT):
            grp = xbuf[kt, pl.ds(base, 8), :].astype(_F32)
            one = jnp.sum(jnp.where(sub8 == token % 8, grp, 0.0), axis=0, keepdims=True)
            x_sel[kt] = jnp.where(sub8 == c, one, x_sel[kt])
    ybuf[...] = jnp.concatenate(x_sel, axis=1)
    r_gate = _sigmoid(r_sel)

    wg_u, wu_u, wd_u, wo_u = (w.bitcast(_U32) for w in (wg, wu, wd, wo))

    def ffn():
        for cp in b_copies:
            cp.wait()
        xs = ybuf[...]
        act = []
        for n in range(FT):
            a = _dot(xs, pltpu.bitcast(wg_u[n], _BF16))
            u = _dot(xs, pltpu.bitcast(wu_u[n], _BF16))
            act.append(a * _sigmoid(a) * u)
        act = jnp.concatenate(act, axis=1)
        for n in range(KT):
            ybuf[:, pl.ds(n * _LANE, _LANE)] = (
                _dot(act, pltpu.bitcast(wd_u[n], _BF16)) * r_gate)

    srow = lax.broadcasted_iota(_I32, (SEG, _LANE), 0)

    def mix(seg):
        r0 = pl.multiple_of(seg * SEG, SEG)
        ru = pl.ds(pl.multiple_of(seg * (SEG // 2), SEG // 2), SEG // 2)
        xs = [pltpu.bitcast(xbuf_u[kt, ru, :], _BF16).astype(_F32) for kt in range(KT)]
        z = xs[0] * gwf[pl.ds(0, 1), :]
        for kt in range(1, KT):
            z = z + xs[kt] * gwf[pl.ds(kt, 1), :]
        g = _sigmoid(jnp.sum(z, axis=-1, keepdims=True))
        hits = [srow == idx_smem[c] - r0 for c in range(_TOPK)]
        slot = seg % abuf.shape[0]
        packed = []
        for kt in range(KT):
            cols = pl.ds(kt * _LANE, _LANE)
            upd = jnp.zeros((SEG, _LANE), _F32)
            for c in range(_TOPK):
                upd = jnp.where(hits[c], ybuf[pl.ds(c, 1), cols], upd)
            res = g * abuf[slot, :, cols] + (1.0 - g) * (xs[kt] + upd)
            packed.append(res.astype(_BF16))
            xbuf_u[kt, ru, :] = pltpu.bitcast(packed[-1], _U32)
        return packed

    def out_copy(seg, n=1):
        r0 = pl.multiple_of(seg * SEG, SEG)
        return [pltpu.make_async_copy(
            xbuf.at[kt, pl.ds(r0, n * SEG), :],
            out_hbm.at[pl.ds(r0, n * SEG), pl.ds(kt * _LANE, _LANE)], sem_out)
            for kt in range(KT)]

    def o_projection(seg):
        o = {h: obuf[h] for h in range(4)}
        p = {4 + h: pbuf[h] for h in range(4)}
        rows = pl.ds(pl.multiple_of(lax.rem(seg * SEG, RING), SEG), SEG)

        def tok(t):
            return jnp.concatenate([mqkv[t], ring_at(t)[rows, :]], axis=0)

        acc = [None] * KT
        for g in range(G):
            lhs = jnp.concatenate([o[4 * g + i] for i in range(4)], axis=1)
            for n in range(KT):
                if n == _QKN and g + 2 < G:
                    for h in range(4 * g + 8, 4 * g + 12):
                        p[h] = probs(tok(h), tok(H + h))
                if n == _PVN and g + 1 < G:
                    for h in range(4 * g + 4, 4 * g + 8):
                        o[h] = _dot(p[h], tok(2 * H + h))
                w = pltpu.bitcast(wo_u[n, pl.ds(g * 2 * DH, 2 * DH), :], _BF16)
                r = _dot(lhs, w)
                acc[n] = r if acc[n] is None else r + acc[n]
        slot = seg % abuf.shape[0]
        for n in range(KT):
            abuf[slot, :, pl.ds(n * _LANE, _LANE)] = acc[n][M:]
        return [a[:M] for a in acc]

    def step(s, carry, *, write):
        mem = o_projection(s - 1)
        x0 = pl.multiple_of(HEAD + (s - 1) * XR, 8)
        wpos = [pl.multiple_of(lax.rem(x0 + 8 * i, RING), 8) for i in range(XR // 8)]
        rpos = pl.multiple_of(lax.rem(s * SEG, RING), SEG)
        u0 = pl.multiple_of((HEAD - M) // 2 + (s - 1) * (XR // 2), 4)
        low = lax.broadcasted_iota(_I32, (8, _LANE), 0) < M // 2
        h_in = []
        for kt in range(KT):
            xw = xbuf_u[kt, pl.ds(u0, SEG // 2), :]
            mw = pltpu.bitcast(jnp.concatenate([mem[kt], mem[kt]], axis=0).astype(_BF16), _U32)
            h_in.append(pltpu.bitcast(
                jnp.concatenate([jnp.where(low, mw, xw[:8]), xw[8:]], axis=0), _BF16))
        qkv = {}
        p = {}
        mixed = mix(s - _LAG) if write else None
        never = s > n_seg

        def finish(t, r):
            for i, w in enumerate(wpos):
                ring_at(t)[pl.ds(w, 8), :] = r[M + 8 * i:M + 8 * i + 8]
            mqkv[t] = r[:M]
            qkv[t] = r[:M]

        def tok(t):
            return jnp.concatenate([qkv[t], ring_at(t)[pl.ds(rpos, SEG), :]], axis=0)

        def weights(t, lo, hi):
            return pltpu.bitcast(wqkv[t, pl.ds(lo * (_LANE // 2), (hi - lo) * (_LANE // 2)), :],
                                 _BF16)

        first = [j * H + h for h in range(2) for j in range(3)][:_NFIRST]
        lo = jnp.concatenate(h_in[:KT // 2], axis=1)
        hi = jnp.concatenate(h_in[KT // 2:], axis=1)
        part = [_dot(lo, weights(t, 0, KT // 2)) for t in first]
        for t, r in zip(first, part):
            finish(t, _dot(hi, weights(t, KT // 2, KT)) + r)
        h_all = jnp.concatenate(h_in, axis=1)
        for g in range(G):
            for i in range(4):
                for j in range(3):
                    t = j * H + 4 * g + i
                    if t not in qkv:
                        lhs = h_all
                        if write and i == _ANCHOR and j == 0:
                            lhs = jnp.concatenate(
                                [jnp.where(never, mixed[g], h_in[0])] + h_in[1:], axis=1)
                        finish(t, _dot(lhs, weights(t, 0, KT)))
                if g == _QKG and i == 0:
                    for h in range(4):
                        p[h] = probs(tok(h), tok(H + h))
                    for h in range(4):
                        pbuf[h] = probs(tok(4 + h), tok(H + 4 + h))
                if g == _PVG and i == 0:
                    for h in range(4):
                        obuf[h] = _dot(p[h], tok(2 * H + h))

        if write and _INLOOP_DMA:
            for cp in out_copy(s - _LAG):
                cp.start()
        return carry

    for cp in wo_copies:
        cp.wait()
    with _scope('steps0'):
        lax.fori_loop(1, _B_STEP, functools.partial(step, write=False), 0)
    with _scope('ffn'):
        ffn()
    with _scope('steps'):
        def multi(it, carry):
            for u in range(_UNROLL):
                step(_B_STEP + it * _UNROLL + u, carry, write=_MIX)
            return carry
        assert (n_seg - _B_STEP) % _UNROLL == 0
        lax.fori_loop(0, (n_seg - _B_STEP) // _UNROLL, multi, 0)

    for seg in range(n_seg - _LAG, n_seg - 1):
        mix(seg)
    for cp in (out_copy(n_seg - _LAG, _LAG - 1) if (_INLOOP_DMA and _MIX) else out_copy(0, n_seg - 1)):
        cp.start()
    o_projection(n_seg - 1)
    mix(n_seg - 1)
    for cp in out_copy(n_seg - 1):
        cp.start()
    for cp in out_copy(0, n_seg):
        cp.wait()


@functools.partial(jax.jit, static_argnames=("A_seg_len",))
def pallas_gated_mix__memory_aug_recurrent_mem_tr__moe_arch_mod__prompt_kernel(
    A_x, A_mem0, A_Wq, A_Wk, A_Wv, A_Wo, A_seg_len, B_x, B_w_r, B_w_gate, B_w_up,
    B_w_down, gate_w,
):
    del B_x
    B, S, D = A_x.shape
    _, H, DH = A_Wq.shape
    M = A_mem0.shape[1]
    SEG = int(A_seg_len)
    F = B_w_gate.shape[1]
    assert (B, DH, M, SEG) == (1, _LANE, 8, 32) and H == 32 and D == 1024 and S == 2048
    L = M + SEG
    KT, FT = D // _LANE, F // _LANE
    ring_rows = S - (S // SEG - 1) * (SEG - M) + M

    any_spec = pl.BlockSpec(memory_space=pl.ANY)
    out = pl.pallas_call(
        functools.partial(_kernel, S=S, D=D, H=H, DH=DH, M=M, SEG=SEG, F=F),
        out_shape=jax.ShapeDtypeStruct((S, D), A_x.dtype),
        in_specs=[any_spec] * 11,
        out_specs=any_spec,
        scratch_shapes=[
            pltpu.VMEM((KT, S, _LANE), _BF16),
            pltpu.VMEM((6 * KT, _LANE, H // 2, DH), _BF16),
            pltpu.VMEM((3 * H, D // 2, DH), _U32),
            pltpu.VMEM((KT, H * DH, _LANE), _BF16),
            pltpu.VMEM((FT, D, _LANE), _BF16),
            pltpu.VMEM((FT, D, _LANE), _BF16),
            pltpu.VMEM((KT, F, _LANE), _BF16),
            [pltpu.VMEM((12, ring_rows, DH), _F32)] * (H // 4),
            pltpu.VMEM((8, SEG, D), _F32),
            pltpu.VMEM((4, L, DH), _F32),
            pltpu.VMEM((4, L, L), _F32),
            pltpu.VMEM((3 * H, M, DH), _F32),
            pltpu.VMEM((_TOPK, D), _F32),
            pltpu.VMEM((KT, M, _LANE), _BF16),
            pltpu.VMEM((KT, _LANE), _BF16),
            pltpu.VMEM((KT, _LANE), _BF16),
            pltpu.VMEM((KT, _LANE), _F32),
            pltpu.SMEM((_TOPK,), _I32),
            pltpu.SemaphoreType.DMA((len(_STAGES),)),
            pltpu.SemaphoreType.DMA((KT,)),
            pltpu.SemaphoreType.DMA(()),
            pltpu.SemaphoreType.DMA((3,)),
            pltpu.SemaphoreType.DMA(()),
            pltpu.SemaphoreType.DMA(()),
            pltpu.SemaphoreType.DMA(()),
        ],
        compiler_params=pltpu.CompilerParams(vmem_limit_bytes=120 * 1024 * 1024,
                                             disable_bounds_checks=True),
        name="gated_mix_rmt_mod",
    )(
        A_x.reshape(S, D), A_mem0.reshape(M, D),
        A_Wq.reshape(D, 2, H // 2, DH), A_Wk.reshape(D, 2, H // 2, DH),
        A_Wv.reshape(D, 2, H // 2, DH),
        A_Wo.reshape(H * DH, D), B_w_r.reshape(KT, _LANE), B_w_gate, B_w_up, B_w_down,
        gate_w.reshape(KT, _LANE),
    )
    return out.reshape(B, S, D)
```

```python
import functools

import jax
import jax.numpy as jnp
import numpy as np
from jax import lax
import jax.experimental.pallas as pl
import jax.experimental.pallas.tpu as pltpu

_F32 = jnp.float32
_BF16 = jnp.bfloat16
_U32 = jnp.uint32
_I32 = jnp.int32
_NN = (((1,), (0,)), ((), ()))
_NT = (((1,), (1,)), ((), ()))

_LANE = 128
_WORDS = _LANE // 2
_TOPK = 8
_UNROLL = 3
_FFN_TILES = 5
_STAGES = (1, 1, 1, 1, 2, 2, 4, 4, 8, 8, 8, 8)
_BATCHES = (1, 1, 1, 1, 2, 2, 4, 4, 4, 4, 4, 4, 8, 8)
_EXTRA = (7,)
_QKN = 0
_PVN = 4
_QKG = 5
_PVG = 6
_NFIRST = 6


def _dot(a, b, dims=_NN):
    return lax.dot_general(a, b, dims, preferred_element_type=_F32)


def _aligned(i, n):
    return i if isinstance(i, int) else pl.multiple_of(i, n)


def _rem(i, n):
    return i % n if isinstance(i, int) else lax.rem(i, n)


def _sigmoid(v):
    return 1.0 / (1.0 + jnp.exp(-v))


def _bf16(words):
    return pltpu.bitcast(words, _BF16)


def _word_sum(a, b, sign):
    halves = []
    for k in range(2):
        u, v = (pltpu.unpack_elementwise(w, index=k, packed_dtype=_BF16, unpacked_dtype=_F32)
                for w in (a, b))
        halves.append(u + v if sign > 0 else u - v)
    return pltpu.bitcast(pltpu.pack_elementwise(halves, packed_dtype=_BF16), _U32)


def _start(copies):
    for cp in copies:
        cp.start()


def _wait(copies):
    for cp in copies:
        cp.wait()


def _kernel(x_hbm, mem_hbm, wq_hbm, wk_hbm, wv_hbm, wo_hbm, wr_hbm, wg_hbm, wu_hbm,
            wd_hbm, gw_hbm, out_hbm,
            xbuf, stage, wqkv, wo, wg, wu, wd, rings, xsum, abuf, obuf, pbuf, mqkv, xsel,
            ybuf, membuf, wr, gw, gwf, rgate, picks,
            sem_w, sem_xh, sem_xt, sem_small, sem_wo, sem_b, sem_out,
            *, S, D, H, DH, M, SEG, F):
    L = M + SEG
    n_seg = S // SEG
    KT = D // _LANE
    FT = F // _LANE
    G = H // 4
    HH = H // 2
    XR = SEG - M
    HEAD = S - (n_seg - 1) * XR
    FAT = HEAD + M
    NB = abuf.shape[0]
    w_hbm = (wq_hbm, wk_hbm, wv_hbm)

    stage_u, xbuf_u, membuf_u, wo_u, wg_u, wu_u, wd_u = (
        r.bitcast(_U32) for r in (stage, xbuf, membuf, wo, wg, wu, wd))

    def ring(t):
        j, h = divmod(t, H)
        return rings[h // 4].at[j * 4 + h % 4]

    picks[0] = 0
    never = picks[0] > 0
    sublane = lax.broadcasted_iota(_I32, (8, _LANE), 0)

    batch_start = np.cumsum((0,) + _BATCHES).tolist()
    stage_start = np.cumsum((0,) + _STAGES).tolist()

    def batch_copies(i):
        copies = []
        for u in range(batch_start[i], batch_start[i + 1]):
            j, kt, half = u // (2 * KT), u // 2 % KT, u % 2
            if j == 0 and half == 0:
                copies.append(pltpu.make_async_copy(
                    x_hbm.at[pl.ds(0, FAT), pl.ds(kt * _LANE, _LANE)],
                    xbuf.at[kt, pl.ds(0, FAT), :], sem_xh.at[kt]))
            copies.append(pltpu.make_async_copy(
                w_hbm[j].at[pl.ds(kt * _LANE, _LANE), half], stage.at[u], sem_w.at[i]))
        return copies

    def strip_copies(src, dst, tiles, sem):
        return [pltpu.make_async_copy(src.at[:, pl.ds(n * _LANE, _LANE)], dst.at[n], sem)
                for n in tiles]

    def ffn_copies(i):
        tiles = range(i * _FFN_TILES, min((i + 1) * _FFN_TILES, FT))
        rows = pl.ds(tiles[0] * _LANE, len(tiles) * _LANE)
        return (strip_copies(wg_hbm, wg, tiles, sem_b.at[i])
                + strip_copies(wu_hbm, wu, tiles, sem_b.at[i])
                + [pltpu.make_async_copy(wd_hbm.at[rows, pl.ds(n * _LANE, _LANE)],
                                         wd.at[n, rows, :], sem_b.at[i]) for n in range(KT)])

    def out_copies(seg, n=1):
        rows = pl.ds(_aligned(seg * SEG, SEG), n * SEG)
        return [pltpu.make_async_copy(xbuf.at[kt, rows, :],
                                      out_hbm.at[rows, pl.ds(kt * _LANE, _LANE)], sem_out)
                for kt in range(KT)]

    mem_copies = strip_copies(mem_hbm, membuf, range(KT), sem_small.at[0])
    vec_copies = [pltpu.make_async_copy(wr_hbm, wr, sem_small.at[1]),
                  pltpu.make_async_copy(gw_hbm, gw, sem_small.at[1])]
    xtail_copies = [pltpu.make_async_copy(
        x_hbm.at[pl.ds(FAT, S - FAT), pl.ds(kt * _LANE, _LANE)],
        xbuf.at[kt, pl.ds(FAT, S - FAT), :], sem_xt) for kt in range(KT)]
    wo_copies = strip_copies(wo_hbm, wo, range(KT), sem_wo)

    queue = [batch_copies(i) for i in range(len(_BATCHES))]
    queue += [vec_copies + xtail_copies, wo_copies, ffn_copies(0), ffn_copies(1)]
    progress = {"started": 0, "arrived": 0}

    def start_next():
        if progress["started"] < len(queue):
            _start(queue[progress["started"]])
            progress["started"] += 1

    def need_unit(u):
        while batch_start[progress["arrived"]] <= u:
            _wait(queue[progress["arrived"]])
            progress["arrived"] += 1
            start_next()

    row = lax.broadcasted_iota(_I32, (L, L), 0)
    col = lax.broadcasted_iota(_I32, (L, L), 1)
    mask = (row < M) | (row >= col)
    scale = DH ** (-0.5)

    def probs(q, k):
        sc = jnp.where(mask[L - q.shape[0]:], _dot(q, k, _NT), -1000000000.0 / scale)
        e = jnp.exp2((sc - jnp.max(sc, axis=-1, keepdims=True)) * float(scale * np.log2(np.e)))
        total = jnp.sum(e, axis=-1, keepdims=True)
        inv = pltpu.reciprocal(total, approx=True)
        return e * (inv * (2.0 - total * inv))

    n_blk = S // _LANE
    score = [None] * n_blk

    def score_job(b, half):
        kts = range(half * KT // 2, (half + 1) * KT // 2)
        wrf = wr[...].astype(_F32)
        w = jnp.concatenate([jnp.broadcast_to(wrf[kt:kt + 1], (8, _LANE)) for kt in kts],
                            axis=1)
        xb = jnp.concatenate([_bf16(xbuf_u[kt, pl.ds(b * _WORDS, _WORDS), :]) for kt in kts],
                             axis=1)
        r = _dot(w, xb, _NT)
        score[b] = r if half == 0 else r + score[b]

    def select_tokens():
        r_all = []
        for b0 in range(0, n_blk, 8):
            r = score[b0]
            for b in range(1, 8):
                r = jnp.where(sublane == b, score[b0 + b], r)
            r_all.append(r)
        r_all = jnp.concatenate(r_all, axis=0).astype(_BF16).astype(_F32)
        r_all = jnp.where(r_all == 0.0, 0.0, r_all)
        bits = pltpu.bitcast(r_all, _I32)
        key = jnp.where(bits < 0, bits ^ np.int32(0x7FFFFFFF), bits) >> 16
        key = jnp.where(r_all != r_all, np.int32(-(1 << 15)), key).astype(_F32)
        pos = (lax.broadcasted_iota(_I32, (n_blk, _LANE), 0) * _LANE
               + lax.broadcasted_iota(_I32, (n_blk, _LANE), 1)).astype(_F32)
        x_sel = [jnp.zeros((_TOPK, _LANE), _F32) for _ in range(KT)]
        r_sel = jnp.zeros((_TOPK, _LANE), _F32)
        for c in range(_TOPK):
            best = jnp.max(key, keepdims=True)
            pick = jnp.min(jnp.where(key == best, pos, float(S)), keepdims=True)
            hit = pos == pick
            key = jnp.where(hit, -float(1 << 17), key)
            r_sel = jnp.where(sublane == c,
                              jnp.sum(jnp.where(hit, r_all, 0.0), keepdims=True), r_sel)
            token = pick[0, 0].astype(_I32)
            picks[c] = token
            base = pl.multiple_of((token >> 3) << 3, 8)
            for kt in range(KT):
                grp = xbuf[kt, pl.ds(base, 8), :].astype(_F32)
                one = jnp.sum(jnp.where(sublane == (token & 7), grp, 0.0), axis=0,
                              keepdims=True)
                x_sel[kt] = jnp.where(sublane == c, one, x_sel[kt])
        xsel[...] = jnp.concatenate(x_sel, axis=1)
        rgate[...] = _sigmoid(r_sel)

    def transpose8(v):
        c = [v[0]] + [pltpu.roll(v[8 - m], 8 - m, 0) for m in range(1, 8)]
        for d in (1, 2, 4):
            c = [jnp.where((sublane & d) != 0, c[m - d], c[m]) for m in range(8)]
        return [c[0]] + [pltpu.roll(c[k], 8 - k, 0) for k in range(1, 8)]

    def relayout(u, db, odd, after=None):
        need_unit(u)
        j, kt, half = u // (2 * KT), u // 2 % KT, u % 2
        words = []
        for t in range(8):
            a = stage_u[u, db * 16 + 2 * t]
            b = stage_u[u, db * 16 + 2 * t + 1]
            if odd:
                words.append((a >> 16) | (b & np.uint32(0xFFFF0000)))
            else:
                words.append((a & np.uint32(0xFFFF)) | (b << 16))
        if after is not None:
            words[0] = jnp.where(never, after, words[0])
        for t, w in enumerate(transpose8(words)):
            wqkv[j * H + half * HH + 2 * t + odd, pl.ds(kt * _WORDS + db * 8, 8), :] = w

    def relayout_jobs(units):
        return [functools.partial(relayout, u, db, odd)
                for u in units for db in range(_LANE // 16) for odd in range(2)]

    def head_rows(kt, r0, n):
        n_x = min(n, HEAD // 2 - r0)
        rows = xbuf_u[kt, pl.ds(r0, n_x), :]
        return rows if n_x == n else jnp.concatenate([rows, membuf_u[kt]], axis=0)

    HW = FAT // 4

    def xsum_job(pair, r0, after):
        a11, a12, a21, a22 = (head_rows(2 * pair + k, half * HW + r0, 8)
                              for half in range(2) for k in range(2))
        a11, a22 = jnp.where(never, after, a11), jnp.where(never, after, a22)
        for k, w in enumerate((_word_sum(a11, a22, 1), _word_sum(a21, a22, 1), a11, a22,
                               _word_sum(a11, a12, 1), _word_sum(a21, a11, -1),
                               _word_sum(a12, a22, -1))):
            xsum[pair, k, pl.ds(r0, 8), :] = w

    def xsum_jobs(pairs):
        return [functools.partial(xsum_job, pair, r0)
                for pair in pairs for r0 in range(0, HW, 8)]

    def run_jobs(jobs, i, n, result):
        mine = jobs[i * len(jobs) // n:(i + 1) * len(jobs) // n]
        for k, job in enumerate(mine):
            r0 = k * (result.shape[0] // 8) // len(mine) * 8
            job(pltpu.bitcast(result[r0:r0 + 8], _U32))

    def project(j, kt, heads, jobs):
        lhs = _bf16(head_rows(kt, 0, FAT // 2))
        for i, h in enumerate(heads):
            r = _dot(lhs, _bf16(wqkv[j * H + h, pl.ds(kt * _WORDS, _WORDS), :]))
            dst = ring(j * H + h)
            dst[...] = r + dst[...] if kt > 0 else r
            if i % 4 == 3:
                run_jobs(jobs, i // 4, len(heads) // 4, r)

    def project_strassen(j, pairs, jobs, side=(), done=()):
        def product(k, b):
            return _dot(jnp.concatenate([_bf16(xsum[p, k]) for p in pairs], axis=1), _bf16(b))

        def block(h, k):
            return jnp.concatenate(
                [wqkv[j * H + h, pl.ds((2 * p + k) * _WORDS, _WORDS), :] for p in pairs],
                axis=0)

        def add(h, half, v, first=False, sign=1):
            rows = pl.ds(half * (FAT // 2), FAT // 2)
            dst = ring(j * H + h)
            if first and pairs[0] == 0:
                dst[rows, :] = v if sign > 0 else -v
            else:
                dst[rows, :] = dst[rows, :] + v if sign > 0 else dst[rows, :] - v

        slot = [0]

        def after(m):
            run_jobs(jobs, slot[0], 7 * G, m)
            if slot[0] in side:
                side[slot[0]]()
            slot[0] += 1

        for g in range(G):
            for h in (4 * g, 4 * g + 2):
                m2 = product(1, block(h, 0))
                m5 = product(4, block(h + 1, 1))
                if len(pairs) > 1:
                    add(h, 1, m2, True), add(h + 1, 1, m2, True, -1)
                    add(h, 0, m5, True, -1), add(h + 1, 0, m5, True)
                after(m2)
                m1 = product(0, _word_sum(block(h, 0), block(h + 1, 1), 1))
                m4 = product(3, _word_sum(block(h, 1), block(h, 0), -1))
                if len(pairs) > 1:
                    add(h, 0, m1 + m4), add(h + 1, 1, m1), add(h, 1, m4)
                else:
                    add(h, 0, m1 + m4 - m5, True), add(h + 1, 1, m1 - m2, True)
                    add(h, 1, m2 + m4, True), add(h + 1, 0, m5, True)
                after(m1)
                m3 = product(2, _word_sum(block(h + 1, 0), block(h + 1, 1), -1))
                m6 = product(5, _word_sum(block(h, 0), block(h + 1, 0), 1))
                add(h + 1, 0, m3), add(h + 1, 1, m3 + m6)
                after(m3)
            for h in (4 * g, 4 * g + 2):
                m7 = product(6, _word_sum(block(h, 1), block(h + 1, 1), 1))
                add(h, 0, m7)
            after(m7)
            if g in done:
                done[g]()

    def first_segment(t):
        return jnp.concatenate([ring(t)[pl.ds(HEAD, M), :], ring(t)[pl.ds(0, SEG), :]], axis=0)

    p_first = []

    def first_scores():
        p_first.extend(probs(first_segment(h), first_segment(H + h)) for h in range(8))

    def first_values():
        for h in range(4):
            obuf[h] = _dot(p_first[h], first_segment(2 * H + h))
            pbuf[h] = p_first[4 + h]

    _start(mem_copies)
    start_next()
    _wait(mem_copies)
    start_next()
    for job in relayout_jobs([0]):
        job()
    for i, n in enumerate(_STAGES):
      u = stage_start[i]
      j, kt = u // (2 * KT), u // 2 % KT
      jobs = relayout_jobs(range(u + n, stage_start[min(i + 2, len(_STAGES))]))
      if i == 0:
          project(j, kt, range(HH), [])
          for job in jobs:
              job()
          continue
      if jobs:
          need_unit(u + n)
      if i in _EXTRA:
          start_next()
      if n <= 2:
          heads = range(H) if n == 2 else range(u % 2 * HH, (u % 2 + 1) * HH)
          project(j, kt, heads, jobs + (xsum_jobs([2]) if _STAGES[i + 1] > 2 else []))
      elif n == 4:
          project_strassen(j, [kt // 2], jobs + xsum_jobs([3] if kt == 4 else [0, 1]))
      elif jobs:
          project_strassen(j, [kt // 2, kt // 2 + 1], jobs)
      else:
          _wait(vec_copies + xtail_copies)
          start_next()
          side = {q: functools.partial(score_job, q // 2, q % 2) for q in range(2 * n_blk)}
          side[2 * n_blk] = select_tokens
          project_strassen(j, [kt // 2, kt // 2 + 1], jobs, side,
                           {0: first_scores, 2: first_values})
    assert progress["started"] == len(queue)
    for t in range(3 * H):
        mqkv[t] = ring(t)[pl.ds(HEAD, M), :]
    gwf[...] = gw[...].astype(_F32)
    ybuf[...] = jnp.zeros(ybuf.shape, _F32)
    xbuf_u[:, pl.ds(S // 2, SEG // 2), :] = jnp.zeros((KT, SEG // 2, _LANE), _U32)

    def ffn_jobs(i):
        part, act = {}, []
        tiles = [i * _FFN_TILES + k for k in range(_FFN_TILES)]
        held = [jnp.minimum(t, FT - 1) for t in tiles]

        def up_job(w, k, half):
            r = _dot(xsel[:, pl.ds(half * (D // 2), D // 2)],
                     _bf16((wg_u, wu_u)[w][held[k], pl.ds(half * (D // 4), D // 4), :]))
            part[w, k] = r if half == 0 else r + part[w, k]

        def down_job(q):
            if q == 0:
                act.extend(jnp.where(t < FT, part[0, k] * _sigmoid(part[0, k]) * part[1, k],
                                     0.0) for k, t in enumerate(tiles))
            for n, k in (divmod(e, _FFN_TILES) for e in range(4 * q, 4 * q + 4)):
                r = _dot(act[k], _bf16(wd_u[n, pl.ds(_aligned(held[k] * _WORDS, _WORDS),
                                                     _WORDS), :]))
                part["y"] = r if k == 0 else r + part["y"]
                if k == _FFN_TILES - 1:
                    ybuf[:, pl.ds(n * _LANE, _LANE)] += part["y"] * rgate[...]

        order = [functools.partial(up_job, w, k, half)
                 for k in range(_FFN_TILES) for w in range(2) for half in range(2)]
        jobs = {2 * q: job for q, job in enumerate(order)}
        jobs.update({44 + 2 * q: functools.partial(down_job, q)
                     for q in range(KT * _FFN_TILES // 4)})
        return jobs

    seg_row = lax.broadcasted_iota(_I32, (SEG, _LANE), 0)

    def mix(seg, a, copies=None):
        rows = pl.ds(_aligned(seg * (SEG // 2), SEG // 2), SEG // 2)
        xs = [_bf16(xbuf_u[kt, rows, :]).astype(_F32) for kt in range(KT)]
        z = xs[0] * gwf[pl.ds(0, 1), :]
        for kt in range(1, KT):
            z = z + xs[kt] * gwf[pl.ds(kt, 1), :]
        g = _sigmoid(jnp.sum(z, axis=-1, keepdims=True))
        hits = [seg_row == picks[c] - seg * SEG for c in range(_TOPK)]
        packed = []
        for kt in range(KT):
            upd = jnp.zeros((SEG, _LANE), _F32)
            for c in range(_TOPK):
                upd = jnp.where(hits[c], ybuf[pl.ds(c, 1), pl.ds(kt * _LANE, _LANE)], upd)
            packed.append((g * a[kt] + (1.0 - g) * (xs[kt] + upd)).astype(_BF16))
            xbuf_u[kt, rows, :] = pltpu.bitcast(packed[-1], _U32)
            if copies:
                copies[kt].start()
        return packed

    def attend_and_project(seg, jobs=(), r0=0):
        rows = pl.ds(_aligned(_rem(seg * SEG, FAT), SEG), SEG)
        o = {h: obuf[h, pl.ds(r0, L - r0), :] for h in range(4)}
        p = {4 + h: pbuf[h, pl.ds(r0, L - r0), :] for h in range(4)}

        def tok(t):
            return jnp.concatenate([mqkv[t], ring(t)[rows, :]], axis=0)

        acc = [None] * KT
        for g in range(G):
            lhs = jnp.concatenate([o[4 * g + i] for i in range(4)], axis=1)
            for n in range(KT):
                if n == _QKN and g + 2 < G:
                    for h in range(4 * g + 8, 4 * g + 12):
                        p[h] = probs(tok(h)[r0:], tok(H + h))
                if n == _PVN and g + 1 < G:
                    for h in range(4 * g + 4, 4 * g + 8):
                        o[h] = _dot(p[h], tok(2 * H + h))
                r = _dot(lhs, _bf16(wo_u[n, pl.ds(g * 4 * _WORDS, 4 * _WORDS), :]))
                acc[n] = r if g == 0 else r + acc[n]
                if g * KT + n in jobs:
                    jobs[g * KT + n]()
        return acc

    def step(s, jobs=(), write=False, backlog=None):
        acc = attend_and_project(s - 1, jobs)
        x0 = HEAD + (s - 1) * XR
        wpos = [_aligned(_rem(x0 + 8 * i, FAT), 8) for i in range(XR // 8)]
        rows = pl.ds(_aligned(_rem(s * SEG, FAT), SEG), SEG)
        h_in = []
        for kt in range(KT):
            xw = xbuf_u[kt, pl.ds(_aligned((HEAD - M) // 2 + (s - 1) * (XR // 2), 4),
                                  SEG // 2), :]
            mw = pltpu.bitcast(jnp.concatenate([acc[kt][:M]] * 2, axis=0).astype(_BF16), _U32)
            h_in.append(_bf16(jnp.concatenate(
                [jnp.where(sublane < M // 2, mw, xw[:8]), xw[8:]], axis=0)))

        tied = {}
        if write:
            tied.update({(g, 3): v for g, v in enumerate(mix(s - 1, [a[M:] for a in acc]))})
        else:
            for n in range(KT):
                abuf[s - 1, n] = acc[n][M:]
        if backlog is not None:
            old = [abuf[jnp.minimum(backlog, NB - 1), n] for n in range(KT)]
            tied.update({(g, 2): v for g, v in enumerate(
                mix(jnp.where(backlog < NB, backlog, n_seg), old))})

        mem_rows, p = {}, {}

        def weights(t, lo, hi):
            return _bf16(wqkv[t, pl.ds(lo * _WORDS, (hi - lo) * _WORDS), :])

        def finish(t, r):
            for i, w in enumerate(wpos):
                ring(t)[pl.ds(w, 8), :] = r[M + 8 * i:M + 8 * i + 8]
            mqkv[t] = mem_rows[t] = r[:M]

        def tok(t):
            return jnp.concatenate([mem_rows[t], ring(t)[rows, :]], axis=0)

        first = [j * H + h for h in range(2) for j in range(3)][:_NFIRST]
        lo = jnp.concatenate(h_in[:KT // 2], axis=1)
        hi = jnp.concatenate(h_in[KT // 2:], axis=1)
        part = [_dot(lo, weights(t, 0, KT // 2)) for t in first]
        for t, r in zip(first, part):
            finish(t, _dot(hi, weights(t, KT // 2, KT)) + r)
        for g in range(G):
            for i in range(4):
                for j in range(3):
                    t = j * H + 4 * g + i
                    if t not in first:
                        h0 = h_in[0]
                        if j == 0 and (g, i) in tied:
                            h0 = jnp.where(never, tied[g, i], h0)
                        finish(t, _dot(jnp.concatenate([h0] + h_in[1:], axis=1),
                                       weights(t, 0, KT)))
                if g == _QKG and i == 0:
                    for h in range(4):
                        p[h] = probs(tok(h), tok(H + h))
                    for h in range(4):
                        pbuf[h] = probs(tok(4 + h), tok(H + 4 + h))
                if g == _PVG and i == 0:
                    for h in range(4):
                        obuf[h] = _dot(p[h], tok(2 * H + h))
        if write:
            _start(out_copies(s - 1))
        if backlog is not None:
            pl.when(backlog < NB)(lambda: _start(out_copies(backlog)))

    def ffn_step(i, carry):
        for k in range(NB):
            @pl.when(i == k)
            def _():
                _wait(ffn_copies(k))
                if k + 2 < NB:
                    _start(ffn_copies(k + 2))
        step(1 + i, jobs=ffn_jobs(i))
        return carry

    def main_steps(i, carry):
        for k in range(_UNROLL):
            step(NB + 1 + i * _UNROLL + k, write=True, backlog=i if k == 0 else None)
        return carry

    n_main = (n_seg - NB - 1) // _UNROLL
    assert n_main >= NB
    _wait(wo_copies)
    lax.fori_loop(0, NB, ffn_step, 0)
    lax.fori_loop(0, n_main, main_steps, 0)
    for s in range(NB + 1 + n_main * _UNROLL, n_seg):
        step(s, write=True)
    mix(n_seg - 1, attend_and_project(n_seg - 1, r0=M), out_copies(n_seg - 1))
    _wait(out_copies(0, n_seg))


@functools.partial(jax.jit, static_argnames=("A_seg_len",))
def pallas_gated_mix__memory_aug_recurrent_mem_tr__moe_arch_mod__prompt_kernel(
    A_x, A_mem0, A_Wq, A_Wk, A_Wv, A_Wo, A_seg_len, B_x, B_w_r, B_w_gate, B_w_up,
    B_w_down, gate_w,
):
    del B_x
    B, S, D = A_x.shape
    _, H, DH = A_Wq.shape
    M = A_mem0.shape[1]
    SEG = int(A_seg_len)
    F = B_w_gate.shape[1]
    assert (B, S, D, H, DH, M, SEG) == (1, 2048, 1024, 32, _LANE, 8, 32) and F % _LANE == 0
    L = M + SEG
    KT, FT = D // _LANE, F // _LANE
    fat = S - (S // SEG - 1) * (SEG - M) + M
    n_ffn = -(-FT // _FFN_TILES)

    any_spec = pl.BlockSpec(memory_space=pl.ANY)
    dma = pltpu.SemaphoreType.DMA
    out = pl.pallas_call(
        functools.partial(_kernel, S=S, D=D, H=H, DH=DH, M=M, SEG=SEG, F=F),
        out_shape=jax.ShapeDtypeStruct((S, D), A_x.dtype),
        in_specs=[any_spec] * 11,
        out_specs=any_spec,
        scratch_shapes=[
            pltpu.VMEM((KT, S + SEG, _LANE), _BF16),
            pltpu.VMEM((6 * KT, _LANE, H // 2, DH), _BF16),
            pltpu.VMEM((3 * H, D // 2, DH), _U32),
            pltpu.VMEM((KT, H * DH, _LANE), _BF16),
            pltpu.VMEM((FT, D, _LANE), _BF16),
            pltpu.VMEM((FT, D, _LANE), _BF16),
            pltpu.VMEM((KT, F, _LANE), _BF16),
            [pltpu.VMEM((12, fat, DH), _F32)] * (H // 4),
            pltpu.VMEM((KT // 2, 7, fat // 4, _LANE), _U32),
            pltpu.VMEM((n_ffn, KT, SEG, _LANE), _F32),
            pltpu.VMEM((4, L, DH), _F32),
            pltpu.VMEM((4, L, L), _F32),
            pltpu.VMEM((3 * H, M, DH), _F32),
            pltpu.VMEM((_TOPK, D), _F32),
            pltpu.VMEM((_TOPK, D), _F32),
            pltpu.VMEM((KT, M, _LANE), _BF16),
            pltpu.VMEM((KT, _LANE), _BF16),
            pltpu.VMEM((KT, _LANE), _BF16),
            pltpu.VMEM((KT, _LANE), _F32),
            pltpu.VMEM((_TOPK, _LANE), _F32),
            pltpu.SMEM((_TOPK,), _I32),
            dma((len(_BATCHES),)), dma((KT,)), dma(()), dma((2,)), dma(()), dma((n_ffn,)),
            dma(()),
        ],
        compiler_params=pltpu.CompilerParams(vmem_limit_bytes=120 * 1024 * 1024,
                                             disable_bounds_checks=True),
        name="gated_mix_rmt_mod",
    )(
        A_x.reshape(S, D), A_mem0.reshape(M, D), A_Wq.reshape(D, 2, H // 2, DH),
        A_Wk.reshape(D, 2, H // 2, DH), A_Wv.reshape(D, 2, H // 2, DH),
        A_Wo.reshape(H * DH, D), B_w_r.reshape(KT, _LANE), B_w_gate, B_w_up, B_w_down,
        gate_w.reshape(KT, _LANE),
    )
    return out.reshape(B, S, D)
```

```python
import functools

import jax
import jax.numpy as jnp
import numpy as np
from jax import lax
import jax.experimental.pallas as pl
import jax.experimental.pallas.tpu as pltpu

_F32 = jnp.float32
_BF16 = jnp.bfloat16
_U32 = jnp.uint32
_I32 = jnp.int32
_NN = (((1,), (0,)), ((), ()))
_NT = (((1,), (1,)), ((), ()))

_LANE = 128
_WORDS = _LANE // 2
_TOPK = 8
_UNROLL = 3
_FFN_TILES = 5
_STAGES = (1, 1, 1, 1, 2, 2, 4, 4, 8, 8, 8, 8)
_BATCHES = (1, 1, 1, 1, 2, 2, 4, 4, 4, 4, 4, 4, 8, 8)
_EXTRA = (7,)
_QKN = 1
_VB = True
_FPOS = [2 * q + 1 for q in range(20)] + [43, 45, 47, 49, 51, 53, 55, 58, 61, 63]
_ONLY_MAIN = False
_MIX0 = 7
_MIXS = 6
_DELAY = 7
_TIEIN = True
_PVN = 5
_QKG = 6
_PVG = 7
_NFIRST = 6


def _dot(a, b, dims=_NN):
    return lax.dot_general(a, b, dims, preferred_element_type=_F32)


def _aligned(i, n):
    return i if isinstance(i, int) else pl.multiple_of(i, n)


def _rem(i, n):
    return i % n if isinstance(i, int) else lax.rem(i, n)


def _sigmoid(v):
    return 1.0 / (1.0 + jnp.exp(-v))


def _bf16(words):
    return pltpu.bitcast(words, _BF16)


def _word_sum(a, b, sign):
    halves = []
    for k in range(2):
        u, v = (pltpu.unpack_elementwise(w, index=k, packed_dtype=_BF16, unpacked_dtype=_F32)
                for w in (a, b))
        halves.append(u + v if sign > 0 else u - v)
    return pltpu.bitcast(pltpu.pack_elementwise(halves, packed_dtype=_BF16), _U32)


def _v(v):
    return v.astype(_BF16) if _VB else v


def _start(copies):
    for cp in copies:
        cp.start()


def _wait(copies):
    for cp in copies:
        cp.wait()


def _kernel(x_hbm, mem_hbm, wq_hbm, wk_hbm, wv_hbm, wo_hbm, wr_hbm, wg_hbm, wu_hbm,
            wd_hbm, gw_hbm, out_hbm,
            xbuf, stage, wqkv, wo, wg, wu, wd, rings, xsum, abuf, obuf, pbuf, mqkv, xsel,
            ybuf, membuf, wr, gw, gwf, rgate, picks,
            sem_w, sem_xh, sem_xt, sem_small, sem_wo, sem_b, sem_out,
            *, S, D, H, DH, M, SEG, F):
    L = M + SEG
    n_seg = S // SEG
    KT = D // _LANE
    FT = F // _LANE
    G = H // 4
    HH = H // 2
    XR = SEG - M
    HEAD = S - (n_seg - 1) * XR
    FAT = HEAD + M
    NB = abuf.shape[0]
    w_hbm = (wq_hbm, wk_hbm, wv_hbm)

    stage_u, xbuf_u, membuf_u, wo_u, wd_u = (
        r.bitcast(_U32) for r in (stage, xbuf, membuf, wo, wd))

    def ring(t):
        j, h = divmod(t, H)
        return rings[h // 4].at[j * 4 + h % 4]

    picks[0] = 0
    never = picks[0] > 0
    sublane = lax.broadcasted_iota(_I32, (8, _LANE), 0)

    batch_start = np.cumsum((0,) + _BATCHES).tolist()
    stage_start = np.cumsum((0,) + _STAGES).tolist()

    def batch_copies(i):
        copies = []
        for u in range(batch_start[i], batch_start[i + 1]):
            j, kt, half = u // (2 * KT), u // 2 % KT, u % 2
            if j == 0 and half == 0:
                copies.append(pltpu.make_async_copy(
                    x_hbm.at[pl.ds(0, FAT), pl.ds(kt * _LANE, _LANE)],
                    xbuf.at[kt, pl.ds(0, FAT), :], sem_xh.at[kt]))
            copies.append(pltpu.make_async_copy(
                w_hbm[j].at[pl.ds(kt * _LANE, _LANE), half], stage.at[u], sem_w.at[i]))
        return copies

    def strip_copies(src, dst, tiles, sem):
        return [pltpu.make_async_copy(src.at[:, pl.ds(n * _LANE, _LANE)], dst.at[n], sem)
                for n in tiles]

    def ffn_copies(i, slot=None):
        slot = i if slot is None else slot
        units = pl.ds(min(i * _FFN_TILES, FT - _FFN_TILES) * _LANE, _FFN_TILES * _LANE)
        return [pltpu.make_async_copy(wg_hbm.at[:, units], wg.at[slot], sem_b.at[slot]),
                pltpu.make_async_copy(wu_hbm.at[:, units], wu.at[slot], sem_b.at[slot])
                ] + strip_copies(wd_hbm.at[units, :], wd.at[slot], range(KT), sem_b.at[slot])

    def out_copies(seg, n=1):
        rows = pl.ds(_aligned(seg * SEG, SEG), n * SEG)
        return [pltpu.make_async_copy(xbuf.at[kt, rows, :],
                                      out_hbm.at[rows, pl.ds(kt * _LANE, _LANE)], sem_out)
                for kt in range(KT)]

    mem_copies = strip_copies(mem_hbm, membuf, range(KT), sem_small.at[0])
    vec_copies = [pltpu.make_async_copy(wr_hbm, wr, sem_small.at[1]),
                  pltpu.make_async_copy(gw_hbm, gw, sem_small.at[1])]
    xtail_copies = [pltpu.make_async_copy(
        x_hbm.at[pl.ds(FAT, S - FAT), pl.ds(kt * _LANE, _LANE)],
        xbuf.at[kt, pl.ds(FAT, S - FAT), :], sem_xt) for kt in range(KT)]
    wo_copies = strip_copies(wo_hbm, wo, range(KT), sem_wo)

    queue = [batch_copies(i) for i in range(len(_BATCHES))]
    queue += [vec_copies + xtail_copies, wo_copies, ffn_copies(0), ffn_copies(1) + ffn_copies(2)]
    progress = {"started": 0, "arrived": 0}

    def start_next():
        if progress["started"] < len(queue):
            _start(queue[progress["started"]])
            progress["started"] += 1

    def need_unit(u):
        while batch_start[progress["arrived"]] <= u:
            _wait(queue[progress["arrived"]])
            progress["arrived"] += 1
            start_next()

    row = lax.broadcasted_iota(_I32, (L, L), 0)
    col = lax.broadcasted_iota(_I32, (L, L), 1)
    mask = (row < M) | (row >= col)
    scale = DH ** (-0.5)

    def probs(q, k):
        sc = jnp.where(mask[L - q.shape[0]:], _dot(q, k, _NT), -1000000000.0 / scale)
        e = jnp.exp2((sc - jnp.max(sc, axis=-1, keepdims=True)) * float(scale * np.log2(np.e)))
        total = jnp.sum(e, axis=-1, keepdims=True)
        inv = pltpu.reciprocal(total, approx=True)
        return e * (inv * (2.0 - total * inv))

    n_blk = S // _LANE
    score = [None] * n_blk

    def score_job(b, half):
        kts = range(half * KT // 2, (half + 1) * KT // 2)
        wrf = wr[...].astype(_F32)
        w = jnp.concatenate([jnp.broadcast_to(wrf[kt:kt + 1], (8, _LANE)) for kt in kts],
                            axis=1)
        xb = jnp.concatenate([_bf16(xbuf_u[kt, pl.ds(b * _WORDS, _WORDS), :]) for kt in kts],
                             axis=1)
        r = _dot(w, xb, _NT)
        score[b] = r if half == 0 else r + score[b]

    def select_tokens():
        r_all = []
        for b0 in range(0, n_blk, 8):
            r = score[b0]
            for b in range(1, 8):
                r = jnp.where(sublane == b, score[b0 + b], r)
            r_all.append(r)
        r_all = jnp.concatenate(r_all, axis=0).astype(_BF16).astype(_F32)
        r_all = jnp.where(r_all == 0.0, 0.0, r_all)
        bits = pltpu.bitcast(r_all, _I32)
        key = jnp.where(bits < 0, bits ^ np.int32(0x7FFFFFFF), bits) >> 16
        key = jnp.where(r_all != r_all, np.int32(-(1 << 15)), key).astype(_F32)
        pos = (lax.broadcasted_iota(_I32, (n_blk, _LANE), 0) * _LANE
               + lax.broadcasted_iota(_I32, (n_blk, _LANE), 1)).astype(_F32)
        x_sel = [jnp.zeros((_TOPK, _LANE), _F32) for _ in range(KT)]
        r_sel = jnp.zeros((_TOPK, _LANE), _F32)
        for c in range(_TOPK):
            best = jnp.max(key, keepdims=True)
            pick = jnp.min(jnp.where(key == best, pos, float(S)), keepdims=True)
            hit = pos == pick
            key = jnp.where(hit, -float(1 << 17), key)
            r_sel = jnp.where(sublane == c,
                              jnp.sum(jnp.where(hit, r_all, 0.0), keepdims=True), r_sel)
            token = pick[0, 0].astype(_I32)
            picks[c] = token
            base = pl.multiple_of((token >> 3) << 3, 8)
            for kt in range(KT):
                grp = xbuf[kt, pl.ds(base, 8), :].astype(_F32)
                one = jnp.sum(jnp.where(sublane == (token & 7), grp, 0.0), axis=0,
                              keepdims=True)
                x_sel[kt] = jnp.where(sublane == c, one, x_sel[kt])
        xsel[...] = jnp.concatenate(x_sel, axis=1)
        rgate[...] = _sigmoid(r_sel)

    def transpose8(v):
        c = [v[0]] + [pltpu.roll(v[8 - m], 8 - m, 0) for m in range(1, 8)]
        for d in (1, 2, 4):
            c = [jnp.where((sublane & d) != 0, c[m - d], c[m]) for m in range(8)]
        return [c[0]] + [pltpu.roll(c[k], 8 - k, 0) for k in range(1, 8)]

    def relayout(u, db, odd, after=None):
        need_unit(u)
        j, kt, half = u // (2 * KT), u // 2 % KT, u % 2
        words = []
        for t in range(8):
            a = stage_u[u, db * 16 + 2 * t]
            b = stage_u[u, db * 16 + 2 * t + 1]
            if odd:
                words.append((a >> 16) | (b & np.uint32(0xFFFF0000)))
            else:
                words.append((a & np.uint32(0xFFFF)) | (b << 16))
        if after is not None:
            words[0] = jnp.where(never, after, words[0])
        for t, w in enumerate(transpose8(words)):
            wqkv[j * H + half * HH + 2 * t + odd, pl.ds(kt * _WORDS + db * 8, 8), :] = w

    def relayout_jobs(units):
        return [functools.partial(relayout, u, db, odd)
                for u in units for db in range(_LANE // 16) for odd in range(2)]

    def head_rows(kt, r0, n):
        n_x = min(n, HEAD // 2 - r0)
        rows = xbuf_u[kt, pl.ds(r0, n_x), :]
        return rows if n_x == n else jnp.concatenate([rows, membuf_u[kt]], axis=0)

    HW = FAT // 4

    def xsum_job(pair, r0, after):
        a11, a12, a21, a22 = (head_rows(2 * pair + k, half * HW + r0, 8)
                              for half in range(2) for k in range(2))
        a11, a22 = jnp.where(never, after, a11), jnp.where(never, after, a22)
        for k, w in enumerate((_word_sum(a11, a22, 1), _word_sum(a21, a22, 1), a11, a22,
                               _word_sum(a11, a12, 1), _word_sum(a21, a11, -1),
                               _word_sum(a12, a22, -1))):
            xsum[pair, k, pl.ds(r0, 8), :] = w

    def xsum_jobs(pairs):
        return [functools.partial(xsum_job, pair, r0)
                for pair in pairs for r0 in range(0, HW, 8)]

    def run_jobs(jobs, i, n, result):
        mine = jobs[i * len(jobs) // n:(i + 1) * len(jobs) // n]
        for k, job in enumerate(mine):
            r0 = k * (result.shape[0] // 8) // len(mine) * 8
            job(pltpu.bitcast(result[r0:r0 + 8], _U32))

    def project(j, kt, heads, jobs):
        lhs = _bf16(head_rows(kt, 0, FAT // 2))
        for i, h in enumerate(heads):
            r = _dot(lhs, _bf16(wqkv[j * H + h, pl.ds(kt * _WORDS, _WORDS), :]))
            dst = ring(j * H + h)
            dst[...] = r + dst[...] if kt > 0 else r
            if i % 4 == 3:
                run_jobs(jobs, i // 4, len(heads) // 4, r)

    def project_strassen(j, pairs, jobs, side=(), done=()):
        def product(k, b):
            return _dot(jnp.concatenate([_bf16(xsum[p, k]) for p in pairs], axis=1), _bf16(b))

        def block(h, k):
            return jnp.concatenate(
                [wqkv[j * H + h, pl.ds((2 * p + k) * _WORDS, _WORDS), :] for p in pairs],
                axis=0)

        def add(h, half, v, first=False, sign=1):
            rows = pl.ds(half * (FAT // 2), FAT // 2)
            dst = ring(j * H + h)
            if first and pairs[0] == 0:
                dst[rows, :] = v if sign > 0 else -v
            else:
                dst[rows, :] = dst[rows, :] + v if sign > 0 else dst[rows, :] - v

        slot = [0]

        def after(m):
            run_jobs(jobs, slot[0], 7 * G, m)
            if slot[0] in side:
                side[slot[0]]()
            slot[0] += 1

        for g in range(G):
            for h in (4 * g, 4 * g + 2):
                m2 = product(1, block(h, 0))
                m5 = product(4, block(h + 1, 1))
                if len(pairs) > 1:
                    add(h, 1, m2, True), add(h + 1, 1, m2, True, -1)
                    add(h, 0, m5, True, -1), add(h + 1, 0, m5, True)
                after(m2)
                m1 = product(0, _word_sum(block(h, 0), block(h + 1, 1), 1))
                m4 = product(3, _word_sum(block(h, 1), block(h, 0), -1))
                if len(pairs) > 1:
                    add(h, 0, m1 + m4), add(h + 1, 1, m1), add(h, 1, m4)
                else:
                    add(h, 0, m1 + m4 - m5, True), add(h + 1, 1, m1 - m2, True)
                    add(h, 1, m2 + m4, True), add(h + 1, 0, m5, True)
                after(m1)
                m3 = product(2, _word_sum(block(h + 1, 0), block(h + 1, 1), -1))
                m6 = product(5, _word_sum(block(h, 0), block(h + 1, 0), 1))
                add(h + 1, 0, m3), add(h + 1, 1, m3 + m6)
                after(m3)
            for h in (4 * g, 4 * g + 2):
                m7 = product(6, _word_sum(block(h, 1), block(h + 1, 1), 1))
                add(h, 0, m7)
            after(m7)
            if g in done:
                done[g]()

    def first_segment(t):
        return jnp.concatenate([ring(t)[pl.ds(HEAD, M), :], ring(t)[pl.ds(0, SEG), :]], axis=0)

    p_first = []

    def first_scores():
        p_first.extend(probs(first_segment(h), first_segment(H + h)) for h in range(8))

    def first_values():
        for h in range(4):
            obuf[h] = _dot(p_first[h], first_segment(2 * H + h))
            pbuf[h] = p_first[4 + h]

    _start(mem_copies)
    start_next()
    _wait(mem_copies)
    start_next()
    for job in relayout_jobs([0]):
        job()
    for i, n in enumerate(_STAGES if not _ONLY_MAIN else ()):
      u = stage_start[i]
      j, kt = u // (2 * KT), u // 2 % KT
      jobs = relayout_jobs(range(u + n, stage_start[min(i + 2, len(_STAGES))]))
      if i == 0:
          project(j, kt, range(HH), [])
          for job in jobs:
              job()
          continue
      if jobs:
          need_unit(u + n)
      if i in _EXTRA:
          start_next()
      if n <= 2:
          heads = range(H) if n == 2 else range(u % 2 * HH, (u % 2 + 1) * HH)
          project(j, kt, heads, jobs + (xsum_jobs([2]) if _STAGES[i + 1] > 2 else []))
      elif n == 4:
          project_strassen(j, [kt // 2], jobs + xsum_jobs([3] if kt == 4 else [0, 1]))
      elif jobs:
          project_strassen(j, [kt // 2, kt // 2 + 1], jobs)
      else:
          _wait(vec_copies + xtail_copies)
          start_next()
          side = {q: functools.partial(score_job, q // 2, q % 2) for q in range(2 * n_blk)}
          side[2 * n_blk] = select_tokens
          project_strassen(j, [kt // 2, kt // 2 + 1], jobs, side,
                           {0: first_scores, 2: first_values})
    assert _ONLY_MAIN or progress["started"] == len(queue)
    for t in range(3 * H):
        mqkv[t] = ring(t)[pl.ds(HEAD, M), :]
    gwf[...] = gw[...].astype(_F32)
    ybuf[...] = jnp.zeros(ybuf.shape, _F32)
    xbuf_u[:, pl.ds(S // 2, SEG // 2), :] = jnp.zeros((KT, SEG // 2, _LANE), _U32)

    def ffn_jobs(i):
        part, act = {}, []
        repeated = i * _FFN_TILES - jnp.minimum(i * _FFN_TILES, FT - _FFN_TILES)

        def up_job(w, k, half):
            span = pl.ds(half * (D // 2), D // 2)
            r = _dot(xsel[:, span], (wg, wu)[w][i, span, pl.ds(k * _LANE, _LANE)])
            part[w, k] = r if half == 0 else r + part[w, k]

        def down_job(q):
            if q == 0:
                act.extend(jnp.where(k >= repeated,
                                     part[0, k] * _sigmoid(part[0, k]) * part[1, k], 0.0)
                           for k in range(_FFN_TILES))
            for n, k in (divmod(e, _FFN_TILES) for e in range(4 * q, 4 * q + 4)):
                r = _dot(act[k], _bf16(wd_u[i, n, pl.ds(k * _WORDS, _WORDS), :]))
                part["y"] = r if k == 0 else r + part["y"]
                if k == _FFN_TILES - 1:
                    ybuf[:, pl.ds(n * _LANE, _LANE)] += part["y"] * rgate[...]

        order = [functools.partial(up_job, w, k, half)
                 for k in range(_FFN_TILES) for w in range(2) for half in range(2)]
        order += [functools.partial(down_job, q) for q in range(KT * _FFN_TILES // 4)]
        jobs = dict(zip(_FPOS, order))
        assert len(jobs) == len(order)
        return jobs

    seg_row = lax.broadcasted_iota(_I32, (SEG, _LANE), 0)

    def mix_jobs(seg, a, copies=None):
        rows = pl.ds(_aligned(seg * (SEG // 2), SEG // 2), SEG // 2)
        gate = []

        def zeros(after):
            z = jnp.zeros((SEG, _LANE), _F32)
            return z if after is None else jnp.where(never, after, z)

        def gate_job(after=None):
            z = zeros(after)
            for kt in range(KT):
                z = z + _bf16(xbuf_u[kt, rows, :]).astype(_F32) * gwf[pl.ds(kt, 1), :]
            gate.append(_sigmoid(jnp.sum(z, axis=-1, keepdims=True)))
            return jnp.broadcast_to(gate[0], (SEG, _LANE)).astype(_BF16)

        def strip_job(kt, after=None):
            upd = zeros(after)
            for c in range(_TOPK):
                upd = jnp.where(seg_row == picks[c] - seg * SEG,
                                ybuf[pl.ds(c, 1), pl.ds(kt * _LANE, _LANE)], upd)
            b = _bf16(xbuf_u[kt, rows, :]).astype(_F32) + upd
            res = (gate[0] * a[kt] + (1.0 - gate[0]) * b).astype(_BF16)
            xbuf_u[kt, rows, :] = pltpu.bitcast(res, _U32)
            if copies:
                copies[kt].start()
            return res

        return [gate_job] + [functools.partial(strip_job, kt) for kt in range(KT)]

    def attend_and_project(seg, jobs=(), r0=0):
        rows = pl.ds(_aligned(_rem(seg * SEG, FAT), SEG), SEG)
        o = {h: obuf[h, pl.ds(r0, L - r0), :] for h in range(4)}
        p = {4 + h: pbuf[h, pl.ds(r0, L - r0), :] for h in range(4)}

        def tok(t):
            return jnp.concatenate([mqkv[t], ring(t)[rows, :]], axis=0)

        acc = [None] * KT
        for g in range(G):
            lhs = jnp.concatenate([o[4 * g + i] for i in range(4)], axis=1)
            for n in range(KT):
                if n == _QKN and g + 2 < G:
                    for h in range(4 * g + 8, 4 * g + 12):
                        p[h] = probs(tok(h)[r0:], tok(H + h))
                if n == _PVN and g + 1 < G:
                    for h in range(4 * g + 4, 4 * g + 8):
                        o[h] = _dot(p[h], _v(tok(2 * H + h)))
                r = _dot(lhs, _bf16(wo_u[n, pl.ds(g * 4 * _WORDS, 4 * _WORDS), :]))
                acc[n] = r if g == 0 else r + acc[n]
                if g * KT + n in jobs:
                    jobs[g * KT + n]()
        return acc

    def step(s, jobs=(), write=False, backlog=None):
        acc = attend_and_project(s - 1, jobs)
        x0 = HEAD + (s - 1) * XR
        wpos = [_aligned(_rem(x0 + 8 * i, FAT), 8) for i in range(XR // 8)]
        rows = pl.ds(_aligned(_rem(s * SEG, FAT), SEG), SEG)
        h_in = []
        for kt in range(KT):
            xw = xbuf_u[kt, pl.ds(_aligned((HEAD - M) // 2 + (s - 1) * (XR // 2), 4),
                                  SEG // 2), :]
            mw = pltpu.bitcast(jnp.concatenate([acc[kt][:M]] * 2, axis=0).astype(_BF16), _U32)
            h_in.append(_bf16(jnp.concatenate(
                [jnp.where(sublane < M // 2, mw, xw[:8]), xw[8:]], axis=0)))

        side = {}
        if write:
            jobs = mix_jobs(s - 1, [a[M:] for a in acc])
            side.update({_MIX0 + _MIXS * k: job for k, job in enumerate(jobs)})
        else:
            for n in range(KT):
                abuf[s - 1, n] = acc[n][M:]
        if backlog is not None:
            jobs = mix_jobs(jnp.where(backlog < NB, backlog, n_seg),
                            [abuf[jnp.minimum(backlog, NB - 1), n] for n in range(KT)])
            side.update({_MIX0 + _MIXS // 2 + _MIXS * k: job for k, job in enumerate(jobs)})

        mem_rows, p, pending = {}, {}, []

        def weights(t, lo, hi):
            return _bf16(wqkv[t, pl.ds(lo * _WORDS, (hi - lo) * _WORDS), :])

        def finish(t, r):
            for i, w in enumerate(wpos):
                ring(t)[pl.ds(w, 8), :] = r[M + 8 * i:M + 8 * i + 8]
            mqkv[t] = mem_rows[t] = r[:M]

        def tok(t):
            return jnp.concatenate([mem_rows[t], ring(t)[rows, :]], axis=0)

        first = [j * H + h for h in range(2) for j in range(3)][:_NFIRST]
        lo = jnp.concatenate(h_in[:KT // 2], axis=1)
        hi = jnp.concatenate(h_in[KT // 2:], axis=1)
        part = [_dot(lo, weights(t, 0, KT // 2)) for t in first]
        for t, r in zip(first, part):
            finish(t, _dot(hi, weights(t, KT // 2, KT)) + r)
        for g in range(G):
            for i in range(4):
                for j in range(3):
                    t = j * H + 4 * g + i
                    if t not in first:
                        h0 = h_in[0]
                        if pending and pending[0][0] == 0:
                            h0 = jnp.where(never, pending.pop(0)[1], h0)
                        pending[:] = [(d - 1, v) for d, v in pending]
                        r = _dot(jnp.concatenate([h0] + h_in[1:], axis=1), weights(t, 0, KT))
                        finish(t, r)
                        if 12 * g + 3 * i + j in side:
                            pending.append((_DELAY, side[12 * g + 3 * i + j](r if _TIEIN else None)))
                if g == _QKG and i == 0:
                    for h in range(4):
                        p[h] = probs(tok(h), tok(H + h))
                    for h in range(4):
                        pbuf[h] = probs(tok(4 + h), tok(H + 4 + h))
                if g == _PVG and i == 0:
                    for h in range(4):
                        obuf[h] = _dot(p[h], _v(tok(2 * H + h)))
        if write:
            _start(out_copies(s - 1))
        if backlog is not None:
            pl.when(backlog < NB)(lambda: _start(out_copies(backlog)))

    def ffn_step(i, carry):
        _wait(ffn_copies(0, i))
        step(1 + i, jobs=ffn_jobs(i))
        return carry

    def main_steps(i, carry):
        for k in range(_UNROLL):
            step(NB + 1 + i * _UNROLL + k, write=True, backlog=i if k == 0 else None)
        return carry

    n_main = (n_seg - NB - 1) // _UNROLL
    assert n_main >= NB
    _wait(wo_copies)
    _start([cp for i in range(3, NB) for cp in ffn_copies(i)])
    if _ONLY_MAIN != 1: lax.fori_loop(0, NB, ffn_step, 0)
    if _ONLY_MAIN != 2: lax.fori_loop(0, n_main, main_steps, 0)
    for s in range(NB + 1 + n_main * _UNROLL, n_seg):
        step(s, write=True)
    for job in mix_jobs(n_seg - 1, attend_and_project(n_seg - 1, r0=M), out_copies(n_seg - 1)):
        job()
    _wait(out_copies(0, n_seg))


@functools.partial(jax.jit, static_argnames=("A_seg_len",))
def pallas_gated_mix__memory_aug_recurrent_mem_tr__moe_arch_mod__prompt_kernel(
    A_x, A_mem0, A_Wq, A_Wk, A_Wv, A_Wo, A_seg_len, B_x, B_w_r, B_w_gate, B_w_up,
    B_w_down, gate_w,
):
    del B_x
    B, S, D = A_x.shape
    _, H, DH = A_Wq.shape
    M = A_mem0.shape[1]
    SEG = int(A_seg_len)
    F = B_w_gate.shape[1]
    assert (B, S, D, H, DH, M, SEG) == (1, 2048, 1024, 32, _LANE, 8, 32) and F % _LANE == 0
    L = M + SEG
    KT, FT = D // _LANE, F // _LANE
    fat = S - (S // SEG - 1) * (SEG - M) + M
    n_ffn = -(-FT // _FFN_TILES)

    any_spec = pl.BlockSpec(memory_space=pl.ANY)
    dma = pltpu.SemaphoreType.DMA
    out = pl.pallas_call(
        functools.partial(_kernel, S=S, D=D, H=H, DH=DH, M=M, SEG=SEG, F=F),
        out_shape=jax.ShapeDtypeStruct((S, D), A_x.dtype),
        in_specs=[any_spec] * 11,
        out_specs=any_spec,
        scratch_shapes=[
            pltpu.VMEM((KT, S + SEG, _LANE), _BF16),
            pltpu.VMEM((6 * KT, _LANE, H // 2, DH), _BF16),
            pltpu.VMEM((3 * H, D // 2, DH), _U32),
            pltpu.VMEM((KT, H * DH, _LANE), _BF16),
            pltpu.VMEM((n_ffn, D, _FFN_TILES * _LANE), _BF16),
            pltpu.VMEM((n_ffn, D, _FFN_TILES * _LANE), _BF16),
            pltpu.VMEM((n_ffn, KT, _FFN_TILES * _LANE, _LANE), _BF16),
            [pltpu.VMEM((12, fat, DH), _F32)] * (H // 4),
            pltpu.VMEM((KT // 2, 7, fat // 4, _LANE), _U32),
            pltpu.VMEM((n_ffn, KT, SEG, _LANE), _F32),
            pltpu.VMEM((4, L, DH), _F32),
            pltpu.VMEM((4, L, L), _F32),
            pltpu.VMEM((3 * H, M, DH), _F32),
            pltpu.VMEM((_TOPK, D), _F32),
            pltpu.VMEM((_TOPK, D), _F32),
            pltpu.VMEM((KT, M, _LANE), _BF16),
            pltpu.VMEM((KT, _LANE), _BF16),
            pltpu.VMEM((KT, _LANE), _BF16),
            pltpu.VMEM((KT, _LANE), _F32),
            pltpu.VMEM((_TOPK, _LANE), _F32),
            pltpu.SMEM((_TOPK,), _I32),
            dma((len(_BATCHES),)), dma((KT,)), dma(()), dma((2,)), dma(()), dma((n_ffn,)),
            dma(()),
        ],
        compiler_params=pltpu.CompilerParams(vmem_limit_bytes=120 * 1024 * 1024,
                                             disable_bounds_checks=True),
        name="gated_mix_rmt_mod",
    )(
        A_x.reshape(S, D), A_mem0.reshape(M, D), A_Wq.reshape(D, 2, H // 2, DH),
        A_Wk.reshape(D, 2, H // 2, DH), A_Wv.reshape(D, 2, H // 2, DH),
        A_Wo.reshape(H * DH, D), B_w_r.reshape(KT, _LANE), B_w_gate, B_w_up, B_w_down,
        gate_w.reshape(KT, _LANE),
    )
    return out.reshape(B, S, D)
```

```python
import functools

import jax
import jax.numpy as jnp
import numpy as np
from jax import lax
import jax.experimental.pallas as pl
import jax.experimental.pallas.tpu as pltpu

_F32 = jnp.float32
_BF16 = jnp.bfloat16
_U32 = jnp.uint32
_I32 = jnp.int32
_NN = (((1,), (0,)), ((), ()))
_NT = (((1,), (1,)), ((), ()))

_LANE = 128
_WORDS = _LANE // 2
_TOPK = 8
_UNROLL = 4
_FFN_TILES = 4
_STAGES = (1, 1, 1, 1, 2, 2, 4, 4, 8, 8, 8, 8)
_BATCHES = (1, 1, 1, 1, 2, 2, 4, 4, 4, 4, 4, 4, 8, 8)
_EXTRA = (7,)
_QKN = 0
_VB = True
_FPOS = [1 + 5 * q // 2 for q in range(16)] + [45, 47, 50, 53, 55, 58, 61, 63]
_SQK = (1, 10)
_SPV = (0, 18)
_SLAST = True
_ONLY_MAIN = False
_MIX0 = 7
_MIXS = 6
_DELAY = 7
_TIEIN = True
_PVN = 3
_QKG = 6
_PVG = 7
_NFIRST = 6


def _dot(a, b, dims=_NN):
    return lax.dot_general(a, b, dims, preferred_element_type=_F32)


def _aligned(i, n):
    return i if isinstance(i, int) else pl.multiple_of(i, n)


def _rem(i, n):
    return i % n if isinstance(i, int) else lax.rem(i, n)


def _sigmoid(v):
    return 1.0 / (1.0 + jnp.exp(-v))


def _bf16(words):
    return pltpu.bitcast(words, _BF16)


def _word_sum(a, b, sign):
    halves = []
    for k in range(2):
        u, v = (pltpu.unpack_elementwise(w, index=k, packed_dtype=_BF16, unpacked_dtype=_F32)
                for w in (a, b))
        halves.append(u + v if sign > 0 else u - v)
    return pltpu.bitcast(pltpu.pack_elementwise(halves, packed_dtype=_BF16), _U32)


def _v(v):
    return v.astype(_BF16) if _VB else v


def _start(copies):
    for cp in copies:
        cp.start()


def _wait(copies):
    for cp in copies:
        cp.wait()


def _kernel(x_hbm, mem_hbm, wq_hbm, wk_hbm, wv_hbm, wo_hbm, wr_hbm, wg_hbm, wu_hbm,
            wd_hbm, gw_hbm, out_hbm,
            xbuf, stage, wqkv, wo, wg, wu, wd, rings, xsum, abuf, obuf, pbuf, mqkv, xsel,
            ybuf, membuf, wr, gw, gwf, rgate, picks,
            sem_w, sem_xh, sem_xt, sem_small, sem_wo, sem_b, sem_out,
            *, S, D, H, DH, M, SEG, F):
    L = M + SEG
    n_seg = S // SEG
    KT = D // _LANE
    FT = F // _LANE
    G = H // 4
    HH = H // 2
    XR = SEG - M
    HEAD = S - (n_seg - 1) * XR
    FAT = HEAD + M
    NB = wg.shape[0]
    w_hbm = (wq_hbm, wk_hbm, wv_hbm)

    stage_u, xbuf_u, membuf_u, wo_u, wd_u = (
        r.bitcast(_U32) for r in (stage, xbuf, membuf, wo, wd))

    def ring(t):
        j, h = divmod(t, H)
        return rings[h // 4].at[j * 4 + h % 4]

    picks[0] = 0
    never = picks[0] > 0
    sublane = lax.broadcasted_iota(_I32, (8, _LANE), 0)

    batch_start = np.cumsum((0,) + _BATCHES).tolist()
    stage_start = np.cumsum((0,) + _STAGES).tolist()

    def batch_copies(i):
        copies = []
        for u in range(batch_start[i], batch_start[i + 1]):
            j, kt, half = u // (2 * KT), u // 2 % KT, u % 2
            if j == 0 and half == 0:
                copies.append(pltpu.make_async_copy(
                    x_hbm.at[pl.ds(0, FAT), pl.ds(kt * _LANE, _LANE)],
                    xbuf.at[kt, pl.ds(0, FAT), :], sem_xh.at[kt]))
            copies.append(pltpu.make_async_copy(
                w_hbm[j].at[pl.ds(kt * _LANE, _LANE), half], stage.at[u], sem_w.at[i]))
        return copies

    def strip_copies(src, dst, tiles, sem):
        return [pltpu.make_async_copy(src.at[:, pl.ds(n * _LANE, _LANE)], dst.at[n], sem)
                for n in tiles]

    def ffn_copies(i, slot=None):
        slot = i if slot is None else slot
        units = pl.ds(i * _FFN_TILES * _LANE, _FFN_TILES * _LANE)
        return [pltpu.make_async_copy(wg_hbm.at[:, units], wg.at[slot], sem_b.at[slot]),
                pltpu.make_async_copy(wu_hbm.at[:, units], wu.at[slot], sem_b.at[slot])
                ] + strip_copies(wd_hbm.at[units, :], wd.at[slot], range(KT), sem_b.at[slot])

    def out_copies(seg, n=1):
        rows = pl.ds(_aligned(seg * SEG, SEG), n * SEG)
        return [pltpu.make_async_copy(xbuf.at[kt, rows, :],
                                      out_hbm.at[rows, pl.ds(kt * _LANE, _LANE)], sem_out)
                for kt in range(KT)]

    mem_copies = strip_copies(mem_hbm, membuf, range(KT), sem_small.at[0])
    vec_copies = [pltpu.make_async_copy(wr_hbm, wr, sem_small.at[1]),
                  pltpu.make_async_copy(gw_hbm, gw, sem_small.at[1])]
    xtail_copies = [pltpu.make_async_copy(
        x_hbm.at[pl.ds(FAT, S - FAT), pl.ds(kt * _LANE, _LANE)],
        xbuf.at[kt, pl.ds(FAT, S - FAT), :], sem_xt) for kt in range(KT)]
    wo_copies = strip_copies(wo_hbm, wo, range(KT), sem_wo)

    queue = [batch_copies(i) for i in range(len(_BATCHES))]
    queue += [vec_copies + xtail_copies, wo_copies, ffn_copies(0), ffn_copies(1) + ffn_copies(2)]
    progress = {"started": 0, "arrived": 0}

    def start_next():
        if progress["started"] < len(queue):
            _start(queue[progress["started"]])
            progress["started"] += 1

    def need_unit(u):
        while batch_start[progress["arrived"]] <= u:
            _wait(queue[progress["arrived"]])
            progress["arrived"] += 1
            start_next()

    row = lax.broadcasted_iota(_I32, (L, L), 0)
    col = lax.broadcasted_iota(_I32, (L, L), 1)
    mask = (row < M) | (row >= col)
    scale = DH ** (-0.5)

    def probs(q, k):
        sc = jnp.where(mask[L - q.shape[0]:], _dot(q, k, _NT), -1000000000.0 / scale)
        e = jnp.exp2((sc - jnp.max(sc, axis=-1, keepdims=True)) * float(scale * np.log2(np.e)))
        total = jnp.sum(e, axis=-1, keepdims=True)
        inv = pltpu.reciprocal(total, approx=True)
        return e * (inv * (2.0 - total * inv))

    n_blk = S // _LANE
    score = [None] * n_blk

    def score_job(b, half):
        kts = range(half * KT // 2, (half + 1) * KT // 2)
        wrf = wr[...].astype(_F32)
        w = jnp.concatenate([jnp.broadcast_to(wrf[kt:kt + 1], (8, _LANE)) for kt in kts],
                            axis=1)
        xb = jnp.concatenate([_bf16(xbuf_u[kt, pl.ds(b * _WORDS, _WORDS), :]) for kt in kts],
                             axis=1)
        r = _dot(w, xb, _NT)
        score[b] = r if half == 0 else r + score[b]

    def select_tokens():
        r_all = []
        for b0 in range(0, n_blk, 8):
            r = score[b0]
            for b in range(1, 8):
                r = jnp.where(sublane == b, score[b0 + b], r)
            r_all.append(r)
        r_all = jnp.concatenate(r_all, axis=0).astype(_BF16).astype(_F32)
        r_all = jnp.where(r_all == 0.0, 0.0, r_all)
        bits = pltpu.bitcast(r_all, _I32)
        key = jnp.where(bits < 0, bits ^ np.int32(0x7FFFFFFF), bits) >> 16
        key = jnp.where(r_all != r_all, np.int32(-(1 << 15)), key).astype(_F32)
        pos = (lax.broadcasted_iota(_I32, (n_blk, _LANE), 0) * _LANE
               + lax.broadcasted_iota(_I32, (n_blk, _LANE), 1)).astype(_F32)
        x_sel = [jnp.zeros((_TOPK, _LANE), _F32) for _ in range(KT)]
        r_sel = jnp.zeros((_TOPK, _LANE), _F32)
        for c in range(_TOPK):
            best = jnp.max(key, keepdims=True)
            pick = jnp.min(jnp.where(key == best, pos, float(S)), keepdims=True)
            hit = pos == pick
            key = jnp.where(hit, -float(1 << 17), key)
            r_sel = jnp.where(sublane == c,
                              jnp.sum(jnp.where(hit, r_all, 0.0), keepdims=True), r_sel)
            token = pick[0, 0].astype(_I32)
            picks[c] = token
            base = pl.multiple_of((token >> 3) << 3, 8)
            for kt in range(KT):
                grp = xbuf[kt, pl.ds(base, 8), :].astype(_F32)
                one = jnp.sum(jnp.where(sublane == (token & 7), grp, 0.0), axis=0,
                              keepdims=True)
                x_sel[kt] = jnp.where(sublane == c, one, x_sel[kt])
        xsel[...] = jnp.concatenate(x_sel, axis=1)
        rgate[...] = _sigmoid(r_sel)

    def transpose8(v):
        c = [v[0]] + [pltpu.roll(v[8 - m], 8 - m, 0) for m in range(1, 8)]
        for d in (1, 2, 4):
            c = [jnp.where((sublane & d) != 0, c[m - d], c[m]) for m in range(8)]
        return [c[0]] + [pltpu.roll(c[k], 8 - k, 0) for k in range(1, 8)]

    def relayout(u, db, odd, after=None):
        need_unit(u)
        j, kt, half = u // (2 * KT), u // 2 % KT, u % 2
        words = []
        for t in range(8):
            a = stage_u[u, db * 16 + 2 * t]
            b = stage_u[u, db * 16 + 2 * t + 1]
            if odd:
                words.append((a >> 16) | (b & np.uint32(0xFFFF0000)))
            else:
                words.append((a & np.uint32(0xFFFF)) | (b << 16))
        if after is not None:
            words[0] = jnp.where(never, after, words[0])
        for t, w in enumerate(transpose8(words)):
            wqkv[j * H + half * HH + 2 * t + odd, pl.ds(kt * _WORDS + db * 8, 8), :] = w

    def relayout_jobs(units):
        return [functools.partial(relayout, u, db, odd)
                for u in units for db in range(_LANE // 16) for odd in range(2)]

    def head_rows(kt, r0, n):
        n_x = min(n, HEAD // 2 - r0)
        rows = xbuf_u[kt, pl.ds(r0, n_x), :]
        return rows if n_x == n else jnp.concatenate([rows, membuf_u[kt]], axis=0)

    HW = FAT // 4

    def xsum_job(pair, r0, after):
        a11, a12, a21, a22 = (head_rows(2 * pair + k, half * HW + r0, 8)
                              for half in range(2) for k in range(2))
        a11, a22 = jnp.where(never, after, a11), jnp.where(never, after, a22)
        for k, w in enumerate((_word_sum(a11, a22, 1), _word_sum(a21, a22, 1), a11, a22,
                               _word_sum(a11, a12, 1), _word_sum(a21, a11, -1),
                               _word_sum(a12, a22, -1))):
            xsum[pair, k, pl.ds(r0, 8), :] = w

    def xsum_jobs(pairs):
        return [functools.partial(xsum_job, pair, r0)
                for pair in pairs for r0 in range(0, HW, 8)]

    def run_jobs(jobs, i, n, result):
        mine = jobs[i * len(jobs) // n:(i + 1) * len(jobs) // n]
        for k, job in enumerate(mine):
            r0 = k * (result.shape[0] // 8) // len(mine) * 8
            job(pltpu.bitcast(result[r0:r0 + 8], _U32))

    def project(j, kt, heads, jobs):
        lhs = _bf16(head_rows(kt, 0, FAT // 2))
        for i, h in enumerate(heads):
            r = _dot(lhs, _bf16(wqkv[j * H + h, pl.ds(kt * _WORDS, _WORDS), :]))
            dst = ring(j * H + h)
            dst[...] = r + dst[...] if kt > 0 else r
            if i % 4 == 3:
                run_jobs(jobs, i // 4, len(heads) // 4, r)

    def project_strassen(j, pairs, jobs, side=(), done=()):
        def product(k, b):
            return _dot(jnp.concatenate([_bf16(xsum[p, k]) for p in pairs], axis=1), _bf16(b))

        def block(h, k):
            return jnp.concatenate(
                [wqkv[j * H + h, pl.ds((2 * p + k) * _WORDS, _WORDS), :] for p in pairs],
                axis=0)

        def add(h, half, v, first=False, sign=1):
            rows = pl.ds(half * (FAT // 2), FAT // 2)
            dst = ring(j * H + h)
            if first and pairs[0] == 0:
                dst[rows, :] = v if sign > 0 else -v
            else:
                dst[rows, :] = dst[rows, :] + v if sign > 0 else dst[rows, :] - v

        slot = [0]

        def after(m):
            run_jobs(jobs, slot[0], 7 * G, m)
            if slot[0] in side:
                side[slot[0]]()
            slot[0] += 1

        for g in range(G):
            for h in (4 * g, 4 * g + 2):
                m2 = product(1, block(h, 0))
                m5 = product(4, block(h + 1, 1))
                if len(pairs) > 1:
                    add(h, 1, m2, True), add(h + 1, 1, m2, True, -1)
                    add(h, 0, m5, True, -1), add(h + 1, 0, m5, True)
                after(m2)
                m1 = product(0, _word_sum(block(h, 0), block(h + 1, 1), 1))
                m4 = product(3, _word_sum(block(h, 1), block(h, 0), -1))
                if len(pairs) > 1:
                    add(h, 0, m1 + m4), add(h + 1, 1, m1), add(h, 1, m4)
                else:
                    add(h, 0, m1 + m4 - m5, True), add(h + 1, 1, m1 - m2, True)
                    add(h, 1, m2 + m4, True), add(h + 1, 0, m5, True)
                after(m1)
                m3 = product(2, _word_sum(block(h + 1, 0), block(h + 1, 1), -1))
                m6 = product(5, _word_sum(block(h, 0), block(h + 1, 0), 1))
                add(h + 1, 0, m3), add(h + 1, 1, m3 + m6)
                after(m3)
            for h in (4 * g, 4 * g + 2):
                m7 = product(6, _word_sum(block(h, 1), block(h + 1, 1), 1))
                add(h, 0, m7)
            after(m7)
            if g in done:
                done[g]()

    def first_segment(t):
        return jnp.concatenate([ring(t)[pl.ds(HEAD, M), :], ring(t)[pl.ds(0, SEG), :]], axis=0)

    p_first = []

    def first_scores():
        p_first.extend(probs(first_segment(h), first_segment(H + h)) for h in range(8))

    def first_values():
        for h in range(4):
            obuf[h] = _dot(p_first[h], first_segment(2 * H + h))
            pbuf[h] = p_first[4 + h]

    _start(mem_copies)
    start_next()
    _wait(mem_copies)
    start_next()
    for job in relayout_jobs([0]):
        job()
    for i, n in enumerate(_STAGES if not _ONLY_MAIN else ()):
      u = stage_start[i]
      j, kt = u // (2 * KT), u // 2 % KT
      jobs = relayout_jobs(range(u + n, stage_start[min(i + 2, len(_STAGES))]))
      if i == 0:
          project(j, kt, range(HH), [])
          for job in jobs:
              job()
          continue
      if jobs:
          need_unit(u + n)
      if i in _EXTRA:
          start_next()
      if n <= 2:
          heads = range(H) if n == 2 else range(u % 2 * HH, (u % 2 + 1) * HH)
          project(j, kt, heads, jobs + (xsum_jobs([2]) if _STAGES[i + 1] > 2 else []))
      elif n == 4:
          project_strassen(j, [kt // 2], jobs + xsum_jobs([3] if kt == 4 else [0, 1]))
      elif jobs:
          project_strassen(j, [kt // 2, kt // 2 + 1], jobs)
      else:
          _wait(vec_copies + xtail_copies)
          start_next()
          side = {q: functools.partial(score_job, q // 2, q % 2) for q in range(2 * n_blk)}
          side[2 * n_blk] = select_tokens
          project_strassen(j, [kt // 2, kt // 2 + 1], jobs, side,
                           {0: first_scores, 2: first_values})
    assert _ONLY_MAIN or progress["started"] == len(queue)
    for t in range(3 * H):
        mqkv[t] = ring(t)[pl.ds(HEAD, M), :]
    gwf[...] = gw[...].astype(_F32)
    ybuf[...] = jnp.zeros(ybuf.shape, _F32)
    xbuf_u[:, pl.ds(S // 2, SEG // 2), :] = jnp.zeros((KT, SEG // 2, _LANE), _U32)

    def ffn_jobs(i):
        part, act = {}, []

        def up_job(w, k, half, _):
            span = pl.ds(half * (D // 2), D // 2)
            r = _dot(xsel[:, span], (wg, wu)[w][i, span, pl.ds(k * _LANE, _LANE)])
            part[w, k] = r if half == 0 else r + part[w, k]

        def down_job(n, _):
            if n == 0:
                act.extend(part[0, k] * _sigmoid(part[0, k]) * part[1, k]
                           for k in range(_FFN_TILES))
            r = _dot(jnp.concatenate(act, axis=1), _bf16(wd_u[i, n]))
            ybuf[:, pl.ds(n * _LANE, _LANE)] += r * rgate[...]

        order = [functools.partial(up_job, w, k, half)
                 for k in range(_FFN_TILES) for w in range(2) for half in range(2)]
        order += [functools.partial(down_job, q) for q in range(KT)]
        jobs = dict(zip(_FPOS, order))
        assert len(jobs) == len(order)
        return jobs

    seg_row = lax.broadcasted_iota(_I32, (SEG, _LANE), 0)

    def mix_jobs(seg, a, copies=None):
        rows = pl.ds(_aligned(seg * (SEG // 2), SEG // 2), SEG // 2)
        gate = []

        def zeros(after):
            z = jnp.zeros((SEG, _LANE), _F32)
            return z if after is None else jnp.where(never, after, z)

        def gate_job(after=None):
            z = zeros(after)
            for kt in range(KT):
                z = z + _bf16(xbuf_u[kt, rows, :]).astype(_F32) * gwf[pl.ds(kt, 1), :]
            gate.append(_sigmoid(jnp.sum(z, axis=-1, keepdims=True)))
            return jnp.broadcast_to(gate[0], (SEG, _LANE)).astype(_BF16)

        def strip_job(kt, after=None):
            upd = zeros(after)
            for c in range(_TOPK):
                upd = jnp.where(seg_row == picks[c] - seg * SEG,
                                ybuf[pl.ds(c, 1), pl.ds(kt * _LANE, _LANE)], upd)
            b = _bf16(xbuf_u[kt, rows, :]).astype(_F32) + upd
            res = (gate[0] * a[kt] + (1.0 - gate[0]) * b).astype(_BF16)
            xbuf_u[kt, rows, :] = pltpu.bitcast(res, _U32)
            if copies:
                copies[kt].start()
            return res

        return [gate_job] + [functools.partial(strip_job, kt) for kt in range(KT)]

    def attention(seg, r0=0):
        rows = pl.ds(_aligned(_rem(seg * SEG, FAT), SEG), SEG)
        o = {h: obuf[h, pl.ds(r0, L - r0), :] for h in range(4)}
        p = {4 + h: pbuf[h, pl.ds(r0, L - r0), :] for h in range(4)}

        def tok(t):
            return jnp.concatenate([mqkv[t], ring(t)[rows, :]], axis=0)

        def scores(g):
            for h in range(4 * g, min(4 * g + 4, H)):
                p[h] = probs(tok(h)[r0:], tok(H + h))

        def values(g):
            for h in range(4 * g, min(4 * g + 4, H)):
                o[h] = _dot(p[h], _v(tok(2 * H + h)))

        return o, scores, values

    def wo_block(g, n):
        return wo_u[n, pl.ds(g * 4 * _WORDS, 4 * _WORDS), :]

    def output_projection(attn, n_rows, jobs=()):
        o, scores, values = attn
        acc = [None] * KT
        for g in range(G):
            lhs = jnp.concatenate([o[4 * g + i][:n_rows] for i in range(4)], axis=1)
            if n_rows % 16 == 0:
                lhs = lhs.astype(_BF16)
            for n in range(KT):
                if n == _QKN:
                    scores(g + 2)
                if n == _PVN:
                    values(g + 1)
                r = _dot(lhs, _bf16(wo_block(g, n)))
                acc[n] = r if g == 0 else r + acc[n]
                if g * KT + n in jobs:
                    jobs[g * KT + n](r)
        return acc

    def wo_sum(gp, np_, k):
        return gp * 5 + k, np_ * (_WORDS // 2)

    def wo_sum_jobs(gp):
        def job(np_, r0, after):
            b11, b12, b21, b22 = (
                wo_u[2 * np_ + c, pl.ds(_aligned((2 * gp + r) * 4 * _WORDS + r0, SEG), SEG), :]
                for r in range(2) for c in range(2))
            after = pltpu.bitcast(after, _U32)
            b11, b22 = jnp.where(never, after, b11), jnp.where(never, after, b22)
            sums = (_word_sum(b11, b22, 1), _word_sum(b12, b22, -1), _word_sum(b21, b11, -1),
                    _word_sum(b11, b12, 1), _word_sum(b21, b22, 1))
            for k, w in enumerate(sums):
                unit, v0 = wo_sum(gp, np_, k)
                stage_u[unit, pl.ds(v0 + r0 // 8, SEG // 8)] = w.reshape(SEG // 8, 8, _LANE)
            return _bf16(sums[4][:SEG // 2])

        return [functools.partial(job, np_, r0)
                for np_ in range(KT // 2) for r0 in range(0, 4 * _WORDS, SEG)]

    def output_projection_strassen(attn, held):
        o, scores, values = attn
        m = {}
        for gp in range(G // 2):
            def rows(g):
                heads = range(4 * g, 4 * g + 4)
                return (jnp.concatenate([jnp.concatenate([o[h][:M]] + [x[h] for x in held],
                                                         axis=0) for h in heads], axis=1),
                        jnp.concatenate([o[h][M:] for h in heads], axis=1))

            count = [0]

            def products(k, lhs, block):
                lhs = lhs.astype(_BF16)
                for np_ in range(KT // 2):
                    for d in range(2):
                        if count[0] == _SQK[d]:
                            scores(2 * gp + 2 + d)
                        if count[0] == _SPV[d]:
                            values(2 * gp + 1 + d)
                    count[0] += 1
                    if isinstance(block, int):
                        unit, v0 = wo_sum(gp, np_, block)
                        w = stage_u[unit, pl.ds(v0, _WORDS // 2)].reshape(4 * _WORDS, _LANE)
                    else:
                        w = wo_block(2 * gp + block[0], 2 * np_ + block[1])
                    r = _dot(lhs, _bf16(w))
                    m[k, np_] = r if gp == 0 else r + m[k, np_]

            a11, a21 = rows(2 * gp)
            products(3, a11, 1)
            products(6, a21 - a11, 3)
            a12, a22 = rows(2 * gp + 1)
            products(1, a11 + a22, 0)
            products(4, a22, 2)
            products(7, a12 - a22, 4)
            products(5, a11 + a12, (1, 1))
            products(2, a21 + a22, (0, 0))
        top, bottom = [], []
        for n in range(KT // 2):
            top += [m[1, n] + m[4, n] + m[7, n] - m[5, n], m[3, n] + m[5, n]]
            bottom += [m[2, n] + m[4, n], m[1, n] + m[3, n] + m[6, n] - m[2, n]]
        return top, bottom

    def project_memory(s, mem, jobs, backlog_jobs=()):
        x0 = HEAD + (s - 1) * XR
        wpos = [_aligned(_rem(x0 + 8 * i, FAT), 8) for i in range(XR // 8)]
        rows = pl.ds(_aligned(_rem(s * SEG, FAT), SEG), SEG)
        h_in = []
        for kt in range(KT):
            xw = xbuf_u[kt, pl.ds(_aligned((HEAD - M) // 2 + (s - 1) * (XR // 2), 4),
                                  SEG // 2), :]
            mw = pltpu.bitcast(jnp.concatenate([mem[kt]] * 2, axis=0).astype(_BF16), _U32)
            h_in.append(_bf16(jnp.concatenate(
                [jnp.where(sublane < M // 2, mw, xw[:8]), xw[8:]], axis=0)))

        stride = _MIXS if len(jobs) < 16 else 2
        side = {_MIX0 + stride * k: job for k, job in enumerate(jobs)}
        side.update({_MIX0 + stride // 2 + stride * k: job for k, job in enumerate(backlog_jobs)})
        mem_rows, p, pending = {}, {}, []

        def weights(t, lo, hi):
            return _bf16(wqkv[t, pl.ds(lo * _WORDS, (hi - lo) * _WORDS), :])

        def finish(t, r):
            for i, w in enumerate(wpos):
                ring(t)[pl.ds(w, 8), :] = r[M + 8 * i:M + 8 * i + 8]
            mqkv[t] = mem_rows[t] = r[:M]

        def tok(t):
            return jnp.concatenate([mem_rows[t], ring(t)[rows, :]], axis=0)

        first = [j * H + h for h in range(2) for j in range(3)][:_NFIRST]
        lo = jnp.concatenate(h_in[:KT // 2], axis=1)
        hi = jnp.concatenate(h_in[KT // 2:], axis=1)
        part = [_dot(lo, weights(t, 0, KT // 2)) for t in first]
        for t, r in zip(first, part):
            finish(t, _dot(hi, weights(t, KT // 2, KT)) + r)
        for g in range(G):
            for i in range(4):
                for j in range(3):
                    t = j * H + 4 * g + i
                    if t not in first:
                        h0 = h_in[0]
                        if pending and pending[0][0] == 0:
                            h0 = jnp.where(never, pending.pop(0)[1], h0)
                        pending[:] = [(d - 1, v) for d, v in pending]
                        r = _dot(jnp.concatenate([h0] + h_in[1:], axis=1), weights(t, 0, KT))
                        finish(t, r)
                        if 12 * g + 3 * i + j in side:
                            pending.append((_DELAY, side[12 * g + 3 * i + j](r if _TIEIN else None)))
                if g == _QKG and i == 0:
                    for h in range(4):
                        p[h] = probs(tok(h), tok(H + h))
                    for h in range(4):
                        pbuf[h] = probs(tok(4 + h), tok(H + 4 + h))
                if g == _PVG and i == 0:
                    for h in range(4):
                        obuf[h] = _dot(p[h], _v(tok(2 * H + h)))

    def slot(seg):
        return _rem(seg, abuf.shape[0])

    def block_rows(seg):
        return [abuf[slot(seg), n] for n in range(KT)]

    def ffn_step(i, carry):
        _wait(ffn_copies(0, i))
        acc = output_projection(attention(i), L, ffn_jobs(i))
        for n in range(KT):
            abuf[i, n] = acc[n][M:]
        project_memory(i + 1, [a[:M] for a in acc], wo_sum_jobs(jnp.minimum(i, G // 2 - 1)))
        return carry

    LAG = SEG // M

    def main_steps(i, carry):
        held = []
        for k in range(LAG):
            seg = NB + i * LAG + k
            attn = attention(seg)
            if k < LAG - 1:
                acc = output_projection(attn, SEG)
                held.append({h: v[SEG:] for h, v in attn[0].items()})
                for n in range(KT):
                    abuf[slot(seg), n, pl.ds(0, XR), :] = acc[n][M:]
            else:
                acc, tokens = output_projection_strassen(attn, held)
                for n in range(KT):
                    abuf[slot(seg), n] = tokens[n]
                    for e in range(1, LAG):
                        abuf[slot(seg - LAG + e), n, pl.ds(XR, M), :] = acc[n][e * M:e * M + M]
            if k == 0:
                old = mix_jobs(jnp.where(i < n_old, i, n_seg), block_rows(i))
            done = seg - LAG + 1
            project_memory(seg + 1, [a[:M] for a in acc], mix_jobs(done, block_rows(done)),
                           old if k == 0 else ())
            _start(out_copies(done))
            if k == 0:
                pl.when(i < n_old)(lambda: _start(out_copies(i)))
        return carry

    n_old = NB - LAG + 1
    assert (n_seg - 1 - NB) % LAG == 0
    _wait(wo_copies)
    _start([cp for i in range(3, NB) for cp in ffn_copies(i)])
    if _ONLY_MAIN != 1: lax.fori_loop(0, NB, ffn_step, 0)
    if _ONLY_MAIN != 2: lax.fori_loop(0, (n_seg - 1 - NB) // LAG, main_steps, 0)
    jobs = [job for seg in range(n_seg - LAG, n_seg - 1)
            for job in mix_jobs(seg, block_rows(seg), out_copies(seg))]
    acc = output_projection(attention(n_seg - 1, M), SEG,
                            {2 * q: job for q, job in enumerate(jobs)})
    for job in mix_jobs(n_seg - 1, acc, out_copies(n_seg - 1)):
        job()
    _wait(out_copies(0, n_seg))


@functools.partial(jax.jit, static_argnames=("A_seg_len",))
def pallas_gated_mix__memory_aug_recurrent_mem_tr__moe_arch_mod__prompt_kernel(
    A_x, A_mem0, A_Wq, A_Wk, A_Wv, A_Wo, A_seg_len, B_x, B_w_r, B_w_gate, B_w_up,
    B_w_down, gate_w,
):
    del B_x
    B, S, D = A_x.shape
    _, H, DH = A_Wq.shape
    M = A_mem0.shape[1]
    SEG = int(A_seg_len)
    F = B_w_gate.shape[1]
    assert (B, S, D, H, DH, M, SEG) == (1, 2048, 1024, 32, _LANE, 8, 32) and F == 3584
    L = M + SEG
    KT, FT = D // _LANE, F // _LANE
    fat = S - (S // SEG - 1) * (SEG - M) + M
    n_ffn = -(-FT // _FFN_TILES)

    any_spec = pl.BlockSpec(memory_space=pl.ANY)
    dma = pltpu.SemaphoreType.DMA
    out = pl.pallas_call(
        functools.partial(_kernel, S=S, D=D, H=H, DH=DH, M=M, SEG=SEG, F=F),
        out_shape=jax.ShapeDtypeStruct((S, D), A_x.dtype),
        in_specs=[any_spec] * 11,
        out_specs=any_spec,
        scratch_shapes=[
            pltpu.VMEM((KT, S + SEG, _LANE), _BF16),
            pltpu.VMEM((6 * KT, _LANE, H // 2, DH), _BF16),
            pltpu.VMEM((3 * H, D // 2, DH), _U32),
            pltpu.VMEM((KT, H * DH, _LANE), _BF16),
            pltpu.VMEM((n_ffn, D, _FFN_TILES * _LANE), _BF16),
            pltpu.VMEM((n_ffn, D, _FFN_TILES * _LANE), _BF16),
            pltpu.VMEM((n_ffn, KT, _FFN_TILES * _LANE, _LANE), _BF16),
            [pltpu.VMEM((12, fat, DH), _F32)] * (H // 4),
            pltpu.VMEM((KT // 2, 7, fat // 4, _LANE), _U32),
            pltpu.VMEM((20, KT, SEG, _LANE), _F32),
            pltpu.VMEM((4, L, DH), _F32),
            pltpu.VMEM((4, L, L), _F32),
            pltpu.VMEM((3 * H, M, DH), _F32),
            pltpu.VMEM((_TOPK, D), _F32),
            pltpu.VMEM((_TOPK, D), _F32),
            pltpu.VMEM((KT, M, _LANE), _BF16),
            pltpu.VMEM((KT, _LANE), _BF16),
            pltpu.VMEM((KT, _LANE), _BF16),
            pltpu.VMEM((KT, _LANE), _F32),
            pltpu.VMEM((_TOPK, _LANE), _F32),
            pltpu.SMEM((_TOPK,), _I32),
            dma((len(_BATCHES),)), dma((KT,)), dma(()), dma((2,)), dma(()), dma((n_ffn,)),
            dma(()),
        ],
        compiler_params=pltpu.CompilerParams(vmem_limit_bytes=120 * 1024 * 1024,
                                             disable_bounds_checks=True),
        name="gated_mix_rmt_mod",
    )(
        A_x.reshape(S, D), A_mem0.reshape(M, D), A_Wq.reshape(D, 2, H // 2, DH),
        A_Wk.reshape(D, 2, H // 2, DH), A_Wv.reshape(D, 2, H // 2, DH),
        A_Wo.reshape(H * DH, D), B_w_r.reshape(KT, _LANE), B_w_gate, B_w_up, B_w_down,
        gate_w.reshape(KT, _LANE),
    )
    return out.reshape(B, S, D)
```

```python
import functools

import jax
import jax.numpy as jnp
import numpy as np
from jax import lax
import jax.experimental.pallas as pl
import jax.experimental.pallas.tpu as pltpu

_F32 = jnp.float32
_BF16 = jnp.bfloat16
_U32 = jnp.uint32
_I32 = jnp.int32
_NN = (((1,), (0,)), ((), ()))
_NT = (((1,), (1,)), ((), ()))

_LANE = 128
_WORDS = _LANE // 2
_TOPK = 8
_FFN_TILES = 4
_STAGES = (1, 1, 1, 1, 2, 2, 4, 4, 8, 8, 8, 8)
_BATCHES = (1, 1, 1, 1, 2, 2, 4, 4, 4, 4, 4, 4, 8, 8)


def _dot(a, b, dims=_NN):
    return lax.dot_general(a, b, dims, preferred_element_type=_F32)


def _aligned(i, n):
    return i if isinstance(i, int) else pl.multiple_of(i, n)


def _rem(i, n):
    return i % n if isinstance(i, int) else lax.rem(i, n)


def _sigmoid(v):
    return 1.0 / (1.0 + jnp.exp(-v))


def _bf16(words):
    return pltpu.bitcast(words, _BF16)


def _words(v):
    return pltpu.bitcast(v, _U32)


def _sum(a, b, sign):
    a, b = _bf16(a).astype(_F32), _bf16(b).astype(_F32)
    return (a + b if sign > 0 else a - b).astype(_BF16)


def _start(copies):
    for cp in copies:
        cp.start()


def _wait(copies):
    for cp in copies:
        cp.wait()


def _kernel(x_hbm, mem_hbm, wq_hbm, wk_hbm, wv_hbm, wo_hbm, wr_hbm, wg_hbm, wu_hbm,
            wd_hbm, gw_hbm, out_hbm,
            xbuf, stage, wqkv, wo, wg, wu, wd, rings, xsum, abuf, obuf, pbuf, mqkv, xsel,
            ybuf, membuf, wr, gw, gwf, rgate, picks,
            sem_w, sem_xh, sem_xt, sem_small, sem_wo, sem_b, sem_out,
            *, S, D, H, DH, M, SEG):
    L = M + SEG
    n_seg = S // SEG
    KT = D // _LANE
    G = H // 4
    HH = H // 2
    XR = SEG - M
    HEAD = S - (n_seg - 1) * XR
    FAT = HEAD + M
    NB = wg.shape[0]
    PERIOD = SEG // M
    w_hbm = (wq_hbm, wk_hbm, wv_hbm)

    stage_u, xbuf_u, membuf_u, wo_u, wd_u = (
        r.bitcast(_U32) for r in (stage, xbuf, membuf, wo, wd))

    def ring(t):
        j, h = divmod(t, H)
        return rings[h // 4].at[j * 4 + h % 4]

    picks[0] = 0
    never = picks[0] > 0

    def after(other, v):
        return v if other is None else jnp.where(never, other, v)

    sublane = lax.broadcasted_iota(_I32, (8, _LANE), 0)

    batch_start = np.cumsum((0,) + _BATCHES).tolist()
    stage_start = np.cumsum((0,) + _STAGES).tolist()

    def batch_copies(i):
        copies = []
        for u in range(batch_start[i], batch_start[i + 1]):
            j, kt, half = u // (2 * KT), u // 2 % KT, u % 2
            if j == 0 and half == 0:
                copies.append(pltpu.make_async_copy(
                    x_hbm.at[pl.ds(0, FAT), pl.ds(kt * _LANE, _LANE)],
                    xbuf.at[kt, pl.ds(0, FAT), :], sem_xh.at[kt]))
            copies.append(pltpu.make_async_copy(
                w_hbm[j].at[pl.ds(kt * _LANE, _LANE), half], stage.at[u], sem_w.at[i]))
        return copies

    def strip_copies(src, dst, sem):
        return [pltpu.make_async_copy(src.at[:, pl.ds(n * _LANE, _LANE)], dst.at[n], sem)
                for n in range(KT)]

    def ffn_copies(i):
        units = pl.ds(_aligned(i * _FFN_TILES * _LANE, _LANE), _FFN_TILES * _LANE)
        return [pltpu.make_async_copy(wg_hbm.at[:, units], wg.at[i], sem_b.at[i]),
                pltpu.make_async_copy(wu_hbm.at[:, units], wu.at[i], sem_b.at[i])
                ] + strip_copies(wd_hbm.at[units, :], wd.at[i], sem_b.at[i])

    def out_copies(seg, n=1):
        rows = pl.ds(_aligned(seg * SEG, SEG), n * SEG)
        return [pltpu.make_async_copy(xbuf.at[kt, rows, :],
                                      out_hbm.at[rows, pl.ds(kt * _LANE, _LANE)], sem_out)
                for kt in range(KT)]

    mem_copies = strip_copies(mem_hbm, membuf, sem_small.at[0])
    rest_copies = [pltpu.make_async_copy(wr_hbm, wr, sem_small.at[1]),
                   pltpu.make_async_copy(gw_hbm, gw, sem_small.at[1])]
    rest_copies += [pltpu.make_async_copy(
        x_hbm.at[pl.ds(FAT, S - FAT), pl.ds(kt * _LANE, _LANE)],
        xbuf.at[kt, pl.ds(FAT, S - FAT), :], sem_xt) for kt in range(KT)]
    wo_copies = strip_copies(wo_hbm, wo, sem_wo)

    queue = [batch_copies(i) for i in range(len(_BATCHES))]
    queue += [rest_copies, wo_copies, ffn_copies(0), ffn_copies(1)]
    progress = {"started": 0, "arrived": 0}

    def start_next():
        _start(queue[progress["started"]])
        progress["started"] += 1

    def need_unit(u):
        while batch_start[progress["arrived"]] <= u:
            _wait(queue[progress["arrived"]])
            progress["arrived"] += 1
            start_next()

    row = lax.broadcasted_iota(_I32, (L, L), 0)
    col = lax.broadcasted_iota(_I32, (L, L), 1)
    mask = (row < M) | (row >= col)
    scale = DH ** (-0.5)

    def probs(q, k):
        sc = jnp.where(mask[L - q.shape[0]:], _dot(q, k, _NT), -1000000000.0 / scale)
        e = jnp.exp2((sc - jnp.max(sc, axis=-1, keepdims=True)) * float(scale * np.log2(np.e)))
        total = jnp.sum(e, axis=-1, keepdims=True)
        inv = pltpu.reciprocal(total, approx=True)
        return e * (inv * (2.0 - total * inv))

    def weighted(p, v):
        return _dot(p, v.astype(_BF16))

    n_blk = S // _LANE
    score = [None] * n_blk

    def score_job(b, half):
        kts = range(half * KT // 2, (half + 1) * KT // 2)
        wrf = wr[...].astype(_F32)
        w = jnp.concatenate([jnp.broadcast_to(wrf[kt:kt + 1], (8, _LANE)) for kt in kts],
                            axis=1)
        xb = jnp.concatenate([_bf16(xbuf_u[kt, pl.ds(b * _WORDS, _WORDS), :]) for kt in kts],
                             axis=1)
        r = _dot(w, xb, _NT)
        score[b] = r if half == 0 else r + score[b]

    def select_jobs():
        state = {}
        pos = (lax.broadcasted_iota(_I32, (n_blk, _LANE), 0) * _LANE
               + lax.broadcasted_iota(_I32, (n_blk, _LANE), 1)).astype(_F32)

        def job(c):
            if c == 0:
                r_all = []
                for b0 in range(0, n_blk, 8):
                    r = score[b0]
                    for b in range(1, 8):
                        r = jnp.where(sublane == b, score[b0 + b], r)
                    r_all.append(r)
                r_all = jnp.concatenate(r_all, axis=0).astype(_BF16).astype(_F32)
                r_all = jnp.where(r_all == 0.0, 0.0, r_all)
                bits = pltpu.bitcast(r_all, _I32)
                key = jnp.where(bits < 0, bits ^ np.int32(0x7FFFFFFF), bits) >> 16
                key = jnp.where(r_all != r_all, np.int32(-(1 << 15)), key)
                state.update(r=r_all, key=key.astype(_F32))
            best = jnp.max(state["key"], keepdims=True)
            pick = jnp.min(jnp.where(state["key"] == best, pos, float(S)), keepdims=True)
            hit = pos == pick
            state["key"] = jnp.where(hit, -float(1 << 17), state["key"])
            r_c = jnp.sum(jnp.where(hit, state["r"], 0.0), keepdims=True)
            rgate[pl.ds(c, 1), :] = jnp.broadcast_to(_sigmoid(r_c), (1, _LANE))
            token = pick[0, 0].astype(_I32)
            picks[c] = token
            base = pl.multiple_of((token >> 3) << 3, 8)
            for kt in range(KT):
                grp = xbuf[kt, pl.ds(base, 8), :].astype(_F32)
                one = jnp.sum(jnp.where(sublane == (token & 7), grp, 0.0), axis=0,
                              keepdims=True)
                xsel[pl.ds(c, 1), pl.ds(kt * _LANE, _LANE)] = one
            return _words(jnp.broadcast_to(one, (8, _LANE)))

        return [functools.partial(job, c) for c in range(_TOPK)]

    def transpose8(v):
        c = [v[0]] + [pltpu.roll(v[8 - m], 8 - m, 0) for m in range(1, 8)]
        for d in (1, 2, 4):
            c = [jnp.where((sublane & d) != 0, c[m - d], c[m]) for m in range(8)]
        return [c[0]] + [pltpu.roll(c[k], 8 - k, 0) for k in range(1, 8)]

    def relayout(u, db, odd, prev=None):
        need_unit(u)
        j, kt, half = u // (2 * KT), u // 2 % KT, u % 2
        words = []
        for t in range(8):
            a = stage_u[u, db * 16 + 2 * t]
            b = stage_u[u, db * 16 + 2 * t + 1]
            if odd:
                words.append((a >> 16) | (b & np.uint32(0xFFFF0000)))
            else:
                words.append((a & np.uint32(0xFFFF)) | (b << 16))
        words[0] = after(prev, words[0])
        for t, w in enumerate(transpose8(words)):
            wqkv[j * H + half * HH + 2 * t + odd, pl.ds(kt * _WORDS + db * 8, 8), :] = w

    def relayout_jobs(units):
        return [functools.partial(relayout, u, db, odd)
                for u in units for db in range(_LANE // 16) for odd in range(2)]

    def head_rows(kt, r0, n):
        n_x = min(n, HEAD // 2 - r0)
        rows = xbuf_u[kt, pl.ds(r0, n_x), :]
        return rows if n_x == n else jnp.concatenate([rows, membuf_u[kt]], axis=0)

    def xsum_job(pair, r0, prev):
        a11, a12, a21, a22 = (head_rows(2 * pair + k, half * (FAT // 4) + r0, 8)
                              for half in range(2) for k in range(2))
        a11, a22 = after(prev, a11), after(prev, a22)
        factors = (_words(_sum(a11, a22, 1)), _words(_sum(a21, a22, 1)), a11, a22,
                   _words(_sum(a11, a12, 1)), _words(_sum(a21, a11, -1)),
                   _words(_sum(a12, a22, -1)))
        for k, w in enumerate(factors):
            xsum[pair, k, pl.ds(r0, 8), :] = w

    def xsum_jobs(pairs):
        return [functools.partial(xsum_job, pair, r0)
                for pair in pairs for r0 in range(0, FAT // 4, 8)]

    def run_share(jobs, i, n, result):
        mine = jobs[i * len(jobs) // n:(i + 1) * len(jobs) // n]
        for k, job in enumerate(mine):
            r0 = k * (result.shape[0] // 8) // len(mine) * 8
            job(_words(result[r0:r0 + 8]))

    def project(j, kt, heads, jobs):
        lhs = _bf16(head_rows(kt, 0, FAT // 2))
        for i, h in enumerate(heads):
            r = _dot(lhs, _bf16(wqkv[j * H + h, pl.ds(kt * _WORDS, _WORDS), :]))
            dst = ring(j * H + h)
            dst[...] = r + dst[...] if kt > 0 else r
            if i % 4 == 3:
                run_share(jobs, i // 4, len(heads) // 4, r)

    def project_strassen(j, pairs, jobs, side=()):
        slot, due = [0], {}

        def product(k, b):
            lhs = [xsum[p, k - 1] for p in pairs]
            if slot[0] in due:
                lhs[0] = jnp.concatenate([after(due.pop(slot[0]), lhs[0][:8]), lhs[0][8:]],
                                         axis=0)
            return _dot(jnp.concatenate([_bf16(a) for a in lhs], axis=1), b)

        def block(h, k):
            return jnp.concatenate(
                [wqkv[j * H + h, pl.ds((2 * p + k) * _WORDS, _WORDS), :] for p in pairs],
                axis=0)

        def add(h, half, v, first=False, sign=1):
            rows = pl.ds(half * (FAT // 2), FAT // 2)
            dst = ring(j * H + h)
            if first and pairs[0] == 0:
                dst[rows, :] = v if sign > 0 else -v
            else:
                dst[rows, :] = dst[rows, :] + v if sign > 0 else dst[rows, :] - v

        def next_slot(m):
            run_share(jobs, slot[0], 7 * G, m)
            for job in side[slot[0]] if slot[0] in side else ():
                v = job()
                if v is not None:
                    due[slot[0] + 5] = v
            slot[0] += 1

        for g in range(G):
            for h in (4 * g, 4 * g + 2):
                m2 = product(2, _bf16(block(h, 0)))
                m5 = product(5, _bf16(block(h + 1, 1)))
                if len(pairs) > 1:
                    add(h, 1, m2, True)
                    add(h + 1, 1, m2, True, -1)
                    add(h, 0, m5, True, -1)
                    add(h + 1, 0, m5, True)
                next_slot(m2)
                m1 = product(1, _sum(block(h, 0), block(h + 1, 1), 1))
                m4 = product(4, _sum(block(h, 1), block(h, 0), -1))
                if len(pairs) > 1:
                    add(h, 0, m1 + m4)
                    add(h + 1, 1, m1)
                    add(h, 1, m4)
                else:
                    add(h, 0, m1 + m4 - m5, True)
                    add(h + 1, 1, m1 - m2, True)
                    add(h, 1, m2 + m4, True)
                    add(h + 1, 0, m5, True)
                next_slot(m1)
                m3 = product(3, _sum(block(h + 1, 0), block(h + 1, 1), -1))
                m6 = product(6, _sum(block(h, 0), block(h + 1, 0), 1))
                add(h + 1, 0, m3)
                add(h + 1, 1, m3 + m6)
                next_slot(m3)
            for h in (4 * g, 4 * g + 2):
                m7 = product(7, _sum(block(h, 1), block(h + 1, 1), 1))
                add(h, 0, m7)
            next_slot(m7)

    def first_segment(t):
        return jnp.concatenate([ring(t)[pl.ds(HEAD, M), :], ring(t)[pl.ds(0, SEG), :]], axis=0)

    p_first = []

    def first_scores():
        p_first.extend(probs(first_segment(h), first_segment(H + h)) for h in range(8))

    def first_values():
        for h in range(4):
            obuf[h] = weighted(p_first[h], first_segment(2 * H + h))
            pbuf[h] = p_first[4 + h]

    _start(mem_copies)
    start_next()
    _wait(mem_copies)
    start_next()
    for job in relayout_jobs([0]):
        job()
    for i, n in enumerate(_STAGES):
        u = stage_start[i]
        j, kt = u // (2 * KT), u // 2 % KT
        jobs = relayout_jobs(range(u + n, stage_start[min(i + 2, len(_STAGES))]))
        if i == 0:
            project(j, kt, range(HH), [])
            for job in jobs:
                job()
            continue
        if jobs:
            need_unit(u + n)
        if i in (7, 8):
            start_next()
        if i == len(_STAGES) - 2:
            _wait(rest_copies)
        if n <= 2:
            heads = range(H) if n == 2 else range(u % 2 * HH, (u % 2 + 1) * HH)
            project(j, kt, heads, jobs + (xsum_jobs([2]) if _STAGES[i + 1] > 2 else []))
        elif n == 4:
            project_strassen(j, [kt // 2], jobs + xsum_jobs([3] if kt == 4 else [0, 1]))
        elif jobs:
            project_strassen(j, [kt // 2, kt // 2 + 1], jobs)
        else:
            side = {q: [functools.partial(score_job, q // 2, q % 2)] for q in range(2 * n_blk)}
            side.update({2 * n_blk + 5 * c // 2: [job] for c, job in enumerate(select_jobs())})
            side[6].append(first_scores)
            side[20].append(first_values)
            project_strassen(j, [kt // 2, kt // 2 + 1], jobs, side)
    assert progress["started"] == len(queue)
    for t in range(3 * H):
        mqkv[t] = ring(t)[pl.ds(HEAD, M), :]
    gwf[...] = gw[...].astype(_F32)
    ybuf[...] = jnp.zeros(ybuf.shape, _F32)
    xbuf_u[:, pl.ds(S // 2, SEG // 2), :] = jnp.zeros((KT, SEG // 2, _LANE), _U32)

    def ffn_jobs(i):
        part, act = {}, []

        def up_job(w, k, half, _):
            span = pl.ds(half * (D // 2), D // 2)
            r = _dot(xsel[:, span], (wg, wu)[w][i, span, pl.ds(k * _LANE, _LANE)])
            part[w, k] = r if half == 0 else r + part[w, k]

        def down_job(n, _):
            if n == 0:
                act.extend(part[0, k] * _sigmoid(part[0, k]) * part[1, k]
                           for k in range(_FFN_TILES))
            r = _dot(jnp.concatenate(act, axis=1), _bf16(wd_u[i, n]))
            ybuf[:, pl.ds(n * _LANE, _LANE)] += r * rgate[...]

        ups = [functools.partial(up_job, w, k, half)
               for k in range(_FFN_TILES) for w in range(2) for half in range(2)]
        jobs = {1 + 5 * q // 2: job for q, job in enumerate(ups)}
        jobs.update({q: functools.partial(down_job, n)
                     for n, q in enumerate((45, 47, 50, 53, 55, 58, 61, 63))})
        return jobs

    seg_row = lax.broadcasted_iota(_I32, (SEG, _LANE), 0)

    def mix_jobs(seg, a, copies=None):
        rows = pl.ds(_aligned(seg * (SEG // 2), SEG // 2), SEG // 2)
        gate = []

        def gate_job(prev=None):
            z = after(prev, jnp.zeros((SEG, _LANE), _F32))
            for kt in range(KT):
                z = z + _bf16(xbuf_u[kt, rows, :]).astype(_F32) * gwf[pl.ds(kt, 1), :]
            gate.append(_sigmoid(jnp.sum(z, axis=-1, keepdims=True)))
            return jnp.broadcast_to(gate[0], (SEG, _LANE)).astype(_BF16)

        def strip_job(kt, prev=None):
            upd = after(prev, jnp.zeros((SEG, _LANE), _F32))
            for c in range(_TOPK):
                upd = jnp.where(seg_row == picks[c] - seg * SEG,
                                ybuf[pl.ds(c, 1), pl.ds(kt * _LANE, _LANE)], upd)
            b = _bf16(xbuf_u[kt, rows, :]).astype(_F32) + upd
            res = (gate[0] * a[kt] + (1.0 - gate[0]) * b).astype(_BF16)
            xbuf_u[kt, rows, :] = _words(res)
            if copies:
                copies[kt].start()
            return res

        return [gate_job] + [functools.partial(strip_job, kt) for kt in range(KT)]

    def attention(seg, r0=0):
        rows = pl.ds(_aligned(_rem(seg * SEG, FAT), SEG), SEG)
        o = {h: obuf[h, pl.ds(r0, L - r0), :] for h in range(4)}
        p = {4 + h: pbuf[h, pl.ds(r0, L - r0), :] for h in range(4)}

        def tok(t):
            return jnp.concatenate([mqkv[t], ring(t)[rows, :]], axis=0)

        def scores(g):
            for h in range(4 * g, min(4 * g + 4, H)):
                p[h] = probs(tok(h)[r0:], tok(H + h))

        def values(g):
            for h in range(4 * g, min(4 * g + 4, H)):
                o[h] = weighted(p[h], tok(2 * H + h))

        return o, scores, values

    def wo_block(g, n):
        return wo_u[n, pl.ds(g * 4 * _WORDS, 4 * _WORDS), :]

    def output_projection(attn, n_rows, jobs=()):
        o, scores, values = attn
        acc, due = [None] * KT, {}
        for g in range(G):
            lhs = [o[4 * g + i][:n_rows] for i in range(4)]
            if n_rows % 16 == 0:
                lhs = [v.astype(_BF16) for v in lhs]
            for n in range(KT):
                if n == 1:
                    scores(g + 2)
                if n == 3:
                    values(g + 1)
                q = g * KT + n
                r = _dot(jnp.concatenate([after(due.get(q), lhs[0])] + lhs[1:], axis=1),
                         _bf16(wo_block(g, n)))
                acc[n] = r if g == 0 else r + acc[n]
                if q in jobs:
                    due[q + 17] = jobs[q](r)
        return acc

    def wo_sum_jobs(gp):
        def job(c, r0, prev):
            b11, b12, b21, b22 = (
                wo_u[2 * c + n, pl.ds(_aligned((2 * gp + g) * 4 * _WORDS + r0, SEG), SEG), :]
                for g in range(2) for n in range(2))
            b11, b22 = after(_words(prev), b11), after(_words(prev), b22)
            sums = [_words(v) for v in (_sum(b11, b22, 1), _sum(b12, b22, -1),
                                        _sum(b21, b11, -1), _sum(b11, b12, 1),
                                        _sum(b21, b22, 1))]
            for k, w in enumerate(sums):
                stage_u[gp * 5 + k, pl.ds(c * (_WORDS // 2) + r0 // 8, SEG // 8)] = (
                    w.reshape(SEG // 8, 8, _LANE))
            return _bf16(sums[-1][:SEG // 2])

        return [functools.partial(job, c, r0)
                for c in range(KT // 2) for r0 in range(0, 4 * _WORDS, SEG)]

    def output_projection_strassen(attn, held):
        o, scores, values = attn
        m = {}
        for gp in range(G // 2):
            due = {0: functools.partial(values, 2 * gp + 1),
                   1: functools.partial(scores, 2 * gp + 2),
                   10: functools.partial(scores, 2 * gp + 3),
                   18: functools.partial(values, 2 * gp + 2)}
            count = [0]

            def halves(g):
                heads = range(4 * g, 4 * g + 4)
                return (jnp.concatenate([jnp.concatenate([o[h][:M]] + [x[h] for x in held],
                                                         axis=0) for h in heads], axis=1),
                        jnp.concatenate([o[h][M:] for h in heads], axis=1))

            def products(k, lhs, factor):
                lhs = lhs.astype(_BF16)
                for c in range(KT // 2):
                    if count[0] in due:
                        due[count[0]]()
                    count[0] += 1
                    r = _dot(lhs, _bf16(factor(c)))
                    m[k, c] = r if gp == 0 else r + m[k, c]

            def kept(k):
                return lambda c: stage_u[gp * 5 + k, pl.ds(c * (_WORDS // 2), _WORDS // 2)
                                         ].reshape(4 * _WORDS, _LANE)

            a11, a21 = halves(2 * gp)
            products(3, a11, kept(1))
            products(6, a21 - a11, kept(3))
            a12, a22 = halves(2 * gp + 1)
            products(1, a11 + a22, kept(0))
            products(4, a22, kept(2))
            products(7, a12 - a22, kept(4))
            products(5, a11 + a12, lambda c: wo_block(2 * gp + 1, 2 * c + 1))
            products(2, a21 + a22, lambda c: wo_block(2 * gp, 2 * c))
        top, bottom = [], []
        for c in range(KT // 2):
            top += [m[1, c] + m[4, c] + m[7, c] - m[5, c], m[3, c] + m[5, c]]
            bottom += [m[2, c] + m[4, c], m[1, c] + m[3, c] + m[6, c] - m[2, c]]
        return top, bottom

    def project_memory(s, mem, jobs):
        x0 = HEAD + (s - 1) * XR
        wpos = [_aligned(_rem(x0 + 8 * i, FAT), 8) for i in range(XR // 8)]
        rows = pl.ds(_aligned(_rem(s * SEG, FAT), SEG), SEG)
        h_in = []
        for kt in range(KT):
            xw = xbuf_u[kt, pl.ds(_aligned((HEAD - M) // 2 + (s - 1) * (XR // 2), 4),
                                  SEG // 2), :]
            mw = _words(jnp.concatenate([mem[kt]] * 2, axis=0).astype(_BF16))
            h_in.append(_bf16(jnp.concatenate(
                [jnp.where(sublane < M // 2, mw, xw[:8]), xw[8:]], axis=0)))
        mem_rows, p, due = {}, {}, {}

        def weights(t, lo, hi):
            return _bf16(wqkv[t, pl.ds(lo * _WORDS, (hi - lo) * _WORDS), :])

        def finish(t, r):
            for i, w in enumerate(wpos):
                ring(t)[pl.ds(w, 8), :] = r[M + 8 * i:M + 8 * i + 8]
            mqkv[t] = mem_rows[t] = r[:M]

        def tok(t):
            return jnp.concatenate([mem_rows[t], ring(t)[rows, :]], axis=0)

        tiles = [j * H + h for h in range(H) for j in range(3)]
        lo = jnp.concatenate(h_in[:KT // 2], axis=1)
        hi = jnp.concatenate(h_in[KT // 2:], axis=1)
        part = [_dot(lo, weights(t, 0, KT // 2)) for t in tiles[:6]]
        for q, t in enumerate(tiles):
            if q < len(part):
                finish(t, _dot(hi, weights(t, KT // 2, KT)) + part[q])
                continue
            r = _dot(jnp.concatenate([after(due.get(q), h_in[0])] + h_in[1:], axis=1),
                     weights(t, 0, KT))
            finish(t, r)
            if q in jobs:
                due[q + 8] = jobs[q](r)
            if q == 74:
                for h in range(4):
                    p[h] = probs(tok(h), tok(H + h))
                for h in range(4):
                    pbuf[h] = probs(tok(4 + h), tok(H + 4 + h))
            if q == 86:
                for h in range(4):
                    obuf[h] = weighted(p[h], tok(2 * H + h))

    def slot(seg):
        return _rem(seg, abuf.shape[0])

    def block_rows(seg):
        return [abuf[slot(seg), n] for n in range(KT)]

    def ffn_step(i, carry):
        _wait(ffn_copies(i))
        pl.when(i + 2 < NB)(lambda: _start(ffn_copies(i + 2)))
        acc = output_projection(attention(i), L, ffn_jobs(i))
        for n in range(KT):
            abuf[i, n] = acc[n][M:]
        jobs = wo_sum_jobs(jnp.minimum(i, G // 2 - 1))
        project_memory(i + 1, [a[:M] for a in acc],
                       {7 + 2 * k: job for k, job in enumerate(jobs)})
        return carry

    n_old = NB - PERIOD + 1

    def main_steps(i, carry):
        held = []
        for k in range(PERIOD):
            seg = NB + i * PERIOD + k
            attn = attention(seg)
            if k < PERIOD - 1:
                acc = output_projection(attn, SEG)
                held.append({h: v[SEG:] for h, v in attn[0].items()})
                for n in range(KT):
                    abuf[slot(seg), n, pl.ds(0, XR), :] = acc[n][M:]
            else:
                acc, tokens = output_projection_strassen(attn, held)
                for n in range(KT):
                    abuf[slot(seg), n] = tokens[n]
                    for e in range(1, PERIOD):
                        abuf[slot(seg - PERIOD + e), n, pl.ds(XR, M), :] = (
                            acc[n][e * M:e * M + M])
            jobs = {}
            if k == 0:
                old = mix_jobs(jnp.where(i < n_old, i, n_seg), block_rows(i))
                jobs.update({10 + 6 * q: job for q, job in enumerate(old)})
            done = seg - PERIOD + 1
            jobs.update({7 + 6 * q: job
                         for q, job in enumerate(mix_jobs(done, block_rows(done)))})
            project_memory(seg + 1, [a[:M] for a in acc], jobs)
            _start(out_copies(done))
            if k == 0:
                pl.when(i < n_old)(lambda: _start(out_copies(i)))
        return carry

    assert (n_seg - 1 - NB) % PERIOD == 0
    _wait(wo_copies)
    lax.fori_loop(0, NB, ffn_step, 0)
    lax.fori_loop(0, (n_seg - 1 - NB) // PERIOD, main_steps, 0)
    jobs = [job for seg in range(n_seg - PERIOD, n_seg - 1)
            for job in mix_jobs(seg, block_rows(seg), out_copies(seg))]
    acc = output_projection(attention(n_seg - 1, M), SEG,
                            {q * 7 // 4: job for q, job in enumerate(jobs)})
    for job in mix_jobs(n_seg - 1, acc, out_copies(n_seg - 1)):
        job()
    _wait(out_copies(0, n_seg))


@functools.partial(jax.jit, static_argnames=("A_seg_len",))
def pallas_gated_mix__memory_aug_recurrent_mem_tr__moe_arch_mod__prompt_kernel(
    A_x, A_mem0, A_Wq, A_Wk, A_Wv, A_Wo, A_seg_len, B_x, B_w_r, B_w_gate, B_w_up,
    B_w_down, gate_w,
):
    del B_x
    B, S, D = A_x.shape
    _, H, DH = A_Wq.shape
    M = A_mem0.shape[1]
    SEG = int(A_seg_len)
    F = B_w_gate.shape[1]
    assert (B, S, D, H, DH, M, SEG, F) == (1, 2048, 1024, 32, _LANE, 8, 32, 3584)
    L = M + SEG
    KT = D // _LANE
    fat = S - (S // SEG - 1) * (SEG - M) + M
    units = _FFN_TILES * _LANE
    n_ffn = F // units

    any_spec = pl.BlockSpec(memory_space=pl.ANY)
    dma = pltpu.SemaphoreType.DMA
    out = pl.pallas_call(
        functools.partial(_kernel, S=S, D=D, H=H, DH=DH, M=M, SEG=SEG),
        out_shape=jax.ShapeDtypeStruct((S, D), A_x.dtype),
        in_specs=[any_spec] * 11,
        out_specs=any_spec,
        scratch_shapes=[
            pltpu.VMEM((KT, S + SEG, _LANE), _BF16),
            pltpu.VMEM((6 * KT, _LANE, H // 2, DH), _BF16),
            pltpu.VMEM((3 * H, D // 2, DH), _U32),
            pltpu.VMEM((KT, H * DH, _LANE), _BF16),
            pltpu.VMEM((n_ffn, D, units), _BF16),
            pltpu.VMEM((n_ffn, D, units), _BF16),
            pltpu.VMEM((n_ffn, KT, units, _LANE), _BF16),
            [pltpu.VMEM((12, fat, DH), _F32)] * (H // 4),
            pltpu.VMEM((KT // 2, 7, fat // 4, _LANE), _U32),
            pltpu.VMEM((20, KT, SEG, _LANE), _F32),
            pltpu.VMEM((4, L, DH), _F32),
            pltpu.VMEM((4, L, L), _F32),
            pltpu.VMEM((3 * H, M, DH), _F32),
            pltpu.VMEM((_TOPK, D), _F32),
            pltpu.VMEM((_TOPK, D), _F32),
            pltpu.VMEM((KT, M, _LANE), _BF16),
            pltpu.VMEM((KT, _LANE), _BF16),
            pltpu.VMEM((KT, _LANE), _BF16),
            pltpu.VMEM((KT, _LANE), _F32),
            pltpu.VMEM((_TOPK, _LANE), _F32),
            pltpu.SMEM((_TOPK,), _I32),
            dma((len(_BATCHES),)), dma((KT,)), dma(()), dma((2,)), dma(()), dma((n_ffn,)),
            dma(()),
        ],
        compiler_params=pltpu.CompilerParams(vmem_limit_bytes=120 * 1024 * 1024,
                                             disable_bounds_checks=True),
        name="gated_mix_rmt_mod",
    )(
        A_x.reshape(S, D), A_mem0.reshape(M, D), A_Wq.reshape(D, 2, H // 2, DH),
        A_Wk.reshape(D, 2, H // 2, DH), A_Wv.reshape(D, 2, H // 2, DH),
        A_Wo.reshape(H * DH, D), B_w_r.reshape(KT, _LANE), B_w_gate, B_w_up, B_w_down,
        gate_w.reshape(KT, _LANE),
    )
    return out.reshape(B, S, D)
```

```python
import functools

import jax
import jax.numpy as jnp
import numpy as np
from jax import lax
import jax.experimental.pallas as pl
import jax.experimental.pallas.tpu as pltpu

_F32 = jnp.float32
_BF16 = jnp.bfloat16
_U32 = jnp.uint32
_I32 = jnp.int32
_NN = (((1,), (0,)), ((), ()))
_NT = (((1,), (1,)), ((), ()))

_LANE = 128
_WORDS = _LANE // 2
_TOPK = 8
_JOB = 4
_FFN_TILES = 4
_STAGES = (1, 1, 1, 1, 2, 2, 4, 4, 8, 8, 8, 8)
_BATCHES = (1, 1, 1, 1, 2, 2, 4, 4, 4, 4, 4, 4, 8, 8)


def _dot(a, b, dims=_NN):
    return lax.dot_general(a, b, dims, preferred_element_type=_F32)


def _aligned(i, n):
    return i if isinstance(i, int) else pl.multiple_of(i, n)


def _rem(i, n):
    return i % n if isinstance(i, int) else lax.rem(i, n)


def _sigmoid(v):
    return 1.0 / (1.0 + jnp.exp(-v))


def _bf16(words):
    return pltpu.bitcast(words, _BF16)


def _words(v):
    return pltpu.bitcast(v, _U32)


def _sum(a, b, sign):
    a, b = _bf16(a).astype(_F32), _bf16(b).astype(_F32)
    return (a + b if sign > 0 else a - b).astype(_BF16)


def _start(copies):
    for cp in copies:
        cp.start()


def _wait(copies):
    for cp in copies:
        cp.wait()


def _kernel(x_hbm, mem_hbm, wq_hbm, wk_hbm, wv_hbm, wo_hbm, wr_hbm, wg_hbm, wu_hbm,
            wd_hbm, gw_hbm, out_hbm,
            xbuf, stage, wqkv, wo, wg, wu, wd, rings, xsum, abuf, obuf, pbuf, mqkv, xsel,
            ybuf, membuf, wr, gw, gwf, rgate, picks,
            sem_w, sem_xh, sem_xt, sem_small, sem_wo, sem_b, sem_out,
            *, S, D, H, DH, M, SEG):
    L = M + SEG
    n_seg = S // SEG
    KT = D // _LANE
    G = H // 4
    HH = H // 2
    XR = SEG - M
    HEAD = S - (n_seg - 1) * XR
    FAT = HEAD + M
    NB = wg.shape[0]
    PERIOD = SEG // M
    w_hbm = (wq_hbm, wk_hbm, wv_hbm)

    stage_u, xbuf_u, membuf_u, wo_u, wd_u = (
        r.bitcast(_U32) for r in (stage, xbuf, membuf, wo, wd))

    def ring(t):
        j, h = divmod(t, H)
        return rings[h // 4].at[j * 4 + h % 4]

    picks[0] = 0
    never = picks[0] > 0

    def after(other, v):
        return v if other is None else jnp.where(never, other, v)

    sublane = lax.broadcasted_iota(_I32, (8, _LANE), 0)

    batch_start = np.cumsum((0,) + _BATCHES).tolist()
    stage_start = np.cumsum((0,) + _STAGES).tolist()

    def batch_copies(i):
        copies = []
        for u in range(batch_start[i], batch_start[i + 1]):
            j, kt, half = u // (2 * KT), u // 2 % KT, u % 2
            if j == 0 and half == 0:
                copies.append(pltpu.make_async_copy(
                    x_hbm.at[pl.ds(0, FAT), pl.ds(kt * _LANE, _LANE)],
                    xbuf.at[kt, pl.ds(0, FAT), :], sem_xh.at[kt]))
            copies.append(pltpu.make_async_copy(
                w_hbm[j].at[pl.ds(kt * _LANE, _LANE), half], stage.at[u], sem_w.at[i]))
        return copies

    def strip_copies(src, dst, sem):
        return [pltpu.make_async_copy(src.at[:, pl.ds(n * _LANE, _LANE)], dst.at[n], sem)
                for n in range(KT)]

    def ffn_copies(i):
        units = pl.ds(_aligned(i * _FFN_TILES * _LANE, _LANE), _FFN_TILES * _LANE)
        return [pltpu.make_async_copy(wg_hbm.at[:, units], wg.at[i], sem_b.at[i]),
                pltpu.make_async_copy(wu_hbm.at[:, units], wu.at[i], sem_b.at[i])
                ] + strip_copies(wd_hbm.at[units, :], wd.at[i], sem_b.at[i])

    def out_copies(seg):
        rows = pl.ds(_aligned(seg * SEG, SEG), SEG)
        return [pltpu.make_async_copy(xbuf.at[kt, rows, :],
                                      out_hbm.at[rows, pl.ds(kt * _LANE, _LANE)], sem_out)
                for kt in range(KT)]

    mem_copies = strip_copies(mem_hbm, membuf, sem_small.at[0])
    rest_copies = [pltpu.make_async_copy(wr_hbm, wr, sem_small.at[1]),
                   pltpu.make_async_copy(gw_hbm, gw, sem_small.at[1])]
    rest_copies += [pltpu.make_async_copy(
        x_hbm.at[pl.ds(FAT, S - FAT), pl.ds(kt * _LANE, _LANE)],
        xbuf.at[kt, pl.ds(FAT, S - FAT), :], sem_xt) for kt in range(KT)]
    wo_copies = strip_copies(wo_hbm, wo, sem_wo)

    queue = [batch_copies(i) for i in range(len(_BATCHES))]
    queue += [rest_copies, wo_copies, ffn_copies(0), ffn_copies(1)]
    progress = {"started": 0, "arrived": 0}

    def start_next():
        _start(queue[progress["started"]])
        progress["started"] += 1

    def need_unit(u):
        while batch_start[progress["arrived"]] <= u:
            _wait(queue[progress["arrived"]])
            progress["arrived"] += 1
            start_next()

    row = lax.broadcasted_iota(_I32, (L, L), 0)
    col = lax.broadcasted_iota(_I32, (L, L), 1)
    mask = (row < M) | (row >= col)
    scale = DH ** (-0.5)

    def probs(q, k):
        sc = jnp.where(mask[L - q.shape[0]:], _dot(q, k, _NT), -1000000000.0 / scale)
        e = jnp.exp2((sc - jnp.max(sc, axis=-1, keepdims=True)) * float(scale * np.log2(np.e)))
        total = jnp.sum(e, axis=-1, keepdims=True)
        inv = pltpu.reciprocal(total, approx=True)
        return e * (inv * (2.0 - total * inv))

    def weighted(p, v):
        return _dot(p, v.astype(_BF16))

    n_blk = S // _LANE
    score = [None] * n_blk

    def score_job(b, half):
        kts = range(half * KT // 2, (half + 1) * KT // 2)
        wrf = wr[...].astype(_F32)
        w = jnp.concatenate([jnp.broadcast_to(wrf[kt:kt + 1], (8, _LANE)) for kt in kts],
                            axis=1)
        xb = jnp.concatenate([_bf16(xbuf_u[kt, pl.ds(b * _WORDS, _WORDS), :]) for kt in kts],
                             axis=1)
        r = _dot(w, xb, _NT)
        score[b] = r if half == 0 else r + score[b]

    def select_jobs():
        state = {}
        pos = (lax.broadcasted_iota(_I32, (n_blk, _LANE), 0) * _LANE
               + lax.broadcasted_iota(_I32, (n_blk, _LANE), 1)).astype(_F32)

        def job(c):
            if c == 0:
                r_all = []
                for b0 in range(0, n_blk, 8):
                    r = score[b0]
                    for b in range(1, 8):
                        r = jnp.where(sublane == b, score[b0 + b], r)
                    r_all.append(r)
                r_all = jnp.concatenate(r_all, axis=0).astype(_BF16).astype(_F32)
                r_all = jnp.where(r_all == 0.0, 0.0, r_all)
                bits = pltpu.bitcast(r_all, _I32)
                key = jnp.where(bits < 0, bits ^ np.int32(0x7FFFFFFF), bits) >> 16
                key = jnp.where(r_all != r_all, np.int32(-(1 << 15)), key)
                state.update(r=r_all, key=key.astype(_F32))
            best = jnp.max(state["key"], keepdims=True)
            pick = jnp.min(jnp.where(state["key"] == best, pos, float(S)), keepdims=True)
            hit = pos == pick
            state["key"] = jnp.where(hit, -float(1 << 17), state["key"])
            r_c = jnp.sum(jnp.where(hit, state["r"], 0.0), keepdims=True)
            rgate[pl.ds(c, 1), :] = jnp.broadcast_to(_sigmoid(r_c), (1, _LANE))
            token = pick[0, 0].astype(_I32)
            picks[c] = token
            base = pl.multiple_of((token >> 3) << 3, 8)
            for kt in range(KT):
                grp = xbuf[kt, pl.ds(base, 8), :].astype(_F32)
                one = jnp.sum(jnp.where(sublane == (token & 7), grp, 0.0), axis=0,
                              keepdims=True)
                xsel[pl.ds(c, 1), pl.ds(kt * _LANE, _LANE)] = one
            return _words(jnp.broadcast_to(one, (8, _LANE)))

        return [functools.partial(job, c) for c in range(_TOPK)]

    index_bits = [(lax.broadcasted_iota(_I32, (_JOB, 8, _LANE), 1) & d) != 0
                  for d in (1, 2, 4)]

    def transpose8(v):
        c = [v[0]] + [pltpu.roll(v[8 - m], 8 - m, 1) for m in range(1, 8)]
        for d, bit in zip((1, 2, 4), index_bits):
            c = [lax.select(bit, c[m - d], c[m]) for m in range(8)]
        return [c[0]] + [pltpu.roll(c[k], 8 - k, 1) for k in range(1, 8)]

    def relayout(u, d0, odd, prev=None):
        need_unit(u)
        j, kt, half = u // (2 * KT), u // 2 % KT, u % 2
        rows = stage_u[u, pl.ds(d0, 16 * _JOB)].reshape(_JOB, 8, 2, 8, _LANE)
        a, b = rows[:, :, 0], rows[:, :, 1]
        if odd:
            words = (a >> 16) | (b & np.uint32(0xFFFF0000))
        else:
            words = (a & np.uint32(0xFFFF)) | (b << 16)
        words = [words[:, t] for t in range(8)]
        words[0] = after(prev, words[0])
        for t, w in enumerate(transpose8(words)):
            wqkv[j * H + half * HH + 2 * t + odd, pl.ds(kt * _WORDS + d0 // 2, 8 * _JOB), :] = (
                w.reshape(8 * _JOB, _LANE))

    def relayout_jobs(units):
        return [functools.partial(relayout, u, d0, odd)
                for u in units for d0 in range(0, _LANE, 16 * _JOB) for odd in range(2)]

    def head_rows(kt, r0, n):
        n_x = min(n, HEAD // 2 - r0)
        rows = xbuf_u[kt, pl.ds(r0, n_x), :]
        return rows if n_x == n else jnp.concatenate([rows, membuf_u[kt]], axis=0)

    def xsum_rows(pair, r0, prev):
        a11, a12, a21, a22 = (head_rows(2 * pair + k, half * (FAT // 4) + r0, 8)
                              for half in range(2) for k in range(2))
        a11, a22 = after(prev, a11), after(prev, a22)
        factors = (_words(_sum(a11, a22, 1)), _words(_sum(a21, a22, 1)), a11, a22,
                   _words(_sum(a11, a12, 1)), _words(_sum(a21, a11, -1)),
                   _words(_sum(a12, a22, -1)))
        for k, w in enumerate(factors):
            xsum[pair, k, pl.ds(r0, 8), :] = w

    def xsum_jobs(pairs):
        def job(parts, prev):
            for e, (pair, r0) in enumerate(parts):
                xsum_rows(pair, r0, prev[e])

        parts = [(pair, r0) for pair in pairs for r0 in range(0, FAT // 4, 8)]
        return [functools.partial(job, parts[i:i + _JOB]) for i in range(0, len(parts), _JOB)]

    def run_share(jobs, i, n, result):
        mine = jobs[i * len(jobs) // n:(i + 1) * len(jobs) // n]
        for k, job in enumerate(mine):
            starts = [(k * _JOB + e) * (result.shape[0] // 8) // (len(mine) * _JOB) * 8
                      for e in range(_JOB)]
            job(_words(jnp.stack([result[r0:r0 + 8] for r0 in starts])))

    def project(j, kt, heads, jobs):
        lhs = _bf16(head_rows(kt, 0, FAT // 2))
        for i, h in enumerate(heads):
            r = _dot(lhs, _bf16(wqkv[j * H + h, pl.ds(kt * _WORDS, _WORDS), :]))
            dst = ring(j * H + h)
            dst[...] = r + dst[...] if kt > 0 else r
            if i % 4 == 3:
                run_share(jobs, i // 4, len(heads) // 4, r)

    def project_strassen(j, pairs, jobs, side=()):
        slot, due = [0], {}

        def product(k, b):
            lhs = [xsum[p, k - 1] for p in pairs]
            if slot[0] in due:
                lhs[0] = jnp.concatenate([after(due.pop(slot[0]), lhs[0][:8]), lhs[0][8:]],
                                         axis=0)
            return _dot(jnp.concatenate([_bf16(a) for a in lhs], axis=1), b)

        def block(h, k):
            return jnp.concatenate(
                [wqkv[j * H + h, pl.ds((2 * p + k) * _WORDS, _WORDS), :] for p in pairs],
                axis=0)

        def add(h, half, v, first=False, sign=1):
            rows = pl.ds(half * (FAT // 2), FAT // 2)
            dst = ring(j * H + h)
            if first and pairs[0] == 0:
                dst[rows, :] = v if sign > 0 else -v
            else:
                dst[rows, :] = dst[rows, :] + v if sign > 0 else dst[rows, :] - v

        def next_slot(m):
            run_share(jobs, slot[0], 7 * G, m)
            for job in side[slot[0]] if slot[0] in side else ():
                v = job()
                if v is not None:
                    due[slot[0] + 5] = v
            slot[0] += 1

        for g in range(G):
            for h in (4 * g, 4 * g + 2):
                m2 = product(2, _bf16(block(h, 0)))
                m5 = product(5, _bf16(block(h + 1, 1)))
                if len(pairs) > 1:
                    add(h, 1, m2, True)
                    add(h + 1, 1, m2, True, -1)
                    add(h, 0, m5, True, -1)
                    add(h + 1, 0, m5, True)
                next_slot(m2)
                m1 = product(1, _sum(block(h, 0), block(h + 1, 1), 1))
                m4 = product(4, _sum(block(h, 1), block(h, 0), -1))
                if len(pairs) > 1:
                    add(h, 0, m1 + m4)
                    add(h + 1, 1, m1)
                    add(h, 1, m4)
                else:
                    add(h, 0, m1 + m4 - m5, True)
                    add(h + 1, 1, m1 - m2, True)
                    add(h, 1, m2 + m4, True)
                    add(h + 1, 0, m5, True)
                next_slot(m1)
                m3 = product(3, _sum(block(h + 1, 0), block(h + 1, 1), -1))
                m6 = product(6, _sum(block(h, 0), block(h + 1, 0), 1))
                add(h + 1, 0, m3)
                add(h + 1, 1, m3 + m6)
                next_slot(m3)
            for h in (4 * g, 4 * g + 2):
                m7 = product(7, _sum(block(h, 1), block(h + 1, 1), 1))
                add(h, 0, m7)
            next_slot(m7)

    def first_segment(t):
        return jnp.concatenate([ring(t)[pl.ds(HEAD, M), :], ring(t)[pl.ds(0, SEG), :]], axis=0)

    p_first = []

    def first_scores():
        p_first.extend(probs(first_segment(h), first_segment(H + h)) for h in range(8))

    def first_values():
        for h in range(4):
            obuf[h] = weighted(p_first[h], first_segment(2 * H + h))
            pbuf[h] = p_first[4 + h]

    _start(mem_copies)
    start_next()
    _wait(mem_copies)
    start_next()
    for job in relayout_jobs([0]):
        job()
    for i, n in enumerate(_STAGES):
        u = stage_start[i]
        j, kt = u // (2 * KT), u // 2 % KT
        jobs = relayout_jobs(range(u + n, stage_start[min(i + 2, len(_STAGES))]))
        if i == 0:
            project(j, kt, range(HH), [])
            for job in jobs:
                job()
            continue
        if jobs:
            need_unit(u + n)
        if i in (7, 8):
            start_next()
        if i == len(_STAGES) - 2:
            _wait(rest_copies)
        if n <= 2:
            heads = range(H) if n == 2 else range(u % 2 * HH, (u % 2 + 1) * HH)
            project(j, kt, heads, jobs + (xsum_jobs([2]) if _STAGES[i + 1] > 2 else []))
        elif n == 4:
            project_strassen(j, [kt // 2], jobs + xsum_jobs([3] if kt == 4 else [0, 1]))
        elif jobs:
            project_strassen(j, [kt // 2, kt // 2 + 1], jobs)
        else:
            side = {q: [functools.partial(score_job, q // 2, q % 2)] for q in range(2 * n_blk)}
            side.update({2 * n_blk + 5 * c // 2: [job] for c, job in enumerate(select_jobs())})
            side[6].append(first_scores)
            side[20].append(first_values)
            project_strassen(j, [kt // 2, kt // 2 + 1], jobs, side)
    assert progress["started"] == len(queue)
    for t in range(3 * H):
        mqkv[t] = ring(t)[pl.ds(HEAD, M), :]
    gwf[...] = gw[...].astype(_F32)
    ybuf[...] = jnp.zeros(ybuf.shape, _F32)
    xbuf_u[:, pl.ds(S // 2, SEG // 2), :] = jnp.zeros((KT, SEG // 2, _LANE), _U32)

    def ffn_jobs(i):
        part, act = {}, []

        def up_job(w, k, half, _):
            span = pl.ds(half * (D // 2), D // 2)
            r = _dot(xsel[:, span], (wg, wu)[w][i, span, pl.ds(k * _LANE, _LANE)])
            part[w, k] = r if half == 0 else r + part[w, k]

        def down_job(n, _):
            if n == 0:
                act.extend(part[0, k] * _sigmoid(part[0, k]) * part[1, k]
                           for k in range(_FFN_TILES))
            r = _dot(jnp.concatenate(act, axis=1), _bf16(wd_u[i, n]))
            ybuf[:, pl.ds(n * _LANE, _LANE)] += r * rgate[...]

        ups = [functools.partial(up_job, w, k, half)
               for k in range(_FFN_TILES) for w in range(2) for half in range(2)]
        jobs = {1 + 5 * q // 2: job for q, job in enumerate(ups)}
        jobs.update({q: functools.partial(down_job, n)
                     for n, q in enumerate((45, 47, 50, 53, 55, 58, 61, 63))})
        return jobs

    seg_row = lax.broadcasted_iota(_I32, (SEG, _LANE), 0)

    def mix_jobs(seg, a, copies=None):
        rows = pl.ds(_aligned(seg * (SEG // 2), SEG // 2), SEG // 2)
        gate = []

        def gate_job(prev=None):
            z = after(prev, jnp.zeros((SEG, _LANE), _F32))
            for kt in range(KT):
                z = z + _bf16(xbuf_u[kt, rows, :]).astype(_F32) * gwf[pl.ds(kt, 1), :]
            gate.append(_sigmoid(jnp.sum(z, axis=-1, keepdims=True)))
            return jnp.broadcast_to(gate[0], (SEG, _LANE)).astype(_BF16)

        def strip_job(kt, prev=None):
            upd = after(prev, jnp.zeros((SEG, _LANE), _F32))
            for c in range(_TOPK):
                upd = jnp.where(seg_row == picks[c] - seg * SEG,
                                ybuf[pl.ds(c, 1), pl.ds(kt * _LANE, _LANE)], upd)
            b = _bf16(xbuf_u[kt, rows, :]).astype(_F32) + upd
            res = (gate[0] * a[kt] + (1.0 - gate[0]) * b).astype(_BF16)
            xbuf_u[kt, rows, :] = _words(res)
            if copies:
                copies[kt].start()
            return res

        return [gate_job] + [functools.partial(strip_job, kt) for kt in range(KT)]

    def attention(seg, r0=0):
        rows = pl.ds(_aligned(_rem(seg * SEG, FAT), SEG), SEG)
        o = {h: obuf[h, pl.ds(r0, L - r0), :] for h in range(4)}
        p = {4 + h: pbuf[h, pl.ds(r0, L - r0), :] for h in range(4)}

        def tok(t):
            return jnp.concatenate([mqkv[t], ring(t)[rows, :]], axis=0)

        def scores(g):
            for h in range(4 * g, min(4 * g + 4, H)):
                p[h] = probs(tok(h)[r0:], tok(H + h))

        def values(g):
            for h in range(4 * g, min(4 * g + 4, H)):
                o[h] = weighted(p[h], tok(2 * H + h))

        return o, scores, values

    def wo_block(g, n):
        return wo_u[n, pl.ds(g * 4 * _WORDS, 4 * _WORDS), :]

    def output_projection(attn, n_rows, jobs=()):
        o, scores, values = attn
        acc, due = [None] * KT, {}
        for g in range(G):
            lhs = [o[4 * g + i][:n_rows] for i in range(4)]
            if n_rows % 16 == 0:
                lhs = [v.astype(_BF16) for v in lhs]
            for n in range(KT):
                if n == 1:
                    scores(g + 2)
                if n == (4 if n_rows == SEG else 5):
                    values(g + 1)
                q = g * KT + n
                r = _dot(jnp.concatenate([after(due.get(q), lhs[0])] + lhs[1:], axis=1),
                         _bf16(wo_block(g, n)))
                acc[n] = r if g == 0 else r + acc[n]
                if q in jobs:
                    due[q + 17] = jobs[q](r)
        return acc

    def wo_sum_jobs(gp):
        def job(c, r0, prev):
            b11, b12, b21, b22 = (
                wo_u[2 * c + n, pl.ds(_aligned((2 * gp + g) * 4 * _WORDS + r0, SEG), SEG), :]
                for g in range(2) for n in range(2))
            b11, b22 = after(_words(prev), b11), after(_words(prev), b22)
            sums = [_words(v) for v in (_sum(b11, b22, 1), _sum(b12, b22, -1),
                                        _sum(b21, b11, -1), _sum(b11, b12, 1),
                                        _sum(b21, b22, 1))]
            for k, w in enumerate(sums):
                stage_u[gp * 5 + k, pl.ds(c * (_WORDS // 2) + r0 // 8, SEG // 8)] = (
                    w.reshape(SEG // 8, 8, _LANE))
            return _bf16(sums[-1][:SEG // 2])

        return [functools.partial(job, c, r0)
                for c in range(KT // 2) for r0 in range(0, 4 * _WORDS, SEG)]

    def output_projection_strassen(attn, held):
        o, scores, values = attn
        m = {}
        for gp in range(G // 2):
            due = {1: functools.partial(values, 2 * gp + 1),
                   2: functools.partial(scores, 2 * gp + 2),
                   12: functools.partial(scores, 2 * gp + 3),
                   20: functools.partial(values, 2 * gp + 2)}
            count = [0]

            def halves(g):
                heads = range(4 * g, 4 * g + 4)
                return (jnp.concatenate([jnp.concatenate([o[h][:M]] + [x[h] for x in held],
                                                         axis=0) for h in heads], axis=1),
                        jnp.concatenate([o[h][M:] for h in heads], axis=1))

            def products(k, lhs, factor):
                lhs = lhs.astype(_BF16)
                for c in range(KT // 2):
                    if count[0] in due:
                        due[count[0]]()
                    count[0] += 1
                    r = _dot(lhs, _bf16(factor(c)))
                    m[k, c] = r if gp == 0 else r + m[k, c]

            def kept(k):
                return lambda c: stage_u[gp * 5 + k, pl.ds(c * (_WORDS // 2), _WORDS // 2)
                                         ].reshape(4 * _WORDS, _LANE)

            a11, a21 = halves(2 * gp)
            products(3, a11, kept(1))
            products(6, a21 - a11, kept(3))
            a12, a22 = halves(2 * gp + 1)
            products(1, a11 + a22, kept(0))
            products(4, a22, kept(2))
            products(7, a12 - a22, kept(4))
            products(5, a11 + a12, lambda c: wo_block(2 * gp + 1, 2 * c + 1))
            products(2, a21 + a22, lambda c: wo_block(2 * gp, 2 * c))
        top, bottom = [], []
        for c in range(KT // 2):
            top += [m[1, c] + m[4, c] + m[7, c] - m[5, c], m[3, c] + m[5, c]]
            bottom += [m[2, c] + m[4, c], m[1, c] + m[3, c] + m[6, c] - m[2, c]]
        return top, bottom

    def project_memory(s, mem, jobs):
        x0 = HEAD + (s - 1) * XR
        wpos = [_aligned(_rem(x0 + 8 * i, FAT), 8) for i in range(XR // 8)]
        rows = pl.ds(_aligned(_rem(s * SEG, FAT), SEG), SEG)
        h_in = []
        for kt in range(KT):
            xw = xbuf_u[kt, pl.ds(_aligned((HEAD - M) // 2 + (s - 1) * (XR // 2), 4),
                                  SEG // 2), :]
            mw = _words(jnp.concatenate([mem[kt]] * 2, axis=0).astype(_BF16))
            h_in.append(_bf16(jnp.concatenate(
                [jnp.where(sublane < M // 2, mw, xw[:8]), xw[8:]], axis=0)))
        mem_rows, p, due = {}, {}, {}

        def weights(t, lo, hi):
            return _bf16(wqkv[t, pl.ds(lo * _WORDS, (hi - lo) * _WORDS), :])

        def finish(t, r):
            for i, w in enumerate(wpos):
                ring(t)[pl.ds(w, 8), :] = r[M + 8 * i:M + 8 * i + 8]
            mqkv[t] = mem_rows[t] = r[:M]

        def tok(t):
            return jnp.concatenate([mem_rows[t], ring(t)[rows, :]], axis=0)

        tiles = [j * H + h for h in range(H) for j in range(3)]
        lo = jnp.concatenate(h_in[:KT // 2], axis=1)
        hi = jnp.concatenate(h_in[KT // 2:], axis=1)
        part = [_dot(lo, weights(t, 0, KT // 2)) for t in tiles[:6]]
        for q, t in enumerate(tiles):
            if q < len(part):
                finish(t, _dot(hi, weights(t, KT // 2, KT)) + part[q])
                continue
            r = _dot(jnp.concatenate([after(due.get(q), h_in[0])] + h_in[1:], axis=1),
                     weights(t, 0, KT))
            finish(t, r)
            if q in jobs:
                due[q + 8] = jobs[q](r)
            if q == 74:
                for h in range(4):
                    p[h] = probs(tok(h), tok(H + h))
                for h in range(4):
                    pbuf[h] = probs(tok(4 + h), tok(H + 4 + h))
            if q == 86:
                for h in range(4):
                    obuf[h] = weighted(p[h], tok(2 * H + h))

    def slot(seg):
        return _rem(seg, abuf.shape[0])

    def block_rows(seg):
        return [abuf[slot(seg), n] for n in range(KT)]

    def ffn_step(i, carry):
        _wait(ffn_copies(i))
        pl.when(i + 2 < NB)(lambda: _start(ffn_copies(i + 2)))
        acc = output_projection(attention(i), L, ffn_jobs(i))
        for n in range(KT):
            abuf[i, n] = acc[n][M:]
        jobs = wo_sum_jobs(jnp.minimum(i, G // 2 - 1))
        project_memory(i + 1, [a[:M] for a in acc],
                       {7 + 2 * k: job for k, job in enumerate(jobs)})
        return carry

    n_old = NB - PERIOD + 1

    def main_steps(i, carry):
        held = []
        for k in range(PERIOD):
            seg = NB + i * PERIOD + k
            attn = attention(seg)
            if k < PERIOD - 1:
                acc = output_projection(attn, SEG)
                held.append({h: v[SEG:] for h, v in attn[0].items()})
                for n in range(KT):
                    abuf[slot(seg), n, pl.ds(0, XR), :] = acc[n][M:]
            else:
                acc, tokens = output_projection_strassen(attn, held)
                for n in range(KT):
                    abuf[slot(seg), n] = tokens[n]
                    for e in range(1, PERIOD):
                        abuf[slot(seg - PERIOD + e), n, pl.ds(XR, M), :] = (
                            acc[n][e * M:e * M + M])
            jobs = {}
            if k == 0:
                old = mix_jobs(jnp.where(i < n_old, i, n_seg), block_rows(i))
                jobs.update({10 + 6 * q: job for q, job in enumerate(old)})
            done = seg - PERIOD + 1
            jobs.update({7 + 6 * q: job
                         for q, job in enumerate(mix_jobs(done, block_rows(done)))})
            project_memory(seg + 1, [a[:M] for a in acc], jobs)
            _start(out_copies(done))
            if k == 0:
                pl.when(i < n_old)(lambda: _start(out_copies(i)))
        return carry

    assert (n_seg - 1 - NB) % PERIOD == 0
    _wait(wo_copies)
    lax.fori_loop(0, NB, ffn_step, 0)
    lax.fori_loop(0, (n_seg - 1 - NB) // PERIOD, main_steps, 0)
    jobs = [job for seg in range(n_seg - PERIOD, n_seg - 1)
            for job in mix_jobs(seg, block_rows(seg), out_copies(seg))]
    acc = output_projection(attention(n_seg - 1, M), SEG,
                            {q * 7 // 4: job for q, job in enumerate(jobs)})
    for job in mix_jobs(n_seg - 1, acc, out_copies(n_seg - 1)):
        job()
    pltpu.make_async_copy(out_hbm, out_hbm, sem_out).wait()


@functools.partial(jax.jit, static_argnames=("A_seg_len",))
def pallas_gated_mix__memory_aug_recurrent_mem_tr__moe_arch_mod__prompt_kernel(
    A_x, A_mem0, A_Wq, A_Wk, A_Wv, A_Wo, A_seg_len, B_x, B_w_r, B_w_gate, B_w_up,
    B_w_down, gate_w,
):
    del B_x
    B, S, D = A_x.shape
    _, H, DH = A_Wq.shape
    M = A_mem0.shape[1]
    SEG = int(A_seg_len)
    F = B_w_gate.shape[1]
    assert (B, S, D, H, DH, M, SEG, F) == (1, 2048, 1024, 32, _LANE, 8, 32, 3584)
    L = M + SEG
    KT = D // _LANE
    fat = S - (S // SEG - 1) * (SEG - M) + M
    units = _FFN_TILES * _LANE
    n_ffn = F // units

    any_spec = pl.BlockSpec(memory_space=pl.ANY)
    dma = pltpu.SemaphoreType.DMA
    out = pl.pallas_call(
        functools.partial(_kernel, S=S, D=D, H=H, DH=DH, M=M, SEG=SEG),
        out_shape=jax.ShapeDtypeStruct((S, D), A_x.dtype),
        in_specs=[any_spec] * 11,
        out_specs=any_spec,
        scratch_shapes=[
            pltpu.VMEM((KT, S + SEG, _LANE), _BF16),
            pltpu.VMEM((6 * KT, _LANE, H // 2, DH), _BF16),
            pltpu.VMEM((3 * H, D // 2, DH), _U32),
            pltpu.VMEM((KT, H * DH, _LANE), _BF16),
            pltpu.VMEM((n_ffn, D, units), _BF16),
            pltpu.VMEM((n_ffn, D, units), _BF16),
            pltpu.VMEM((n_ffn, KT, units, _LANE), _BF16),
            [pltpu.VMEM((12, fat, DH), _F32)] * (H // 4),
            pltpu.VMEM((KT // 2, 7, fat // 4, _LANE), _U32),
            pltpu.VMEM((20, KT, SEG, _LANE), _F32),
            pltpu.VMEM((4, L, DH), _F32),
            pltpu.VMEM((4, L, L), _F32),
            pltpu.VMEM((3 * H, M, DH), _F32),
            pltpu.VMEM((_TOPK, D), _F32),
            pltpu.VMEM((_TOPK, D), _F32),
            pltpu.VMEM((KT, M, _LANE), _BF16),
            pltpu.VMEM((KT, _LANE), _BF16),
            pltpu.VMEM((KT, _LANE), _BF16),
            pltpu.VMEM((KT, _LANE), _F32),
            pltpu.VMEM((_TOPK, _LANE), _F32),
            pltpu.SMEM((_TOPK,), _I32),
            dma((len(_BATCHES),)), dma((KT,)), dma(()), dma((2,)), dma(()), dma((n_ffn,)),
            dma(()),
        ],
        compiler_params=pltpu.CompilerParams(vmem_limit_bytes=120 * 1024 * 1024,
                                             disable_bounds_checks=True),
        name="gated_mix_rmt_mod",
    )(
        A_x.reshape(S, D), A_mem0.reshape(M, D), A_Wq.reshape(D, 2, H // 2, DH),
        A_Wk.reshape(D, 2, H // 2, DH), A_Wv.reshape(D, 2, H // 2, DH),
        A_Wo.reshape(H * DH, D), B_w_r.reshape(KT, _LANE), B_w_gate, B_w_up, B_w_down,
        gate_w.reshape(KT, _LANE),
    )
    return out.reshape(B, S, D)
```
